```python
import jax
import jax.numpy as jnp

def _softmax(x, axis=-1):
    return jax.nn.softmax(x, axis=axis)
def _gelu(x):
    return jax.nn.gelu(x, approximate=True)
def _silu(x):
    return jax.nn.silu(x)
def _sigmoid(x):
    return jax.nn.sigmoid(x)
def _layernorm(x, axis=-1, eps=1e-5):
    m = jnp.mean(x, axis=axis, keepdims=True)
    v = jnp.var(x, axis=axis, keepdims=True)
    return (x - m) / jnp.sqrt(v + eps)
def _scatter_add(tgt, idx, src, axis=0):
    return tgt.at[idx].add(src)
def _segment_sum(src, seg, n):
    return jax.ops.segment_sum(src, seg, n)
class _Rng:
    def __init__(self, key):
        self._k = key
    def _next(self):
        self._k, sub = jax.random.split(self._k)
        return sub
    def normal(self, shape):
        return jax.random.normal(self._next(), shape, dtype=jnp.bfloat16)
    def randint(self, lo, hi, shape):
        return jax.random.randint(self._next(), shape, lo, hi, dtype=jnp.int32)
    def uniform(self, shape, lo=0.0, hi=1.0):
        return jax.random.uniform(self._next(), shape, jnp.bfloat16, lo, hi)
    def permutation(self, n):
        return jax.random.permutation(self._next(), n)


kernel_name = 'standalone__adm_resblock__diffusion'

def setup_inputs():
    _rng = _Rng(jax.random.key(int.from_bytes(__import__("os").urandom(4), "little")))
    _w = (lambda a: (lambda t: t.astype(jnp.bfloat16) if jnp.issubdtype(t.dtype, jnp.floating) else t)(jnp.asarray(a)))
    B, C, HW, E = 2, 512, 64, 1152
    sc = (9.0 * C) ** -0.5
    return {
        "x": _w((lambda *s: _rng.normal(s) * 0.05)(B, C, HW, HW)),
        "t_emb": _w((lambda *s: _rng.normal(s) * 0.05)(B, E)),
        "g1": _w(1.0 + 0.1 * (lambda *s: _rng.normal(s) * 0.05)(C)),
        "be1": _w(0.1 * (lambda *s: _rng.normal(s) * 0.05)(C)),
        "w1": _w((lambda *s: _rng.normal(s) * 0.05)(C, C, 3, 3) * sc),
        "w_emb": _w((lambda *s: _rng.normal(s) * 0.05)(E, C) * (E ** -0.5)),
        "g2": _w(1.0 + 0.1 * (lambda *s: _rng.normal(s) * 0.05)(C)),
        "be2": _w(0.1 * (lambda *s: _rng.normal(s) * 0.05)(C)),
        "w2": _w((lambda *s: _rng.normal(s) * 0.05)(C, C, 3, 3) * sc),
    }

def reference(x, t_emb, g1, be1, w1, w_emb, g2, be2, w2):
    B, C, H, W = x.shape
    G, eps = 4, 1e-5
    def gn(z, gamma, beta):
        zr = z.reshape(B, G, (C // G) * H * W)
        mu = zr.mean(-1).reshape(B, G, 1)
        var = ((zr - mu) ** 2).mean(-1).reshape(B, G, 1)
        zn = ((zr - mu) / jnp.sqrt(var + eps)).reshape(B, C, H, W)
        return zn * gamma.reshape(1, C, 1, 1) + beta.reshape(1, C, 1, 1)
    def conv3(z, w):
        zp = jnp.pad(z, ((0, 0), (0, 0), (1, 1), (1, 1)))
        taps = [jnp.einsum("bchw,oc->bohw", zp[:, :, i:i+H, j:j+W], w[:, :, i, j]) for i in range(3) for j in range(3)]
        out = taps[0]
        for t in taps[1:]:
            out = out + t
        return out
    h = conv3(_silu(gn(x, g1, be1)), w1)
    emb = _silu(t_emb) @ w_emb
    h = h + emb.reshape(B, C, 1, 1)
    h = conv3(_silu(gn(h, g2, be2)), w2)
    return x + h
```

```python
import functools
import jax
import jax.numpy as jnp
from jax import lax
from jax.experimental import pallas as pl
from jax.experimental.pallas import tpu as pltpu

B, C, H, W, E = 2, 512, 64, 64, 1152
G = 4
EPS = 1e-5
NCH = C // 128
WT = W // 2
SLOT = 40
NR = (H + 2) * SLOT + 8
T = 8
NU = (H // 2) // T
M = T * WT

F32 = jnp.float32
BF16 = jnp.bfloat16
U32 = jnp.uint32


def _unpack(w):
    e = pltpu.unpack_elementwise(w, index=0, packed_dtype=BF16, unpacked_dtype=F32)
    o = pltpu.unpack_elementwise(w, index=1, packed_dtype=BF16, unpacked_dtype=F32)
    return e, o


def _kernel(x_hbm, temb_ref, g1_ref, be1_ref, w1_hbm, wemb_ref, g2_ref, be2_ref, w2_hbm,
            out_hbm,
            xs, hs, wraw, wt, planes, st, scs, sems):
    def x_copy(b, c):
        return pltpu.make_async_copy(
            x_hbm.at[b, :, pl.ds(c * 128, 128)], xs.bitcast(BF16).at[b, c], sems.at[b * NCH + c])

    def w_copy(k):
        src = w1_hbm if k == 0 else w2_hbm
        return pltpu.make_async_copy(src, wraw.at[k], sems.at[8 + k])

    def out_copy(b, u, c):
        rows = 2 * T * W
        return pltpu.make_async_copy(
            xs.bitcast(BF16).at[b, c, pl.ds(u * rows, rows)],
            out_hbm.at[b, pl.ds(u * rows, rows), pl.ds(c * 128, 128)],
            sems.at[10 + (b * NU + u) * NCH + c])

    for c in range(NCH):
        x_copy(0, c).start()
    w_copy(0).start()
    for c in range(NCH):
        x_copy(1, c).start()
    w_copy(1).start()

    zero8 = jnp.zeros((8, 128), F32)
    zero32 = jnp.zeros((32, 128), F32)
    for p in range(2):
        for c in range(NCH):
            def zb(s, _):
                planes[p, c, pl.ds(pl.multiple_of(s * SLOT, 8), 8), :] = zero8
                return 0
            lax.fori_loop(0, H + 3, zb, 0)
            planes[p, c, pl.ds(8, 32), :] = zero32
            planes[p, c, pl.ds((H + 1) * SLOT + 8, 32), :] = zero32

    te = temb_ref[...].astype(F32)
    th = 0.5 * te
    sil = th + th * jnp.tanh(th)
    emb = jnp.dot(sil.astype(BF16), wemb_ref[...], preferred_element_type=F32)

    def x_stats(b):
        for u in range(NU):
            for c in range(NCH):
                r0 = u * 16 * WT
                w0 = xs[b, c, pl.ds(r0, 8), :]
                piv = _unpack(w0)[0][0:1, :]

                def body(r, carry):
                    s1, s2 = carry
                    w = xs[b, c, pl.ds(pl.multiple_of(r0 + r * WT, 8), WT), :]
                    e, o = _unpack(w)
                    for v in (e, o):
                        d = v - piv
                        dd = d * d
                        for q in range(WT // 8):
                            s1 = s1 + d[q * 8:(q + 1) * 8]
                            s2 = s2 + dd[q * 8:(q + 1) * 8]
                    return s1, s2
                s1, s2 = lax.fori_loop(0, 16, body, (zero8, zero8))
                st[b, u, 0:1, pl.ds(c * 128, 128)] = piv
                st[b, u, 1:2, pl.ds(c * 128, 128)] = jnp.sum(s1, axis=0, keepdims=True)
                st[b, u, 2:3, pl.ds(c * 128, 128)] = jnp.sum(s2, axis=0, keepdims=True)

    def finalize(b, gam_ref, bet_ref, off):
        n = float(16 * W)
        gam = gam_ref[...].astype(F32)
        bet = bet_ref[...].astype(F32)
        means = []
        m2s = []
        for u in range(NU):
            piv = st[b, u, 0:1, :]
            s1 = st[b, u, 1:2, :]
            s2 = st[b, u, 2:3, :]
            mu = piv + s1 * (1.0 / n)
            if off is not None:
                mu = mu + off
            means.append(mu)
            m2s.append(s2 - s1 * s1 * (1.0 / n))
        for c in range(NCH):
            sl = slice(c * 128, (c + 1) * 128)
            tot = means[0][:, sl]
            for u in range(1, NU):
                tot = tot + means[u][:, sl]
            gmean = jnp.sum(tot, axis=1, keepdims=True) * (1.0 / (NU * 128))
            acc = jnp.zeros((1, 128), F32)
            for u in range(NU):
                dm = means[u][:, sl] - gmean
                acc = acc + m2s[u][:, sl] + n * dm * dm
            var = jnp.sum(acc, axis=1, keepdims=True) * (1.0 / (NU * 128 * n))
            rstd = lax.rsqrt(var + EPS)
            sc = 0.5 * gam[:, sl] * rstd
            sh = 0.5 * bet[:, sl] - gmean * sc
            scs[0:1, sl] = sc
            scs[1:2, sl] = sh

    def act_pass(src, b):
        def body(h, _):
            for c in range(NCH):
                sc = scs[0:1, pl.ds(c * 128, 128)]
                sh = scs[1:2, pl.ds(c * 128, 128)]
                w = src[b, c, pl.ds(pl.multiple_of(h * WT, 8), WT), :]
                e, o = _unpack(w)
                dst = pl.multiple_of((h + 1) * SLOT + 8, 8)
                for p, v in ((0, e), (1, o)):
                    uu = v * sc + sh
                    planes[p, c, pl.ds(dst, WT), :] = uu + uu * jnp.tanh(uu)
            return 0
        lax.fori_loop(0, H, body, 0)

    def w_transform(k):
        RB = 16

        def body(rb, _):
            r0 = pl.multiple_of(rb * RB, RB)
            for c in range(NCH):
                g = [[wraw[k, kh * 3 + kw, pl.ds(r0, RB), pl.ds(c * 128, 128)].astype(F32)
                      for kw in range(3)] for kh in range(3)]
                t = []
                for kw in range(3):
                    s = g[0][kw] + g[2][kw]
                    t.append([g[0][kw], 0.5 * (s + g[1][kw]), 0.5 * (s - g[1][kw]), g[2][kw]])
                for i in range(4):
                    s = t[0][i] + t[2][i]
                    row = [t[0][i], 0.5 * (s + t[1][i]), 0.5 * (s - t[1][i]), t[2][i]]
                    for j in range(4):
                        wt[k, i * 4 + j, pl.ds(r0, RB), pl.ds(c * 128, 128)] = row[j].astype(BF16)
            return 0
        lax.fori_loop(0, C // RB, body, 0)

    COL = {0: (1, 7), 1: (0, 8), 2: (1, 8), 3: (0, 9)}
    WJ = {0: (0, 2, -1), 1: (1, 2, 1), 2: (2, 1, -1), 3: (1, 3, -1)}

    def pm(a, b, s):
        return a + b if s > 0 else a - b

    def conv_unit(k, b, u, embrow):
        base = pl.multiple_of(u * (2 * T * SLOT), 8)

        def d(col, c, s):
            p, off = COL[col]
            return planes[p, c, pl.ds(base + s * SLOT + off, WT), :]

        Y = [[None, None], [None, None]]
        for j in range(4):
            ca, cb, sg = WJ[j]
            V = [[pm(d(ca, c, s), d(cb, c, s), sg) for s in range(2 * T + 2)] for c in range(NCH)]
            m = []
            for i in range(4):
                ra, rb, sgi = WJ[i]
                rows = []
                for t in range(T):
                    rows.append(jnp.concatenate(
                        [pm(V[c][2 * t + ra], V[c][2 * t + rb], sgi).astype(BF16) for c in range(NCH)],
                        axis=1))
                U = jnp.concatenate(rows, axis=0)
                m.append(lax.dot_general(U, wt[k, i * 4 + j], (((1,), (1,)), ((), ())),
                                         preferred_element_type=F32))
            z = [m[0] + m[1] + m[2], m[1] - m[2] - m[3]]
            for a in range(2):
                if j == 0:
                    Y[a][0] = z[a]
                elif j == 1:
                    Y[a][0] = Y[a][0] + z[a]
                    Y[a][1] = z[a]
                elif j == 2:
                    Y[a][0] = Y[a][0] + z[a]
                    Y[a][1] = Y[a][1] - z[a]
                else:
                    Y[a][1] = Y[a][1] - z[a]
        for c in range(NCH):
            cs = slice(c * 128, (c + 1) * 128)
            if k == 0:
                piv = Y[0][0][0:1, cs]
                s1 = zero8
                s2 = zero8
                ec = embrow[:, cs]
            for t in range(T):
                for a in range(2):
                    ye = Y[a][0][t * WT:(t + 1) * WT, cs]
                    yo = Y[a][1][t * WT:(t + 1) * WT, cs]
                    row = pl.multiple_of((u * 2 * T + 2 * t + a) * WT, 8)
                    if k == 0:
                        for v in (ye, yo):
                            dd = v - piv
                            d2 = dd * dd
                            for q in range(WT // 8):
                                s1 = s1 + dd[q * 8:(q + 1) * 8]
                                s2 = s2 + d2[q * 8:(q + 1) * 8]
                        hs[b, c, pl.ds(row, WT), :] = pltpu.pack_elementwise(
                            [ye + ec, yo + ec], packed_dtype=BF16)
                    else:
                        xe, xo = _unpack(xs[b, c, pl.ds(row, WT), :])
                        xs[b, c, pl.ds(row, WT), :] = pltpu.pack_elementwise(
                            [ye + xe, yo + xo], packed_dtype=BF16)
            if k == 0:
                st[b, u, 0:1, pl.ds(c * 128, 128)] = piv
                st[b, u, 1:2, pl.ds(c * 128, 128)] = jnp.sum(s1, axis=0, keepdims=True)
                st[b, u, 2:3, pl.ds(c * 128, 128)] = jnp.sum(s2, axis=0, keepdims=True)

    w_copy(0).wait()
    w_transform(0)
    for c in range(NCH):
        x_copy(0, c).wait()
    for c in range(NCH):
        x_copy(1, c).wait()
    w_copy(1).wait()
    w_transform(1)

    def img_loop1(b, _):
        x_stats(b)
        finalize(b, g1_ref, be1_ref, None)
        act_pass(xs, b)
        embrow = jnp.where(b == 0, emb[0:1, :], emb[1:2, :])

        def ub(u, _):
            conv_unit(0, b, u, embrow)
            return 0
        lax.fori_loop(0, NU, ub, 0)
        finalize(b, g2_ref, be2_ref, embrow)
        act_pass(hs, b)

        def ub2(u, _):
            conv_unit(1, b, u, None)
            for c in range(NCH):
                out_copy(b, u, c).start()
            return 0
        lax.fori_loop(0, NU, ub2, 0)
        return 0
    lax.fori_loop(0, B, img_loop1, 0)
    for b in range(B):
        for u in range(NU):
            for c in range(NCH):
                out_copy(b, u, c).wait()


@jax.jit
def pallas_standalone__adm_resblock__diffusion_kernel(x, t_emb, g1, be1, w1, w_emb, g2, be2, w2):
    xn = jnp.transpose(x, (0, 2, 3, 1)).reshape(B, H * W, C)
    w1n = jnp.transpose(w1, (2, 3, 0, 1)).reshape(9, C, C)
    w2n = jnp.transpose(w2, (2, 3, 0, 1)).reshape(9, C, C)
    temb = jnp.pad(t_emb, ((0, 8 - B), (0, 0)))
    vm = pl.BlockSpec(memory_space=pltpu.VMEM)
    hbm = pl.BlockSpec(memory_space=pl.ANY)
    out = pl.pallas_call(
        _kernel,
        out_shape=jax.ShapeDtypeStruct((B, H * W, C), BF16),
        in_specs=[hbm, vm, vm, vm, hbm, vm, vm, vm, hbm],
        out_specs=hbm,
        scratch_shapes=[
            pltpu.VMEM((B, NCH, H * WT, 128), U32),
            pltpu.VMEM((B, NCH, H * WT, 128), U32),
            pltpu.VMEM((2, 9, C, C), BF16),
            pltpu.VMEM((2, 16, C, C), BF16),
            pltpu.VMEM((2, NCH, NR, 128), F32),
            pltpu.VMEM((B, NU, 8, C), F32),
            pltpu.VMEM((8, C), F32),
            pltpu.SemaphoreType.DMA((10 + B * NU * NCH,)),
        ],
        compiler_params=pltpu.CompilerParams(vmem_limit_bytes=110 * 1024 * 1024),
    )(xn, temb, g1.reshape(1, C), be1.reshape(1, C), w1n, w_emb, g2.reshape(1, C), be2.reshape(1, C), w2n)
    return jnp.transpose(out.reshape(B, H, W, C), (0, 3, 1, 2))
```

```python
import functools
import jax
import jax.numpy as jnp
from jax import lax
from jax.experimental import pallas as pl
from jax.experimental.pallas import tpu as pltpu

B, C, H, W, E = 2, 512, 64, 64, 1152
G = 4
EPS = 1e-5
NCH = C // 128
WT = W // 2
SLOT = 40
T = 8
NS = 2 * T + 2
NR = NS * SLOT + 8
NU = (H // 2) // T
M = T * WT

F32 = jnp.float32
BF16 = jnp.bfloat16
U32 = jnp.uint32
PACE = 1


def _unpack(w):
    e = pltpu.unpack_elementwise(w, index=0, packed_dtype=BF16, unpacked_dtype=F32)
    o = pltpu.unpack_elementwise(w, index=1, packed_dtype=BF16, unpacked_dtype=F32)
    return e, o


def _kernel(x_hbm, temb_ref, g1_ref, be1_ref, w1_hbm, wemb_ref, g2_ref, be2_ref, w2_hbm,
            out_hbm,
            S, wraw, wt, PA, PB, st, scs, embs, sems):
    def x_copy(b, c):
        return pltpu.make_async_copy(
            x_hbm.at[b, :, pl.ds(c * 128, 128)], S.bitcast(BF16).at[b, c], sems.at[b * NCH + c])

    def w_copy(k):
        src = w1_hbm if k == 0 else w2_hbm
        return pltpu.make_async_copy(src, wraw.at[k], sems.at[8 + k])

    def out_copy(b, u, c):
        rows = 2 * T * W
        r0 = pl.multiple_of(u * rows, rows)
        return pltpu.make_async_copy(
            S.bitcast(BF16).at[b, c, pl.ds(r0, rows)],
            out_hbm.at[b, pl.ds(r0, rows), pl.ds(c * 128, 128)],
            sems.at[10 + (b * NU + u) * NCH + c])

    for c in range(NCH):
        x_copy(0, c).start()
    w_copy(0).start()
    for c in range(NCH):
        x_copy(1, c).start()
    w_copy(1).start()

    zero8 = jnp.zeros((8, 128), F32)
    for P in (PA, PB):
        for p in range(2):
            for c in range(NCH):
                for s in range(NS + 1):
                    P[p, c, pl.ds(s * SLOT, 8), :] = zero8

    te = temb_ref[...].astype(F32)
    th = 0.5 * te
    sil = th + th * jnp.tanh(th)
    emb = jnp.dot(sil.astype(BF16), wemb_ref[...], preferred_element_type=F32)
    for b in range(B):
        embs[b] = jnp.broadcast_to(emb[b:b + 1, :], (8, C))
    embs[2] = jnp.zeros((8, C), F32)

    def x_stats(b):
        for u in range(NU):
            for c in range(NCH):
                r0 = u * 16 * WT
                w0 = S[b, c, pl.ds(r0, 8), :]
                piv = _unpack(w0)[0][0:1, :]

                def body(r, carry):
                    s1, s2 = carry
                    w = S[b, c, pl.ds(pl.multiple_of(r0 + r * WT, 8), WT), :]
                    e, o = _unpack(w)
                    for v in (e, o):
                        d = v - piv
                        dd = d * d
                        for q in range(WT // 8):
                            s1 = s1 + d[q * 8:(q + 1) * 8]
                            s2 = s2 + dd[q * 8:(q + 1) * 8]
                    return s1, s2
                s1, s2 = lax.fori_loop(0, 16, body, (zero8, zero8))
                st[b, u, 0:1, pl.ds(c * 128, 128)] = piv
                st[b, u, 1:2, pl.ds(c * 128, 128)] = jnp.sum(s1, axis=0, keepdims=True)
                st[b, u, 2:3, pl.ds(c * 128, 128)] = jnp.sum(s2, axis=0, keepdims=True)

    def finalize(b, kdst, gam_ref, bet_ref, off):
        n = float(16 * W)
        gam = gam_ref[...].astype(F32)
        bet = bet_ref[...].astype(F32)
        means = []
        m2s = []
        for u in range(NU):
            piv = st[b, u, 0:1, :]
            s1 = st[b, u, 1:2, :]
            s2 = st[b, u, 2:3, :]
            mu = piv + s1 * (1.0 / n)
            if off is not None:
                mu = mu + off
            means.append(mu)
            m2s.append(s2 - s1 * s1 * (1.0 / n))
        for c in range(NCH):
            sl = slice(c * 128, (c + 1) * 128)
            tot = means[0][:, sl]
            for u in range(1, NU):
                tot = tot + means[u][:, sl]
            gmean = jnp.sum(tot, axis=1, keepdims=True) * (1.0 / (NU * 128))
            acc = jnp.zeros((1, 128), F32)
            for u in range(NU):
                dm = means[u][:, sl] - gmean
                acc = acc + m2s[u][:, sl] + n * dm * dm
            var = jnp.sum(acc, axis=1, keepdims=True) * (1.0 / (NU * 128 * n))
            rstd = lax.rsqrt(var + EPS)
            sc = 0.5 * gam[:, sl] * rstd
            sh = 0.5 * bet[:, sl] - gmean * sc
            scs[kdst, 0:1, sl] = sc
            scs[kdst, 1:2, sl] = sh

    def act_rows(n, P, slots, pace=None):
        k = n // NU
        u = n % NU
        for idx, s in enumerate(slots):
            h = u * (2 * T) - 1 + s
            edge = s == 0 or s == NS - 1
            if edge:
                valid = jnp.logical_and(h >= 0, h < H)
                h = jnp.clip(h, 0, H - 1)
            for c in range(NCH):
                sc = scs[k, 0:1, pl.ds(c * 128, 128)]
                sh = scs[k, 1:2, pl.ds(c * 128, 128)]
                w = S[k, c, pl.ds(pl.multiple_of(h * WT, 8), WT), :]
                if pace is not None:
                    z = pace(idx, c)
                    w = w | jnp.concatenate([z] * (WT // 8), axis=0)
                e, o = _unpack(w)
                for p, v in ((0, e), (1, o)):
                    uu = v * sc + sh
                    a = uu + uu * jnp.tanh(uu)
                    if edge:
                        a = jnp.where(valid, a, 0.0)
                    P[p, c, pl.ds(s * SLOT + 8, WT), :] = a

    def w_transform(k):
        RB = 16

        def body(rb, _):
            r0 = pl.multiple_of(rb * RB, RB)
            for c in range(NCH):
                g = [[wraw[k, kh * 3 + kw, pl.ds(r0, RB), pl.ds(c * 128, 128)].astype(F32)
                      for kw in range(3)] for kh in range(3)]
                t = []
                for kw in range(3):
                    s = g[0][kw] + g[2][kw]
                    t.append([g[0][kw], 0.5 * (s + g[1][kw]), 0.5 * (s - g[1][kw]), g[2][kw]])
                for i in range(4):
                    s = t[0][i] + t[2][i]
                    row = [t[0][i], 0.5 * (s + t[1][i]), 0.5 * (s - t[1][i]), t[2][i]]
                    for j in range(4):
                        wt[k, i * 4 + j, c, pl.ds(r0, RB), :] = row[j].astype(BF16)
            return 0
        lax.fori_loop(0, C // RB, body, 0)

    COL = {0: (1, 7), 1: (0, 8), 2: (1, 8), 3: (0, 9)}
    WJ = {0: (0, 2, -1), 1: (1, 2, 1), 2: (2, 1, -1), 3: (1, 3, -1)}

    def pm(a, b, s):
        return a + b if s > 0 else a - b

    def conv_unit(k, n, P, Pn):
        b = (n // NU) % B
        u = n % NU
        nn = jnp.minimum(n + 1, 4 * NU - 1)
        if not PACE:
            act_rows(nn, Pn, range(NS))

        def d(col, c, s):
            p, off = COL[col]
            return P[p, c, pl.ds(s * SLOT + off, WT), :]

        Y = [[None, None], [None, None]]
        ms = []
        for j in range(4):
            ca, cb, sg = WJ[j]
            V = [[pm(d(ca, c, s), d(cb, c, s), sg) for s in range(NS)] for c in range(NCH)]
            m = []
            for i in range(4):
                ra, rb, sgi = WJ[i]
                rows = []
                for t in range(T):
                    rows.append(jnp.concatenate(
                        [pm(V[c][2 * t + ra], V[c][2 * t + rb], sgi) for c in range(NCH)],
                        axis=1))
                U = jnp.concatenate(rows, axis=0).astype(BF16)
                Wm = jnp.concatenate([wt[k, i * 4 + j, c] for c in range(NCH)], axis=1)
                m.append(lax.dot_general(U, Wm, (((1,), (1,)), ((), ())),
                                         preferred_element_type=F32))
            ms.append(m)
            z = [m[0] + m[1] + m[2], m[1] - m[2] - m[3]]
            for a in range(2):
                if j == 0:
                    Y[a][0] = z[a]
                elif j == 1:
                    Y[a][0] = Y[a][0] + z[a]
                    Y[a][1] = z[a]
                elif j == 2:
                    Y[a][0] = Y[a][0] + z[a]
                    Y[a][1] = Y[a][1] - z[a]
                else:
                    Y[a][1] = Y[a][1] - z[a]
        if PACE:
            zmask = pltpu.bitcast(embs[2, :, 0:128], U32)

            def pace(idx, c):
                q = idx * NCH + c
                ph = (q * 56) // (NS * NCH)
                mi, nt = ph // 4, ph % 4
                j, i = mi // 4, mi % 4
                r = ((q * 5) % 4) * 64
                v = ms[j][i][r:r + 8, nt * 128:(nt + 1) * 128]
                return pltpu.bitcast(v, U32) & zmask
            act_rows(nn, Pn, range(NS), pace)
        for c in range(NCH):
            cs = slice(c * 128, (c + 1) * 128)
            if k == 0:
                piv = Y[0][0][0:1, cs]
                s1 = zero8
                s2 = zero8
                ec = embs[b, 0:1, pl.ds(c * 128, 128)]
            for t in range(T):
                for a in range(2):
                    ye = Y[a][0][t * WT:(t + 1) * WT, cs]
                    yo = Y[a][1][t * WT:(t + 1) * WT, cs]
                    row = pl.multiple_of((u * 2 * T + 2 * t + a) * WT, 8)
                    if k == 0:
                        for v in (ye, yo):
                            dd = v - piv
                            d2 = dd * dd
                            for q in range(WT // 8):
                                s1 = s1 + dd[q * 8:(q + 1) * 8]
                                s2 = s2 + d2[q * 8:(q + 1) * 8]
                        S[2 + b, c, pl.ds(row, WT), :] = pltpu.pack_elementwise(
                            [ye + ec, yo + ec], packed_dtype=BF16)
                    else:
                        xe, xo = _unpack(S[b, c, pl.ds(row, WT), :])
                        S[b, c, pl.ds(row, WT), :] = pltpu.pack_elementwise(
                            [ye + xe, yo + xo], packed_dtype=BF16)
            if k == 0:
                st[b, u, 0:1, pl.ds(c * 128, 128)] = piv
                st[b, u, 1:2, pl.ds(c * 128, 128)] = jnp.sum(s1, axis=0, keepdims=True)
                st[b, u, 2:3, pl.ds(c * 128, 128)] = jnp.sum(s2, axis=0, keepdims=True)
        if k == 1:
            for c in range(NCH):
                out_copy(b, u, c).start()

    for c in range(NCH):
        x_copy(0, c).wait()
    x_stats(0)
    finalize(0, 0, g1_ref, be1_ref, None)
    act_rows(0, PA, range(NS))
    w_copy(0).wait()
    w_transform(0)

    def pair1(p, _):
        @pl.when(p >= 0)
        def _():
            conv_unit(0, 2 * p, PA, PB)

        @pl.when(p >= -1)
        def _():
            conv_unit(0, 2 * p + 1, PB, PA)

        @pl.when(p == 0)
        def _():
            for c in range(NCH):
                x_copy(1, c).wait()
            x_stats(1)
            finalize(1, 1, g1_ref, be1_ref, None)
            w_copy(1).wait()
            w_transform(1)

        @pl.when(p == 1)
        def _():
            finalize(0, 2, g2_ref, be2_ref, embs[0, 0:1, :])

        @pl.when(p == 3)
        def _():
            finalize(1, 3, g2_ref, be2_ref, embs[1, 0:1, :])
        return 0
    lax.fori_loop(0, 4, pair1, 0)

    def pair2(p, _):
        @pl.when(p >= 0)
        def _():
            conv_unit(1, 2 * p, PA, PB)

        @pl.when(p >= -1)
        def _():
            conv_unit(1, 2 * p + 1, PB, PA)
        return 0
    lax.fori_loop(4, 8, pair2, 0)
    for b in range(B):
        for u in range(NU):
            for c in range(NCH):
                out_copy(b, u, c).wait()


@jax.jit
def pallas_standalone__adm_resblock__diffusion_kernel(x, t_emb, g1, be1, w1, w_emb, g2, be2, w2):
    xn = jnp.transpose(x, (0, 2, 3, 1)).reshape(B, H * W, C)
    w1n = jnp.transpose(w1, (2, 3, 0, 1)).reshape(9, C, C)
    w2n = jnp.transpose(w2, (2, 3, 0, 1)).reshape(9, C, C)
    temb = jnp.pad(t_emb, ((0, 8 - B), (0, 0)))
    vm = pl.BlockSpec(memory_space=pltpu.VMEM)
    hbm = pl.BlockSpec(memory_space=pl.ANY)
    out = pl.pallas_call(
        _kernel,
        out_shape=jax.ShapeDtypeStruct((B, H * W, C), BF16),
        in_specs=[hbm, vm, vm, vm, hbm, vm, vm, vm, hbm],
        out_specs=hbm,
        scratch_shapes=[
            pltpu.VMEM((4, NCH, H * WT, 128), U32),
            pltpu.VMEM((2, 9, C, C), BF16),
            pltpu.VMEM((2, 16, NCH, C, 128), BF16),
            pltpu.VMEM((2, NCH, NR, 128), F32),
            pltpu.VMEM((2, NCH, NR, 128), F32),
            pltpu.VMEM((B, NU, 8, C), F32),
            pltpu.VMEM((4, 8, C), F32),
            pltpu.VMEM((3, 8, C), F32),
            pltpu.SemaphoreType.DMA((10 + B * NU * NCH,)),
        ],
        compiler_params=pltpu.CompilerParams(vmem_limit_bytes=110 * 1024 * 1024),
    )(xn, temb, g1.reshape(1, C), be1.reshape(1, C), w1n, w_emb, g2.reshape(1, C), be2.reshape(1, C), w2n)
    return jnp.transpose(out.reshape(B, H, W, C), (0, 3, 1, 2))
```

```python
import jax
import jax.numpy as jnp
from jax import lax
from jax.experimental import pallas as pl
from jax.experimental.pallas import tpu as pltpu

B, C, H, W, E = 2, 512, 64, 64, 1152
EPS = 1e-5
NCH = C // 128
WT = W // 2
SLOT = 40
T = 4
RU = 4 * T
NS = RU + 2
NR = NS * SLOT + 8
NU = H // RU
M = T * WT
NIJ = 24
IORD = (1, 2, 3, 4, 0, 5)

F32 = jnp.float32
BF16 = jnp.bfloat16
U32 = jnp.uint32
PACEU = 1
ACTG = 3

COL = {0: (1, 7), 1: (0, 8), 2: (1, 8), 3: (0, 9)}
WJ = {0: (0, 2, -1), 1: (1, 2, 1), 2: (2, 1, -1), 3: (1, 3, -1)}


def _unpack(w):
    e = pltpu.unpack_elementwise(w, index=0, packed_dtype=BF16, unpacked_dtype=F32)
    o = pltpu.unpack_elementwise(w, index=1, packed_dtype=BF16, unpacked_dtype=F32)
    return e, o


def _pm(a, b, s):
    return a + b if s > 0 else a - b


def _bt43(r):
    d0, d1, d2, d3, d4, d5 = r
    t1 = d4 - 4.0 * d2
    t2 = d3 - 4.0 * d1
    a = d4 - d2
    b = d3 - d1
    b2 = b + b
    return [4.0 * (d0 - d2) + a, t1 + t2, t1 - t2, a + b2, a - b2, (d5 - d3) - (b2 + b2)]


def _or_f32(v, z):
    zz = jnp.concatenate([z] * (v.shape[0] // 8), axis=0)
    return pltpu.bitcast(pltpu.bitcast(v, U32) | zz, F32)


def _kernel(x_hbm, temb_ref, g1_ref, be1_ref, w1_hbm, wemb_hbm, g2_ref, be2_ref, w2_hbm,
            out_hbm,
            S, wraw, wt, wembs, PA, PB, U0, st, scs, zs, sems):
    def x_copy(b, c):
        return pltpu.make_async_copy(
            x_hbm.at[b, :, pl.ds(c * 128, 128)], S.bitcast(BF16).at[b, c], sems.at[b * NCH + c])

    def w_copy(k, c):
        src = w1_hbm if k == 0 else w2_hbm
        return pltpu.make_async_copy(src.at[:, :, pl.ds(c * 128, 128)], wraw.bitcast(BF16).at[k, c],
                                     sems.at[8 + k * NCH + c])

    def wemb_copy():
        return pltpu.make_async_copy(wemb_hbm, wembs, sems.at[16])

    def out_copy(b, u, c):
        rows = RU * W
        r0 = pl.multiple_of(u * rows, rows)
        return pltpu.make_async_copy(
            S.bitcast(BF16).at[b, c, pl.ds(r0, rows)],
            out_hbm.at[b, pl.ds(r0, rows), pl.ds(c * 128, 128)],
            sems.at[17 + (b * NU + u) * NCH + c])

    for c in range(NCH):
        x_copy(0, c).start()
    for c in range(NCH):
        w_copy(0, c).start()
    for c in range(NCH):
        x_copy(1, c).start()
    wemb_copy().start()
    for c in range(NCH):
        w_copy(1, c).start()

    zero8 = jnp.zeros((8, 128), F32)
    for P in (PA, PB):
        for p in range(2):
            for c in range(NCH):
                for s in range(NS + 1):
                    P[p, c, pl.ds(s * SLOT, 8), :] = zero8
    zs[...] = jnp.zeros((8, 128), U32)

    def x_stats(b, c):
        for u in range(NU):
            r0 = u * RU * WT
            w0 = S[b, c, pl.ds(r0, 8), :]
            piv = _unpack(w0)[0][0:1, :]

            def body(r, carry):
                s1, s2 = carry
                w = S[b, c, pl.ds(pl.multiple_of(r0 + r * (2 * WT), 8), 2 * WT), :]
                e, o = _unpack(w)
                for v in (e, o):
                    d = v - piv
                    dd = d * d
                    for q in range(2 * WT // 8):
                        s1 = s1 + d[q * 8:(q + 1) * 8]
                        s2 = s2 + dd[q * 8:(q + 1) * 8]
                return s1, s2
            s1, s2 = lax.fori_loop(0, RU // 2, body, (zero8, zero8))
            st[b, u, 0:1, pl.ds(c * 128, 128)] = piv
            st[b, u, 1:2, pl.ds(c * 128, 128)] = jnp.sum(s1, axis=0, keepdims=True)
            st[b, u, 2:3, pl.ds(c * 128, 128)] = jnp.sum(s2, axis=0, keepdims=True)

    def finalize(b, kdst, c, gam_ref, bet_ref, off):
        n = float(RU * W)
        sl = pl.ds(c * 128, 128)
        gam = gam_ref[sl].astype(F32).reshape(1, 128)
        bet = bet_ref[sl].astype(F32).reshape(1, 128)
        means = []
        m2s = []
        for u in range(NU):
            piv = st[b, u, 0:1, sl]
            s1 = st[b, u, 1:2, sl]
            s2 = st[b, u, 2:3, sl]
            mu = piv + s1 * (1.0 / n)
            if off is not None:
                mu = mu + off
            means.append(mu)
            m2s.append(s2 - s1 * s1 * (1.0 / n))
        tot = means[0]
        for u in range(1, NU):
            tot = tot + means[u]
        gmean = jnp.sum(tot, axis=1, keepdims=True) * (1.0 / (NU * 128))
        acc = jnp.zeros((1, 128), F32)
        for u in range(NU):
            dm = means[u] - gmean
            acc = acc + m2s[u] + n * dm * dm
        var = jnp.sum(acc, axis=1, keepdims=True) * (1.0 / (NU * 128 * n))
        rstd = lax.rsqrt(var + EPS)
        sc = 0.5 * gam * rstd
        sh = 0.5 * bet - gmean * sc
        if off is not None:
            sh = sh + off * sc
        scs[kdst, 0:1, sl] = sc
        scs[kdst, 1:2, sl] = sh

    def act_row(k, u, P, s, c, z=None):
        h = u * RU - 1 + s
        edge = s == 0 or s == NS - 1
        if edge:
            valid = jnp.logical_and(h >= 0, h < H)
            h = jnp.clip(h, 0, H - 1)
        sc = scs[k, 0:1, pl.ds(c * 128, 128)]
        sh = scs[k, 1:2, pl.ds(c * 128, 128)]
        w = S[k, c, pl.ds(pl.multiple_of(h * WT, 8), WT), :]
        if z is not None:
            w = w | jnp.concatenate([z] * (WT // 8), axis=0)
        e, o = _unpack(w)
        for p, v in ((0, e), (1, o)):
            uu = v * sc + sh
            a = uu + uu * jnp.tanh(uu)
            if edge:
                a = jnp.where(valid, a, 0.0)
            P[p, c, pl.ds(s * SLOT + 8, WT), :] = a

    def u_block(P, j, t, c, z=None):
        ca, cb, sg = WJ[j]
        rows = []
        for r in range(6):
            s = 4 * t + r
            pa, oa = COL[ca]
            pb, ob = COL[cb]
            va = P[pa, c, pl.ds(s * SLOT + oa, WT), :]
            vb = P[pb, c, pl.ds(s * SLOT + ob, WT), :]
            if z is not None and r in (2, 3):
                va = _or_f32(va, z)
            rows.append(_pm(va, vb, sg))
        return _bt43(rows)

    def w_block(k, c, r0):
        ge = [[None] * 3 for _ in range(3)]
        go = [[None] * 3 for _ in range(3)]
        for kh in range(3):
            for kw in range(3):
                ge[kh][kw], go[kh][kw] = _unpack(wraw[k, c, kh * 3 + kw, pl.ds(r0, 8), :])
        res = []
        for g in (ge, go):
            t = []
            for kh in range(3):
                s = g[kh][0] + g[kh][2]
                t.append([g[kh][0], 0.5 * (s + g[kh][1]), 0.5 * (s - g[kh][1]), g[kh][2]])
            cols = []
            for j in range(4):
                g0, g1, g2 = t[0][j], t[1][j], t[2][j]
                s = g0 + g2
                u0 = 0.25 * g0
                e = (u0 + g2) * (1.0 / 6.0)
                f = g1 * (1.0 / 12.0)
                cols.append([u0, (s + g1) * (-1.0 / 6.0), (s - g1) * (-1.0 / 6.0), e + f, e - f, g2])
            res.append(cols)
        for j in range(4):
            for i in range(6):
                wt[k, i * 4 + j, c, pl.ds(r0, 8), :] = pltpu.pack_elementwise(
                    [res[0][j][i], res[1][j][i]], packed_dtype=BF16)

    def w_transform(k, c):
        def body(rb, _):
            w_block(k, c, pl.multiple_of(rb * 8, 8))
            return 0
        lax.fori_loop(0, C // 16, body, 0, unroll=2)

    def store_u0(P, zf=None):
        for t in range(T):
            for c in range(NCH):
                z = None if zf is None else zf(t * NCH + c)
                u6 = u_block(P, 0, t, c, z)
                for i in range(6):
                    U0[i, c, pl.ds(t * (WT // 2), WT // 2), :] = pltpu.bitcast(u6[i].astype(BF16), U32)

    def conv_unit(k, n, P, Pn):
        b = (n // NU) % B
        u = n % NU
        nn = jnp.minimum(n + 1, 4 * NU - 1)
        kn = nn // NU
        un = nn % NU
        zmask = zs[...]

        Y = [[[None] * NCH, [None] * NCH] for _ in range(4)]
        ms = []
        U = [jnp.concatenate([pltpu.bitcast(U0[i, c], BF16) for c in range(NCH)], axis=1) for i in range(6)]

        def pz(j, ph, q):
            nt, i = ph // 6, IORD[ph % 6]
            r = (q % 4) * (M // 4)
            v = ms[j][nt][i][r:r + 8, :]
            return pltpu.bitcast(v, U32) & zmask

        for j in range(4):
            msj = []
            for n_ in range(NCH):
                m = [None] * 6
                for i in IORD:
                    Wm = jnp.concatenate(
                        [pltpu.bitcast(wt[k, i * 4 + j, c, pl.ds(n_ * 64, 64), :], BF16) for c in range(NCH)], axis=1)
                    m[i] = lax.dot_general(U[i], Wm, (((1,), (1,)), ((), ())), preferred_element_type=F32)
                msj.append(m)
                sa = m[1] + m[2]
                da = m[1] - m[2]
                sb = m[3] + m[4]
                db = m[3] - m[4]
                z = [m[0] + (sa + sb), da + 2.0 * db, sa + 4.0 * sb, (da + 8.0 * db) + m[5]]
                for a in range(4):
                    if j == 0:
                        Y[a][0][n_] = z[a]
                    elif j == 1:
                        Y[a][0][n_] = Y[a][0][n_] + z[a]
                        Y[a][1][n_] = z[a]
                    elif j == 2:
                        Y[a][0][n_] = Y[a][0][n_] + z[a]
                        Y[a][1][n_] = Y[a][1][n_] - z[a]
                    else:
                        Y[a][1][n_] = Y[a][1][n_] - z[a]
            ms.append(msj)
            if j < ACTG:
                tot = NS * NCH
                lo, hi = (j * tot) // ACTG, ((j + 1) * tot) // ACTG
                for q in range(lo, hi):
                    s, c = q // NCH, q % NCH
                    ph = ((q - lo) * 22) // (hi - lo)
                    act_row(kn, un, Pn, s, c, pz(j, ph, q))
            if j < 3:
                U6 = [[None] * NCH for _ in range(T)]
                for t in range(T):
                    for c in range(NCH):
                        q = t * NCH + c
                        z_ = pz(j, (q * 20) // (T * NCH), q) if PACEU else None
                        U6[t][c] = u_block(P, j + 1, t, c, z_)
                U = []
                for i in range(6):
                    rows = [jnp.concatenate([U6[t][c][i] for c in range(NCH)], axis=1) for t in range(T)]
                    U.append(jnp.concatenate(rows, axis=0).astype(BF16))
            else:
                store_u0(Pn, lambda q: pz(3, (q * 18) // (T * NCH), q))
        for c in range(NCH):
            if k == 0:
                piv = Y[0][0][c][0:1, :]
                s1 = zero8
                s2 = zero8
            for t in range(T):
                for a in range(4):
                    ye = Y[a][0][c][t * WT:(t + 1) * WT, :]
                    yo = Y[a][1][c][t * WT:(t + 1) * WT, :]
                    row = pl.multiple_of((u * RU + 4 * t + a) * WT, 8)
                    if k == 0:
                        for v in (ye, yo):
                            dd = v - piv
                            d2 = dd * dd
                            for q in range(WT // 8):
                                s1 = s1 + dd[q * 8:(q + 1) * 8]
                                s2 = s2 + d2[q * 8:(q + 1) * 8]
                        S[2 + b, c, pl.ds(row, WT), :] = pltpu.pack_elementwise([ye, yo], packed_dtype=BF16)
                    else:
                        xe, xo = _unpack(S[b, c, pl.ds(row, WT), :])
                        S[b, c, pl.ds(row, WT), :] = pltpu.pack_elementwise(
                            [ye + xe, yo + xo], packed_dtype=BF16)
            if k == 0:
                st[b, u, 0:1, pl.ds(c * 128, 128)] = piv
                st[b, u, 1:2, pl.ds(c * 128, 128)] = jnp.sum(s1, axis=0, keepdims=True)
                st[b, u, 2:3, pl.ds(c * 128, 128)] = jnp.sum(s2, axis=0, keepdims=True)
        if k == 1:
            for c in range(NCH):
                out_copy(b, u, c).start()

    def emb_rows():
        te = temb_ref[...].astype(F32)
        th = 0.5 * te
        sil = th + th * jnp.tanh(th)
        return jnp.dot(sil.astype(BF16), wembs[...], preferred_element_type=F32)

    for c in range(NCH):
        x_copy(0, c).wait()
        x_stats(0, c)
        finalize(0, 0, c, g1_ref, be1_ref, None)
        for s in range(NS):
            act_row(0, 0, PA, s, c)
    store_u0(PA)
    for c in range(NCH):
        w_copy(0, c).wait()
        w_transform(0, c)

    def pair1(p, _):
        @pl.when(p >= 0)
        def _():
            conv_unit(0, 2 * p, PA, PB)

        @pl.when(p >= -1)
        def _():
            conv_unit(0, 2 * p + 1, PB, PA)

        @pl.when(p == 0)
        def _():
            for c in range(NCH):
                x_copy(1, c).wait()
                x_stats(1, c)
                finalize(1, 1, c, g1_ref, be1_ref, None)
            wemb_copy().wait()
            for c in range(NCH):
                w_copy(1, c).wait()
                w_transform(1, c)

        @pl.when(p % (NU // 2) == NU // 2 - 1)
        def _():
            bb = p // (NU // 2)
            emb = emb_rows()
            er = jnp.where(bb == 0, emb[0:1, :], emb[1:2, :])
            for c in range(NCH):
                finalize(bb, 2 + bb, c, g2_ref, be2_ref, er[:, c * 128:(c + 1) * 128])
        return 0
    lax.fori_loop(0, NU, pair1, 0)

    def pair2(p, _):
        @pl.when(p >= 0)
        def _():
            conv_unit(1, 2 * p, PA, PB)

        @pl.when(p >= -1)
        def _():
            conv_unit(1, 2 * p + 1, PB, PA)
        return 0
    lax.fori_loop(NU, 2 * NU, pair2, 0)
    for b in range(B):
        for u in range(NU):
            for c in range(NCH):
                out_copy(b, u, c).wait()


@jax.jit
def pallas_standalone__adm_resblock__diffusion_kernel(x, t_emb, g1, be1, w1, w_emb, g2, be2, w2):
    xn = jnp.transpose(x, (0, 2, 3, 1)).reshape(B, H * W, C)
    w1n = jnp.transpose(w1, (2, 3, 0, 1)).reshape(9, C, C)
    w2n = jnp.transpose(w2, (2, 3, 0, 1)).reshape(9, C, C)
    vm = pl.BlockSpec(memory_space=pltpu.VMEM)
    hbm = pl.BlockSpec(memory_space=pl.ANY)
    out = pl.pallas_call(
        _kernel,
        out_shape=jax.ShapeDtypeStruct((B, H * W, C), BF16),
        in_specs=[hbm, vm, vm, vm, hbm, hbm, vm, vm, hbm],
        out_specs=hbm,
        scratch_shapes=[
            pltpu.VMEM((4, NCH, H * WT, 128), U32),
            pltpu.VMEM((2, NCH, 9, C // 2, 128), U32),
            pltpu.VMEM((2, NIJ, NCH, C // 2, 128), U32),
            pltpu.VMEM((E, C), BF16),
            pltpu.VMEM((2, NCH, NR, 128), F32),
            pltpu.VMEM((2, NCH, NR, 128), F32),
            pltpu.VMEM((6, NCH, M // 2, 128), U32),
            pltpu.VMEM((B, NU, 8, C), F32),
            pltpu.VMEM((4, 8, C), F32),
            pltpu.VMEM((8, 128), U32),
            pltpu.SemaphoreType.DMA((17 + B * NU * NCH,)),
        ],
        compiler_params=pltpu.CompilerParams(vmem_limit_bytes=110 * 1024 * 1024),
    )(xn, t_emb, g1, be1, w1n, w_emb, g2, be2, w2n)
    return jnp.transpose(out.reshape(B, H, W, C), (0, 3, 1, 2))
```

```python
import jax
import jax.numpy as jnp
from jax import lax
from jax.experimental import pallas as pl
from jax.experimental.pallas import tpu as pltpu

B, C, H, W, E = 2, 512, 64, 64, 1152
EPS = 1e-5
NCH = C // 128
WT = W // 2
T = 8
RU = 4 * T
NS = RU + 2
NU = H // RU
M = T * 16
ORD = (1, 2, 3, 4, 0, 5)

F32 = jnp.float32
BF16 = jnp.bfloat16
U32 = jnp.uint32

PA_ = 0.65
PB_ = 1.0 / PA_
A2, B2 = PA_ * PA_, PB_ * PB_
A3, B3 = A2 * PA_, B2 * PB_
C1 = 1.0 / (2.0 * A2 * (A2 - B2))
C2 = 1.0 / (2.0 * B2 * (B2 - A2))

ENDA = 29.0
ENDB = 35.0
HLAG = 2
HPRI = 3.0
WAHEAD = 4.0
FILL = 400.0
NACC = 2
STOP = ''
DM = [0, 0]
REP = 1
HPQ = [2, 3]
FREE = 0
FTAU = 200
PACEH = 1


COST = {'r': 110.0, 'h': 44.0, 'w0': 36.0, 'w5': 36.0, 'w1': 116.0, 'w3': 116.0, 'x': 81.0}


def _schedule(extra=(), k=0):
    base = [48.0] * 36
    for g, j in enumerate(ORD):
        p = 6 * g
        base[p + 1] += 32
        base[p + 3] += 160
        base[p + 4] += 16
        base[p + 5] += 16
        fin = 16 * (0 if k == 0 else 2) * 4
        w = {1: 0, 2: 128, 3: 0, 4: 640 + 2 * fin, 0: 64 + fin + 64, 5: 64 + fin + 64}[j]
        if p + 6 < 36:
            base[p + 4] += w * 0.25
            base[p + 5] += w * 0.5
            base[p + 6] += w * 0.25
        else:
            base[p + 4] += w * 0.5
            base[p + 5] += w * 0.5
    nA = int(ENDA * 16)
    nB = int(ENDB * 16)
    cap = [max(FILL - base[t // 16], 24.0) / 16.0 for t in range(36 * 16)]
    A = [('r', s) for s in range(NS)]
    xs = [it for it in extra if it[0] == 'x']
    ws = [it for it in extra if it[0] != 'x']
    if xs:
        mer = []
        ne = 0
        for q, it in enumerate(A):
            mer.append(it)
            while ne < len(xs) and (ne + 0.5) / len(xs) <= (q + 1.0) / len(A):
                mer.append(xs[ne])
                ne += 1
        A = mer + xs[ne:]
    hs = [('h', t, j) for t in range(T) for j in range(6)]

    def sim(lam):
        out = []
        credit = 0.0
        totA = sum(COST[i[0]] for i in A)
        capA = sum(cap[:nA])
        ia = ih = iw = 0
        accA = 0.0
        cumcap = 0.0
        rowrel = {}
        for t in range(nB):
            cumcap += cap[t]
            credit += lam * cap[t]
            while ia < len(A) and (t >= nA - 1 or accA <= totA * cumcap / capA * (nA - 1.0) / nA):
                it = A[ia]
                out.append((it, t))
                accA += COST[it[0]]
                credit -= COST[it[0]]
                if it[0] == 'r':
                    rowrel[it[1]] = t
                ia += 1
            while credit > 0:
                it = None
                hok = ih < len(hs) and (4 * hs[ih][1] + 5) in rowrel and rowrel[4 * hs[ih][1] + 5] + HLAG <= t
                wok = iw < len(ws)
                if hok and wok:
                    it = hs[ih] if ih * len(ws) <= iw * len(hs) + HPRI * len(ws) else ws[iw]
                elif hok:
                    it = hs[ih]
                elif wok and iw * len(hs) <= (ih + WAHEAD) * len(ws):
                    it = ws[iw]
                if it is None:
                    break
                if it[0] == 'h':
                    ih += 1
                else:
                    iw += 1
                out.append((it, t))
                credit -= COST[it[0]]
            credit = min(credit, 60.0)
        return out, (ih == len(hs) and iw == len(ws) and ia == len(A))
    lo, hi = 0.05, 4.0
    for _ in range(30):
        mid = 0.5 * (lo + hi)
        if sim(mid)[1]:
            hi = mid
        else:
            lo = mid
    out, ok = sim(hi)
    assert ok
    q = 0
    while out[q][1] < FTAU:
        q += 1
    out.insert(q, (('f',), FTAU))
    return out


def _sl(hh, p):
    return pl.ds(16 * hh + p, 8, stride=2)


def _unpack(w):
    e = pltpu.unpack_elementwise(w, index=0, packed_dtype=BF16, unpacked_dtype=F32)
    o = pltpu.unpack_elementwise(w, index=1, packed_dtype=BF16, unpacked_dtype=F32)
    return e, o


def _bt6(d):
    d0, d1, d2, d3, d4, d5 = d
    p = A2 * d2
    q = B2 * d2
    ea = d4 - q
    eb = d4 - p
    e0 = (ea - p) + d0
    p3 = A2 * d3
    q3 = B2 * d3
    wa = p3 - d1
    wb = q3 - d1
    oi = (d5 - wa) - q3
    ta = PB_ * wa
    tb = PA_ * wb
    return [e0, ea + ta, ea - ta, eb + tb, eb - tb, oi]


def _g6(g0, g1, g2, c1=C1, c2=C2):
    ea = c1 * g0 + (C1 * A2) * g2
    oa = (C1 * PA_) * g1
    eb = c2 * g0 + (C2 * B2) * g2
    ob = (C2 * PB_) * g1
    return [g0, ea + oa, ea - oa, eb + ob, eb - ob, g2]


class _AT:
    def __init__(self):
        self.v = {}
        self.z = [None] * 4

    def feed(self, i, m):
        v = self.v
        if i in (1, 3):
            v[i] = m
        elif i == 2:
            v['sa'] = v[1] + m
            v['da'] = v[1] - m
        elif i == 4:
            sb = v[3] + m
            db = v[3] - m
            v['p0'] = v['sa'] + sb
            self.z[1] = PA_ * v['da'] + PB_ * db
            self.z[2] = A2 * v['sa'] + B2 * sb
            v['p3'] = A3 * v['da'] + B3 * db
        elif i == 0:
            self.z[0] = v['p0'] + m
        else:
            self.z[3] = v['p3'] + m


def _kernel(x_hbm, temb_ref, g1_ref, be1_ref, w1_hbm, wemb_hbm, g2_ref, be2_ref, w2_hbm,
            out_hbm,
            S, wraw, wt1, wt2, wembs, Wp, UA, UB, st, gb, off, scs, zs, sems):
    wt = (wt1, wt2)

    def x_copy(b, c):
        return pltpu.make_async_copy(
            x_hbm.at[b, :, :, pl.ds(pl.multiple_of(c * 128, 128), 128)], S.bitcast(BF16).at[b, c],
            sems.at[b * NCH + c])

    def w_copy(k, c):
        src = w1_hbm if k == 0 else w2_hbm
        return pltpu.make_async_copy(src.at[:, :, pl.ds(c * 128, 128)], wraw.bitcast(BF16).at[k, c],
                                     sems.at[8 + k * NCH + c])

    def wemb_copy():
        return pltpu.make_async_copy(wemb_hbm, wembs, sems.at[16])

    def out_copy(b, u, c):
        r0 = pl.multiple_of(u * RU, RU)
        return pltpu.make_async_copy(
            S.bitcast(BF16).at[b, c, pl.ds(r0, RU)],
            out_hbm.at[b, pl.ds(r0, RU), :, pl.ds(pl.multiple_of(c * 128, 128), 128)],
            sems.at[17 + (b * NU + u) * NCH + c])

    for c in range(NCH):
        x_copy(0, c).start()
    for c in range(NCH):
        w_copy(0, c).start()
    def start_rest(stage):
        if STOP == 'pro0':
            return
        if stage == DM[0]:
            for c in range(NCH):
                x_copy(1, c).start()
        if stage == DM[1]:
            for c in range(NCH):
                w_copy(1, c).start()
            wemb_copy().start()
    start_rest(0)

    zero8 = jnp.zeros((8, 128), F32)
    zs[...] = jnp.zeros((8, 128), U32)
    for c in range(NCH):
        sl = pl.ds(c * 128, 128)
        for q, r in enumerate((g1_ref, be1_ref, g2_ref, be2_ref)):
            gb[q, c] = jnp.broadcast_to(r[sl].astype(F32).reshape(1, 128), (8, 128))
        off[0, c] = zero8
        off[1, c] = zero8
    sub = lax.broadcasted_iota(jnp.int32, (8, 128), 0)

    def acc_stats(vals, piv, s1, s2):
        for q, v in enumerate(vals):
            d = v - piv
            k_ = q % len(s1)
            s1[k_] = s1[k_] + d
            s2[k_] = s2[k_] + d * d

    def put_stats(slot, c, u, piv, s1, s2):
        t1 = s1[0]
        t2 = s2[0]
        for q in range(1, len(s1)):
            t1 = t1 + s1[q]
            t2 = t2 + s2[q]
        st[slot, c, u, 0] = piv
        st[slot, c, u, 1] = t1
        st[slot, c, u, 2] = t2

    def x_stats_rolled(b, c):
        for u in range(NU):
            w0 = S[b, c, u * RU, pl.ds(0, 8), :]
            piv = jnp.broadcast_to(_unpack(w0)[0][0:1, :], (8, 128))

            def body(r, carry):
                s1 = list(carry[0])
                s2 = list(carry[1])
                vals = []
                for q in range(4):
                    vals += list(_unpack(S[b, c, u * RU + r, pl.ds(q * 8, 8), :]))
                acc_stats(vals, piv, s1, s2)
                return tuple(s1), tuple(s2)
            s1, s2 = lax.fori_loop(0, RU, body, ((zero8,) * 2, (zero8,) * 2), unroll=2)
            put_stats(b, c, u, piv, list(s1), list(s2))

    def finalize(kn, c, z=None):
        n = float(RU * W)
        kg = (kn // 2) * 2
        gam = gb[kg, c]
        bet = gb[kg + 1, c]
        of = off[kn, c]
        means = []
        m2s = []
        for u in range(NU):
            piv = st[kn, c, u, 0]
            t1 = st[kn, c, u, 1]
            t2 = st[kn, c, u, 2]
            if z is not None:
                t1 = z(t1)
                t2 = z(t2)
            s1 = jnp.sum(t1, axis=0, keepdims=True)
            s2 = jnp.sum(t2, axis=0, keepdims=True)
            means.append(piv[0:1] + s1 * (1.0 / n) + of[0:1])
            m2s.append(s2 - s1 * s1 * (1.0 / n))
        tot = means[0]
        for u in range(1, NU):
            tot = tot + means[u]
        gmean = jnp.sum(tot, axis=1, keepdims=True) * (1.0 / (NU * 128))
        acc = jnp.zeros((1, 128), F32)
        for u in range(NU):
            dm = means[u] - gmean
            acc = acc + m2s[u] + n * dm * dm
        var = jnp.sum(acc, axis=1, keepdims=True) * (1.0 / (NU * 128 * n))
        rstd = lax.rsqrt(var + EPS)
        sc = 0.5 * gam * rstd
        sh = 0.5 * bet + (of - gmean) * sc
        return sc, sh

    def w_row(kn, un, c, s, sc, sh, edge):
        h = un * RU - 1 + s
        if edge:
            valid = jnp.logical_and(h >= 0, h < H)
            h = jnp.clip(h, 0, H - 1)
        col = [[None] * 4 for _ in range(2)]
        for hh in range(2):
            for p in range(2):
                w = S[kn, c, h, _sl(hh, p), :]
                for e, v in enumerate(_unpack(w)):
                    uu = v * sc + sh
                    a = uu + uu * jnp.tanh(uu)
                    if edge:
                        a = jnp.where(valid, a, 0.0)
                    col[hh][2 * p + e] = a
        r0 = pltpu.roll(col[0][3], 1, 0)
        r1 = pltpu.roll(col[1][3], 1, 0)
        d0 = [jnp.where(sub == 0, 0.0, r0), jnp.where(sub == 0, r0, r1)]
        l0 = pltpu.roll(col[0][0], 7, 0)
        l1 = pltpu.roll(col[1][0], 7, 0)
        d5 = [jnp.where(sub == 7, l1, l0), jnp.where(sub == 7, 0.0, l1)]
        for hh in range(2):
            r = _bt6([d0[hh]] + col[hh] + [d5[hh]])
            for j in range(6):
                Wp[s, 2 * j + hh] = r[j]

    def h_tile(Ud, c, t, j, z=None):
        r = []
        for hh in range(2):
            d = [Wp[4 * t + q, 2 * j + hh] for q in range(6)]
            if z is not None:
                for q in HPQ:
                    d[q] = z(d[q])
            r.append(_bt6(d))
        r0 = t * 16 if isinstance(t, int) else pl.multiple_of(t * 16, 16)
        for i in range(6):
            Ud[i * 6 + j, c, pl.ds(r0, 16), :] = jnp.concatenate([r[0][i], r[1][i]], axis=0).astype(BF16)

    def produce_rolled(Ud, kn, un, c):
        sc, sh = finalize(kn, c)

        def rbody(s, _):
            w_row(kn, un, c, s, sc, sh, True)
            return 0
        lax.fori_loop(0, NS, rbody, 0, unroll=2)

        def tbody(t, _):
            for j in range(6):
                h_tile(Ud, c, t, j)
            return 0
        lax.fori_loop(0, T, tbody, 0)

    def w_part(ksrc, kdst, c, r0, part, z=None):
        def tap(kh, kw):
            return wraw[ksrc, c, kh * 3 + kw, pl.ds(r0, 8), :]

        def cst(v):
            return v if z is None else z(jnp.full((8, 128), v, F32))
        if part in (0, 5):
            j = part
            w = [tap(kh, 0 if part == 0 else 2) for kh in range(3)]
            g = [_unpack(w[kh]) for kh in range(3)]
            c1, c2 = cst(C1), cst(C2)
            r = [_g6(g[0][h], g[1][h], g[2][h], c1, c2) for h in range(2)]
            wt[kdst][j, c, pl.ds(r0, 8), :] = w[0]
            wt[kdst][30 + j, c, pl.ds(r0, 8), :] = w[2]
            for i in range(1, 5):
                wt[kdst][i * 6 + j, c, pl.ds(r0, 8), :] = pltpu.pack_elementwise(
                    [r[0][i], r[1][i]], packed_dtype=BF16)
            return
        cc, pp = (C1, PA_) if part == 1 else (C2, PB_)
        ccv = cst(cc)
        tp = [[None] * 3 for _ in range(2)]
        tm = [[None] * 3 for _ in range(2)]
        for kh in range(3):
            g = [_unpack(tap(kh, kw)) for kw in range(3)]
            for h in range(2):
                e = ccv * g[0][h] + (cc * pp * pp) * g[2][h]
                o = (cc * pp) * g[1][h]
                tp[h][kh] = e + o
                tm[h][kh] = e - o
        for j, t in ((part, tp), (part + 1, tm)):
            r = [_g6(*t[h]) for h in range(2)]
            for i in range(6):
                wt[kdst][i * 6 + j, c, pl.ds(r0, 8), :] = pltpu.pack_elementwise(
                    [r[0][i], r[1][i]], packed_dtype=BF16)

    def w_block(k, c, r0):
        for part in (0, 1, 3, 5):
            w_part(k, k, c, r0, part)

    def w_transform(k, c):
        def body(rb, _):
            w_block(k, c, pl.multiple_of(rb * 8, 8))
            return 0
        lax.fori_loop(0, C // 16, body, 0, unroll=2)

    def conv_body(k, nu, n, Uc, Un, extra):
        b = (nu // NU) % B
        u = nu % NU
        nn = jnp.minimum(nu + 1, 4 * NU - 1)
        kn = nn // NU
        un = nn % NU
        fmask = zs[...] != 0
        n64 = pl.multiple_of(n * 64, 64)

        ms = []
        col = [_AT() for _ in range(4)]
        fin = [[None] * 4 for _ in range(4)]

        def where(a, t, hh, p):
            return u * RU + 4 * t + a, _sl(hh, p)

        def finish(a, bc):
            y = col[a].z[bc]
            vs = []
            for t in range(T):
                for hh in range(2):
                    q = (2 * t + hh) * 8
                    v = y[q:q + 8]
                    if k == 1:
                        row, dst = where(a, t, hh, bc // 2)
                        v = v + pltpu.unpack_elementwise(S[b, n, row, dst, :], index=bc % 2,
                                                         packed_dtype=BF16, unpacked_dtype=F32)
                    vs.append(v)
            fin[a][bc] = vs

        anchor = pltpu.bitcast(wt[k][ORD[0] * 6 + ORD[0], 0, pl.ds(n64, 8), :], F32)
        for j in ORD:
            at = _AT()
            for i in ORD:
                L = jnp.concatenate(
                    [pltpu.bitcast(Uc.bitcast(U32)[i * 6 + j, c], BF16) for c in range(NCH)], axis=1)
                Wm = jnp.concatenate(
                    [pltpu.bitcast(wt[k][i * 6 + j, c, pl.ds(n64, 64), :], BF16) for c in range(NCH)], axis=1)
                m = lax.dot_general(L, Wm, (((1,), (1,)), ((), ())), preferred_element_type=F32)
                ms.append(m)
                at.feed(i, m)
            for a in (1, 2, 0, 3):
                col[a].feed(j, at.z[a])
                if j == 4:
                    finish(a, 1)
                    finish(a, 2)
                elif j == 0:
                    finish(a, 0)
                elif j == 5:
                    finish(a, 3)

        def pacer(tau):
            ph, q = tau // 16, tau % 16
            mv = ms[ph][q * 8:q * 8 + 8, :]
            return lambda v: jnp.where(fmask, mv, v)

        par = n % 2
        sc = scs[par, 0]
        sh = scs[par, 1]
        nu2 = jnp.where(n == NCH - 1, nu + 1, nu)
        kn2 = jnp.minimum(nu2 + 1, 4 * NU - 1) // NU
        n2 = (n + 1) % NCH
        if extra == 'w':
            items = [('w%d' % part, q) for q in range(16) for part in (1, 0, 3, 5)]
            wc = nu - 1 + n // 2
            wr = (n % 2) * 128
        elif extra == 'x':
            items = [('x', q) for q in range(RU)]
            xsrc = jnp.minimum(nu // 2 + 1, 3)
            xdst = jnp.where(nu == 6, 4, xsrc)
            xs1 = [zero8] * 2
            xs2 = [zero8] * 2
            xpiv = [None, None]
        else:
            items = []
        for it, tau in _schedule(items, k):
            z = pacer(tau)
            if tau < FREE:
                z = lambda v: jnp.where(fmask, anchor, v)
            if it[0] == 'f':
                fsc, fsh = finalize(kn2, n2, z)
                scs[1 - par, 0] = fsc
                scs[1 - par, 1] = fsh
            elif it[0] == 'r':
                s = it[1]
                w_row(kn, un, n, s, z(sc), sh, s == 0 or s == NS - 1)
            elif it[0] == 'h':
                h_tile(Un, n, it[1], it[2], z if PACEH else None)
            elif it[0][0] == 'w':
                w_part(1, 1, wc, pl.multiple_of(wr + it[1] * 8, 8), int(it[0][1]), z)
            else:
                uu, r0 = it[1] // (RU // 2), (it[1] % (RU // 2)) * 2
                if xpiv[uu] is None:
                    xpiv[uu] = jnp.broadcast_to(_unpack(S[xsrc, n, uu * RU, pl.ds(0, 8), :])[0][0:1, :], (8, 128))
                    xs1 = [zero8] * 2
                    xs2 = [zero8] * 2
                pv = z(xpiv[uu])
                vals = []
                for r in range(2):
                    for q in range(4):
                        vals += list(_unpack(S[xsrc, n, uu * RU + r0 + r, pl.ds(q * 8, 8), :]))
                acc_stats(vals, pv, xs1, xs2)
                if r0 == RU - 2:
                    put_stats(xdst, n, uu, xpiv[uu], xs1, xs2)

        for p in range(2):
            for a in (1, 2, 0, 3):
                for t in range(T):
                    for hh in range(2):
                        row, dst = where(a, t, hh, p)
                        S[(2 + b) if k == 0 else b, n, row, dst, :] = pltpu.pack_elementwise(
                            [fin[a][2 * p][2 * t + hh], fin[a][2 * p + 1][2 * t + hh]], packed_dtype=BF16)
        if k == 1:
            out_copy(b, u, n).start()

    def emb_rows():
        te = temb_ref[...].astype(F32)
        th = 0.5 * te
        sil = th + th * jnp.tanh(th)
        return jnp.dot(sil.astype(BF16), wembs[...], preferred_element_type=F32)

    def pro(c, _):
        x_copy(0, c).wait()
        x_stats_rolled(0, c)
        produce_rolled(UA, 0, 0, c)
        return 0
    lax.fori_loop(0, NCH, pro, 0)
    sc0, sh0 = finalize(0, 0)
    scs[0, 0] = sc0
    scs[0, 1] = sh0
    start_rest(1)
    for c in range(NCH):
        w_copy(0, c).wait()
        if c == NCH - 1:
            start_rest(2)
        w_transform(0, c)

    def pair(k):
        def f(p, _):
            nu = 2 * p

            def fa(n, _):
                if k == 0:
                    @pl.when(p == 0)
                    def _():
                        x_copy(1, n).wait()
                conv_body(k, nu, n, UA, UB, 'x')
                return 0

            def fb(n, _):
                conv_body(k, nu + 1, n, UB, UA, 'w' if k == 0 else None)
                return 0
            if k == 0:
                @pl.when(p == 1)
                def _():
                    wemb_copy().wait()
                    emb = emb_rows()
                    for bb in range(B):
                        for c in range(NCH):
                            off[2 + bb, c] = jnp.broadcast_to(emb[bb:bb + 1, c * 128:(c + 1) * 128], (8, 128))
            lax.fori_loop(0, NCH, fa, 0)
            if k == 0:
                @pl.when(p == 0)
                def _():
                    w_copy(1, 0).wait()
                    w_copy(1, 1).wait()

                @pl.when(p == 1)
                def _():
                    w_copy(1, 2).wait()
                    w_copy(1, 3).wait()
            lax.fori_loop(0, NCH, fb, 0)
            return 0
        return f
    if STOP == 'pro0':
        return
    if STOP == 'pro':
        for c in range(NCH):
            x_copy(1, c).wait()
            w_copy(1, c).wait()
        wemb_copy().wait()
        return
    lax.fori_loop(0, NU, pair(0), 0)
    if STOP == 'c1':
        return
    def rep(_, __):
        lax.fori_loop(NU, 2 * NU, pair(1), 0)
        for b in range(B):
            for u in range(NU):
                for c in range(NCH):
                    out_copy(b, u, c).wait()
        return 0
    if REP > 1:
        lax.fori_loop(0, REP, rep, 0)
    else:
        rep(0, 0)


@jax.jit
def pallas_standalone__adm_resblock__diffusion_kernel(x, t_emb, g1, be1, w1, w_emb, g2, be2, w2):
    xn = jnp.transpose(x, (0, 2, 3, 1))
    w1n = jnp.transpose(w1, (2, 3, 0, 1)).reshape(9, C, C)
    w2n = jnp.transpose(w2, (2, 3, 0, 1)).reshape(9, C, C)
    vm = pl.BlockSpec(memory_space=pltpu.VMEM)
    hbm = pl.BlockSpec(memory_space=pl.ANY)
    out = pl.pallas_call(
        _kernel,
        out_shape=jax.ShapeDtypeStruct((B, H, W, C), BF16),
        in_specs=[hbm, vm, vm, vm, hbm, hbm, vm, vm, hbm],
        out_specs=hbm,
        scratch_shapes=[
            pltpu.VMEM((4, NCH, H, WT, 128), U32),
            pltpu.VMEM((2, NCH, 9, C // 2, 128), U32),
            pltpu.VMEM((36, NCH, C // 2, 128), U32),
            pltpu.VMEM((36, NCH, C // 2, 128), U32),
            pltpu.VMEM((E, C), BF16),
            pltpu.VMEM((NS, 12, 8, 128), F32),
            pltpu.VMEM((36, NCH, M, 128), BF16),
            pltpu.VMEM((36, NCH, M, 128), BF16),
            pltpu.VMEM((5, NCH, NU, 3, 8, 128), F32),
            pltpu.VMEM((4, NCH, 8, 128), F32),
            pltpu.VMEM((4, NCH, 8, 128), F32),
            pltpu.VMEM((2, 2, 8, 128), F32),
            pltpu.VMEM((8, 128), U32),
            pltpu.SemaphoreType.DMA((17 + B * NU * NCH,)),
        ],
        compiler_params=pltpu.CompilerParams(vmem_limit_bytes=110 * 1024 * 1024),
    )(xn, t_emb, g1, be1, w1n, w_emb, g2, be2, w2n)
    return jnp.transpose(out, (0, 3, 1, 2))
```

```python
import jax
import jax.numpy as jnp
from jax import lax
from jax.experimental import pallas as pl
from jax.experimental.pallas import tpu as pltpu

B, C, H, W, E = 2, 512, 64, 64, 1152
EPS = 1e-5
NCH = C // 128
WT = W // 2
T = 8
RU = 4 * T
NS = RU + 2
NU = H // RU
M = T * 16
ORD = (1, 2, 3, 4, 0, 5)

F32 = jnp.float32
BF16 = jnp.bfloat16
U32 = jnp.uint32

PA_ = 0.65
PB_ = 1.0 / PA_
A2, B2 = PA_ * PA_, PB_ * PB_
A3, B3 = A2 * PA_, B2 * PB_
C1 = 1.0 / (2.0 * A2 * (A2 - B2))
C2 = 1.0 / (2.0 * B2 * (B2 - A2))

ENDA = 29.0
ENDB = 35.9
HLAG = 2
HPRI = 3.0
WAHEAD = 4.0
FILL = 360.0
NACC = 2
STOP = ''
DM = [0, 0]
REP = 1
HPQ = [2, 3]
FREE = 0
FTAU = 200
SKIP = ''
WPAD = 8
UPAD = 16
PPAD = 1
XR = 8
RR = 33
TR = 8
WR = 8
NP = 4
NSEM = 17 + B * NU * NCH
PACEH = 1


COST = {'r': 110.0, 'h': 44.0, 'w0': 36.0, 'w5': 36.0, 'w1': 116.0, 'w3': 116.0, 'x': 81.0}


def _schedule(extra=(), k=0):
    base = [48.0] * 36
    for g, j in enumerate(ORD):
        p = 6 * g
        base[p + 1] += 32
        base[p + 3] += 160
        base[p + 4] += 16
        base[p + 5] += 16
        fin = 16 * (0 if k == 0 else 2) * 4
        w = {1: 0, 2: 128, 3: 0, 4: 640 + 2 * fin, 0: 64 + fin + 64, 5: 64 + fin + 64}[j]
        if p + 6 < 36:
            base[p + 4] += w * 0.25
            base[p + 5] += w * 0.5
            base[p + 6] += w * 0.25
        else:
            base[p + 4] += w * 0.5
            base[p + 5] += w * 0.5
    nA = int(ENDA * 16)
    nB = int(ENDB * 16)
    cap = [max(FILL - base[t // 16], 24.0) / 16.0 for t in range(36 * 16)]
    A = [('r', s) for s in range(NS)]
    xs = [it for it in extra if it[0] == 'x']
    ws = [it for it in extra if it[0] != 'x']
    if xs:
        mer = []
        ne = 0
        for q, it in enumerate(A):
            mer.append(it)
            while ne < len(xs) and (ne + 0.5) / len(xs) <= (q + 1.0) / len(A):
                mer.append(xs[ne])
                ne += 1
        A = mer + xs[ne:]
    hs = [('h', t, j) for t in range(T) for j in range(6)]

    def sim(lam):
        out = []
        credit = 0.0
        totA = sum(COST[i[0]] for i in A)
        capA = sum(cap[:nA])
        ia = ih = iw = 0
        accA = 0.0
        cumcap = 0.0
        rowrel = {}
        for t in range(nB):
            cumcap += cap[t]
            credit += lam * cap[t]
            while ia < len(A) and (t >= nA - 1 or accA <= totA * cumcap / capA * (nA - 1.0) / nA):
                it = A[ia]
                out.append((it, t))
                accA += COST[it[0]]
                credit -= COST[it[0]]
                if it[0] == 'r':
                    rowrel[it[1]] = t
                ia += 1
            while credit > 0:
                it = None
                hok = ih < len(hs) and (4 * hs[ih][1] + 5) in rowrel and rowrel[4 * hs[ih][1] + 5] + HLAG <= t
                wok = iw < len(ws)
                if hok and wok:
                    it = hs[ih] if ih * len(ws) <= iw * len(hs) + HPRI * len(ws) else ws[iw]
                elif hok:
                    it = hs[ih]
                elif wok and iw * len(hs) <= (ih + WAHEAD) * len(ws):
                    it = ws[iw]
                if it is None:
                    break
                if it[0] == 'h':
                    ih += 1
                else:
                    iw += 1
                out.append((it, t))
                credit -= COST[it[0]]
            credit = min(credit, 60.0)
        return out, (ih == len(hs) and iw == len(ws) and ia == len(A))
    lo, hi = 0.05, 4.0
    for _ in range(30):
        mid = 0.5 * (lo + hi)
        if sim(mid)[1]:
            hi = mid
        else:
            lo = mid
    out, ok = sim(hi)
    assert ok
    q = 0
    while out[q][1] < FTAU:
        q += 1
    out.insert(q, (('f',), FTAU))
    return out


def _sl(hh, p):
    return pl.ds(16 * hh + p, 8, stride=2)


def _unpack(w):
    e = pltpu.unpack_elementwise(w, index=0, packed_dtype=BF16, unpacked_dtype=F32)
    o = pltpu.unpack_elementwise(w, index=1, packed_dtype=BF16, unpacked_dtype=F32)
    return e, o


def _bt6(d):
    d0, d1, d2, d3, d4, d5 = d
    p = A2 * d2
    q = B2 * d2
    ea = d4 - q
    eb = d4 - p
    e0 = (ea - p) + d0
    p3 = A2 * d3
    q3 = B2 * d3
    wa = p3 - d1
    wb = q3 - d1
    oi = (d5 - wa) - q3
    ta = PB_ * wa
    tb = PA_ * wb
    return [e0, ea + ta, ea - ta, eb + tb, eb - tb, oi]


def _g6(g0, g1, g2, c1=C1, c2=C2):
    ea = c1 * g0 + (C1 * A2) * g2
    oa = (C1 * PA_) * g1
    eb = c2 * g0 + (C2 * B2) * g2
    ob = (C2 * PB_) * g1
    return [g0, ea + oa, ea - oa, eb + ob, eb - ob, g2]


class _AT:
    def __init__(self):
        self.v = {}
        self.z = [None] * 4

    def feed(self, i, m):
        v = self.v
        if i in (1, 3):
            v[i] = m
        elif i == 2:
            v['sa'] = v[1] + m
            v['da'] = v[1] - m
        elif i == 4:
            sb = v[3] + m
            db = v[3] - m
            v['p0'] = v['sa'] + sb
            self.z[1] = PA_ * v['da'] + PB_ * db
            self.z[2] = A2 * v['sa'] + B2 * sb
            v['p3'] = A3 * v['da'] + B3 * db
        elif i == 0:
            self.z[0] = v['p0'] + m
        else:
            self.z[3] = v['p3'] + m


def _kernel(x_hbm, temb_hbm, g1_hbm, be1_hbm, w1_hbm, wemb_hbm, g2_hbm, be2_hbm, w2_hbm,
            out_hbm,
            S, wraw, wt1, wt2, wembs, Wp, UA, UB, st, gb, off, scs, scp, zs, temb_ref, g1_ref, be1_ref, g2_ref, be2_ref, sems):
    wt = (wt1, wt2)

    def x_copy(b, c):
        return pltpu.make_async_copy(
            x_hbm.at[b, :, :, pl.ds(pl.multiple_of(c * 128, 128), 128)], S.bitcast(BF16).at[b, c],
            sems.at[b * NCH + c])

    def w_copy(k, c):
        src = w1_hbm if k == 0 else w2_hbm
        return pltpu.make_async_copy(src.at[:, :, pl.ds(c * 128, 128)], wraw.bitcast(BF16).at[k, c],
                                     sems.at[8 + k * NCH + c])

    def w1_piece(c, h):
        return pltpu.make_async_copy(w1_hbm.at[:, pl.ds(h * (C // NP), C // NP), pl.ds(c * 128, 128)],
                                     wraw.bitcast(BF16).at[0, c, :, pl.ds(h * (C // NP), C // NP)],
                                     sems.at[NSEM + c * NP + h])

    def wemb_copy():
        return pltpu.make_async_copy(wemb_hbm, wembs, sems.at[16])

    def out_copy(b, u, c):
        r0 = pl.multiple_of(u * RU, RU)
        return pltpu.make_async_copy(
            S.bitcast(BF16).at[b, c, pl.ds(r0, RU)],
            out_hbm.at[b, pl.ds(r0, RU), :, pl.ds(pl.multiple_of(c * 128, 128), 128)],
            sems.at[17 + (b * NU + u) * NCH + c])

    x_copy(0, 0).start()
    small = [pltpu.make_async_copy(src, dst, sems.at[NSEM + NCH * NP + q]) for q, (src, dst) in enumerate(
        ((g1_hbm, g1_ref), (be1_hbm, be1_ref), (g2_hbm, g2_ref), (be2_hbm, be2_ref), (temb_hbm, temb_ref)))]
    for cp in small:
        cp.start()
    for c in range(1, NCH):
        x_copy(0, c).start()
    for c in range(NCH):
        for h in range(NP):
            w1_piece(c, h).start()
    def start_rest(stage):
        if STOP == 'pro0':
            return
        if stage == DM[0]:
            for c in range(NCH):
                x_copy(1, c).start()
        if stage == DM[1]:
            for c in range(NCH):
                w_copy(1, c).start()
            wemb_copy().start()

    start_rest(0)
    for cp in small:
        cp.wait()
    zero8 = jnp.zeros((8, 128), F32)
    zs[...] = jnp.zeros((8, 128), U32)
    for c in range(NCH):
        sl = pl.ds(c * 128, 128)
        for q, r in enumerate((g1_ref, be1_ref, g2_ref, be2_ref)):
            gb[q, c] = jnp.broadcast_to(r[sl].astype(F32).reshape(1, 128), (8, 128))
        off[0, c] = zero8
        off[1, c] = zero8
    sub = lax.broadcasted_iota(jnp.int32, (8, 128), 0)

    def acc_stats(vals, piv, s1, s2):
        for q, v in enumerate(vals):
            d = v - piv
            k_ = q % len(s1)
            s1[k_] = s1[k_] + d
            s2[k_] = s2[k_] + d * d

    def put_stats(slot, c, u, piv, s1, s2):
        t1 = s1[0]
        t2 = s2[0]
        for q in range(1, len(s1)):
            t1 = t1 + s1[q]
            t2 = t2 + s2[q]
        st[slot, c, u, 0] = piv
        st[slot, c, u, 1] = t1
        st[slot, c, u, 2] = t2

    def x_stats_rolled(b, c):
        for u in range(NU):
            w0 = S[b, c, u * RU, pl.ds(0, 8), :]
            piv = jnp.broadcast_to(_unpack(w0)[0][0:1, :], (8, 128))

            def body(r, carry):
                s1 = list(carry[0])
                s2 = list(carry[1])
                vals = []
                for rr in range(XR):
                    for q in range(4):
                        vals += list(_unpack(S[b, c, u * RU + r * XR + rr, pl.ds(q * 8, 8), :]))
                acc_stats(vals, piv, s1, s2)
                return tuple(s1), tuple(s2)
            if XR == RU:
                s1, s2 = body(0, ((zero8,) * 4, (zero8,) * 4))
            else:
                s1, s2 = lax.fori_loop(0, RU // XR, body, ((zero8,) * 4, (zero8,) * 4))
            put_stats(b, c, u, piv, list(s1), list(s2))

    def finalize(kn, c, z=None):
        n = float(RU * W)
        kg = (kn // 2) * 2
        gam = gb[kg, c]
        bet = gb[kg + 1, c]
        of = off[kn, c]
        means = []
        m2s = []
        for u in range(NU):
            piv = st[kn, c, u, 0]
            t1 = st[kn, c, u, 1]
            t2 = st[kn, c, u, 2]
            if z is not None:
                t1 = z(t1)
                t2 = z(t2)
            s1 = jnp.sum(t1, axis=0, keepdims=True)
            s2 = jnp.sum(t2, axis=0, keepdims=True)
            means.append(piv[0:1] + s1 * (1.0 / n) + of[0:1])
            m2s.append(s2 - s1 * s1 * (1.0 / n))
        tot = means[0]
        for u in range(1, NU):
            tot = tot + means[u]
        gmean = jnp.sum(tot, axis=1, keepdims=True) * (1.0 / (NU * 128))
        acc = jnp.zeros((1, 128), F32)
        for u in range(NU):
            dm = means[u] - gmean
            acc = acc + m2s[u] + n * dm * dm
        var = jnp.sum(acc, axis=1, keepdims=True) * (1.0 / (NU * 128 * n))
        rstd = lax.rsqrt(var + EPS)
        sc = 0.5 * gam * rstd
        sh = 0.5 * bet + (of - gmean) * sc
        return sc, sh

    def w_row(kn, un, c, s, sc, sh, edge):
        h = un * RU - 1 + s
        if edge:
            valid = jnp.logical_and(h >= 0, h < H)
            h = jnp.clip(h, 0, H - 1)
        col = [[None] * 4 for _ in range(2)]
        for hh in range(2):
            for p in range(2):
                w = S[kn, c, h, _sl(hh, p), :]
                for e, v in enumerate(_unpack(w)):
                    uu = v * sc + sh
                    a = uu + uu * jnp.tanh(uu)
                    if edge:
                        a = jnp.where(valid, a, 0.0)
                    col[hh][2 * p + e] = a
        r0 = pltpu.roll(col[0][3], 1, 0)
        r1 = pltpu.roll(col[1][3], 1, 0)
        d0 = [jnp.where(sub == 0, 0.0, r0), jnp.where(sub == 0, r0, r1)]
        l0 = pltpu.roll(col[0][0], 7, 0)
        l1 = pltpu.roll(col[1][0], 7, 0)
        d5 = [jnp.where(sub == 7, l1, l0), jnp.where(sub == 7, 0.0, l1)]
        for hh in range(2):
            r = _bt6([d0[hh]] + col[hh] + [d5[hh]])
            for j in range(6):
                Wp[s, 2 * j + hh] = r[j]

    def h_tile(Ud, c, t, j, z=None):
        r = []
        for hh in range(2):
            d = [Wp[4 * t + q, 2 * j + hh] for q in range(6)]
            if z is not None:
                for q in HPQ:
                    d[q] = z(d[q])
            r.append(_bt6(d))
        r0 = t * 16 if isinstance(t, int) else pl.multiple_of(t * 16, 16)
        for i in range(6):
            Ud[i * 6 + j, c, pl.ds(r0, 16), :] = jnp.concatenate([r[0][i], r[1][i]], axis=0).astype(BF16)

    def produce_rolled(Ud, c):
        sc, sh = finalize(0, c)
        scp[c, 0] = sc
        scp[c, 1] = sh
        for q in range(12):
            Wp[0, q] = zero8

        def rbody(s, _):
            for rr in range(RR):
                w_row(0, 0, c, 1 + s * RR + rr, sc, sh, False)
            return 0
        if RR == NS - 1:
            rbody(0, 0)
        else:
            lax.fori_loop(0, (NS - 1) // RR, rbody, 0)

        def tbody(t, _):
            for tt in range(TR):
                for j in range(6):
                    h_tile(Ud, c, t * TR + tt, j)
            return 0
        if TR == T:
            tbody(0, 0)
        else:
            lax.fori_loop(0, T // TR, tbody, 0)

    def w_part(ksrc, kdst, c, r0, part, z=None):
        def tap(kh, kw):
            return wraw[ksrc, c, kh * 3 + kw, pl.ds(r0, 8), :]

        def cst(v):
            return v if z is None else z(jnp.full((8, 128), v, F32))
        if part in (0, 5):
            j = part
            w = [tap(kh, 0 if part == 0 else 2) for kh in range(3)]
            g = [_unpack(w[kh]) for kh in range(3)]
            c1, c2 = cst(C1), cst(C2)
            r = [_g6(g[0][h], g[1][h], g[2][h], c1, c2) for h in range(2)]
            wt[kdst][j, c, pl.ds(r0, 8), :] = w[0]
            wt[kdst][30 + j, c, pl.ds(r0, 8), :] = w[2]
            for i in range(1, 5):
                wt[kdst][i * 6 + j, c, pl.ds(r0, 8), :] = pltpu.pack_elementwise(
                    [r[0][i], r[1][i]], packed_dtype=BF16)
            return
        cc, pp = (C1, PA_) if part == 1 else (C2, PB_)
        ccv = cst(cc)
        tp = [[None] * 3 for _ in range(2)]
        tm = [[None] * 3 for _ in range(2)]
        for kh in range(3):
            g = [_unpack(tap(kh, kw)) for kw in range(3)]
            for h in range(2):
                e = ccv * g[0][h] + (cc * pp * pp) * g[2][h]
                o = (cc * pp) * g[1][h]
                tp[h][kh] = e + o
                tm[h][kh] = e - o
        for j, t in ((part, tp), (part + 1, tm)):
            r = [_g6(*t[h]) for h in range(2)]
            for i in range(6):
                wt[kdst][i * 6 + j, c, pl.ds(r0, 8), :] = pltpu.pack_elementwise(
                    [r[0][i], r[1][i]], packed_dtype=BF16)

    def w_block(k, c, r0):
        w = [[wraw[k, c, kh * 3 + kw, pl.ds(r0, 8), :] for kw in range(3)] for kh in range(3)]
        g = [[_unpack(w[kh][kw]) for kw in range(3)] for kh in range(3)]
        res = []
        for h in range(2):
            t = [_g6(g[kh][0][h], g[kh][1][h], g[kh][2][h]) for kh in range(3)]
            res.append([_g6(t[0][j], t[1][j], t[2][j]) for j in range(6)])
        for j in range(6):
            for i in range(6):
                if i in (0, 5) and j in (0, 5):
                    v = w[0 if i == 0 else 2][0 if j == 0 else 2]
                else:
                    v = pltpu.pack_elementwise([res[0][j][i], res[1][j][i]], packed_dtype=BF16)
                wt[k][i * 6 + j, c, pl.ds(r0, 8), :] = v

    def w_transform(k, c):
        def body(rb, _):
            w_block(k, c, pl.multiple_of(rb * 8, 8))
            return 0
        lax.fori_loop(0, C // 16, body, 0, unroll=2)

    def conv_body(k, nu, n, Uc, Un, extra):
        b = (nu // NU) % B
        u = nu % NU
        nn = jnp.minimum(nu + 1, 4 * NU - 1)
        kn = nn // NU
        un = nn % NU
        fmask = zs[...] != 0
        n64 = pl.multiple_of(n * 64, 64)

        ms = []
        col = [_AT() for _ in range(4)]
        fin = [[None] * 4 for _ in range(4)]

        def where(a, t, hh, p):
            return u * RU + 4 * t + a, _sl(hh, p)

        def finish(a, bc):
            y = col[a].z[bc]
            vs = []
            for t in range(T):
                for hh in range(2):
                    q = (2 * t + hh) * 8
                    v = y[q:q + 8]
                    if k == 1:
                        row, dst = where(a, t, hh, bc // 2)
                        v = v + pltpu.unpack_elementwise(S[b, n, row, dst, :], index=bc % 2,
                                                         packed_dtype=BF16, unpacked_dtype=F32)
                    vs.append(v)
            fin[a][bc] = vs

        anchor = pltpu.bitcast(wt[k][ORD[0] * 6 + ORD[0], 0, pl.ds(n64, 8), :], F32)
        for j in ORD:
            at = _AT()
            for i in ORD:
                L = jnp.concatenate(
                    [pltpu.bitcast(Uc.bitcast(U32)[i * 6 + j, c, pl.ds(0, M // 2), :], BF16) for c in range(NCH)], axis=1)
                Wm = jnp.concatenate(
                    [pltpu.bitcast(wt[k][i * 6 + j, c, pl.ds(n64, 64), :], BF16) for c in range(NCH)], axis=1)
                m = lax.dot_general(L, Wm, (((1,), (1,)), ((), ())), preferred_element_type=F32)
                ms.append(m)
                at.feed(i, m)
            for a in (1, 2, 0, 3):
                col[a].feed(j, at.z[a])
                if j == 4:
                    finish(a, 1)
                    finish(a, 2)
                elif j == 0:
                    finish(a, 0)
                elif j == 5:
                    finish(a, 3)

        def pacer(tau):
            ph, q = tau // 16, tau % 16
            mv = ms[ph][q * 8:q * 8 + 8, :]
            return lambda v: jnp.where(fmask, mv, v)

        par = n % 2
        sc = scs[par, 0]
        sh = scs[par, 1]
        nu2 = jnp.where(n == NCH - 1, nu + 1, nu)
        kn2 = jnp.minimum(nu2 + 1, 4 * NU - 1) // NU
        n2 = (n + 1) % NCH
        if extra == 'w':
            items = [('w%d' % part, q) for q in range(16) for part in (1, 0, 3, 5)]
            wc = nu - 1 + n // 2
            wr = (n % 2) * 128
        elif extra == 'x':
            items = [('x', q) for q in range(RU)]
            xsrc = jnp.minimum(nu // 2 + 1, 3)
            xdst = jnp.where(nu == 6, 4, xsrc)
            xs1 = [zero8] * 2
            xs2 = [zero8] * 2
            xpiv = [None, None]
        else:
            items = []
        for it, tau in _schedule(items, k):
            z = pacer(tau)
            if tau < FREE:
                z = lambda v: jnp.where(fmask, anchor, v)
            if it[0] == 'f':
                fsc, fsh = finalize(kn2, n2, z)
                scs[1 - par, 0] = fsc
                scs[1 - par, 1] = fsh
            elif it[0] == 'r':
                s = it[1]
                w_row(kn, un, n, s, z(sc), sh, s == 0 or s == NS - 1)
            elif it[0] == 'h':
                h_tile(Un, n, it[1], it[2], z if PACEH else None)
            elif it[0][0] == 'w':
                w_part(1, 1, wc, pl.multiple_of(wr + it[1] * 8, 8), int(it[0][1]), z)
            else:
                uu, r0 = it[1] // (RU // 2), (it[1] % (RU // 2)) * 2
                if xpiv[uu] is None:
                    xpiv[uu] = jnp.broadcast_to(_unpack(S[xsrc, n, uu * RU, pl.ds(0, 8), :])[0][0:1, :], (8, 128))
                    xs1 = [zero8] * 2
                    xs2 = [zero8] * 2
                pv = z(xpiv[uu])
                vals = []
                for r in range(2):
                    for q in range(4):
                        vals += list(_unpack(S[xsrc, n, uu * RU + r0 + r, pl.ds(q * 8, 8), :]))
                acc_stats(vals, pv, xs1, xs2)
                if r0 == RU - 2:
                    put_stats(xdst, n, uu, xpiv[uu], xs1, xs2)

        for p in range(2):
            for a in (1, 2, 0, 3):
                for t in range(T):
                    for hh in range(2):
                        row, dst = where(a, t, hh, p)
                        S[(2 + b) if k == 0 else b, n, row, dst, :] = pltpu.pack_elementwise(
                            [fin[a][2 * p][2 * t + hh], fin[a][2 * p + 1][2 * t + hh]], packed_dtype=BF16)
        if k == 1:
            out_copy(b, u, n).start()

    def emb_rows():
        te = temb_ref[...].astype(F32)
        th = 0.5 * te
        sil = th + th * jnp.tanh(th)
        return jnp.dot(sil.astype(BF16), wembs[...], preferred_element_type=F32)

    def pro(c, _):
        x_copy(0, c).wait()
        if 's' not in SKIP:
            x_stats_rolled(0, c)
        if 'u' not in SKIP:
            produce_rolled(UA, c)
        return 0
    lax.fori_loop(0, NCH, pro, 0)
    scs[0, 0] = scp[0, 0]
    scs[0, 1] = scp[0, 1]
    def wpro(q, _):
        c = q // NP
        h = q % NP
        pltpu.make_async_copy(w1_hbm.at[:, pl.ds(0, C // NP), pl.ds(0, 128)],
                              wraw.bitcast(BF16).at[0, c, :, pl.ds(pl.multiple_of(h * (C // NP), C // NP), C // NP)],
                              sems.at[NSEM + q]).wait()

        def body(rb, _):
            for q2 in range(WR):
                w_block(0, c, pl.multiple_of(h * (C // 2 // NP) + (rb * WR + q2) * 8, 8))
            return 0
        lax.fori_loop(0, C // 16 // NP // WR, body, 0)
        return 0
    lax.fori_loop(0, NCH * NP, wpro, 0)

    def pair(k):
        def f(p, _):
            nu = 2 * p

            def fa(n, _):
                if k == 0 and 'x' not in SKIP:
                    @pl.when(p == 0)
                    def _():
                        x_copy(1, n).wait()
                conv_body(k, nu, n, UA, UB, 'x')
                return 0

            def fb(n, _):
                conv_body(k, nu + 1, n, UB, UA, 'w' if k == 0 else None)
                return 0
            if k == 0:
                @pl.when(p == 1)
                def _():
                    wemb_copy().wait()
                    emb = emb_rows()
                    for bb in range(B):
                        for c in range(NCH):
                            off[2 + bb, c] = jnp.broadcast_to(emb[bb:bb + 1, c * 128:(c + 1) * 128], (8, 128))
            lax.fori_loop(0, NCH, fa, 0)
            if k == 0:
                @pl.when(p == 0)
                def _():
                    if 'x' in SKIP:
                        for c in range(NCH):
                            x_copy(1, c).wait()
                    w_copy(1, 0).wait()
                    w_copy(1, 1).wait()

                @pl.when(p == 1)
                def _():
                    w_copy(1, 2).wait()
                    w_copy(1, 3).wait()
            lax.fori_loop(0, NCH, fb, 0)
            return 0
        return f
    if STOP == 'pro0':
        return
    if STOP == 'pro':
        for c in range(NCH):
            x_copy(1, c).wait()
            w_copy(1, c).wait()
        wemb_copy().wait()
        return
    lax.fori_loop(0, NU, pair(0), 0)
    if STOP == 'c1':
        return
    def rep(_, __):
        lax.fori_loop(NU, 2 * NU, pair(1), 0)
        for b in range(B):
            for u in range(NU):
                for c in range(NCH):
                    out_copy(b, u, c).wait()
        return 0
    if REP > 1:
        lax.fori_loop(0, REP, rep, 0)
    else:
        rep(0, 0)


@jax.jit
def pallas_standalone__adm_resblock__diffusion_kernel(x, t_emb, g1, be1, w1, w_emb, g2, be2, w2):
    xn = jnp.transpose(x, (0, 2, 3, 1))
    w1n = jnp.transpose(w1, (2, 3, 0, 1)).reshape(9, C, C)
    w2n = jnp.transpose(w2, (2, 3, 0, 1)).reshape(9, C, C)
    vm = pl.BlockSpec(memory_space=pltpu.VMEM)
    hbm = pl.BlockSpec(memory_space=pl.ANY)
    out = pl.pallas_call(
        _kernel,
        out_shape=jax.ShapeDtypeStruct((B, H, W, C), BF16),
        in_specs=[hbm] * 9,
        out_specs=hbm,
        scratch_shapes=[
            pltpu.VMEM((4, NCH, H, WT, 128), U32),
            pltpu.VMEM((2, NCH, 9, C // 2, 128), U32),
            pltpu.VMEM((36, NCH, C // 2 + WPAD, 128), U32),
            pltpu.VMEM((36, NCH, C // 2 + WPAD, 128), U32),
            pltpu.VMEM((E, C), BF16),
            pltpu.VMEM((NS, 12 + PPAD, 8, 128), F32),
            pltpu.VMEM((36, NCH, M + UPAD, 128), BF16),
            pltpu.VMEM((36, NCH, M + UPAD, 128), BF16),
            pltpu.VMEM((5, NCH, NU, 3, 8, 128), F32),
            pltpu.VMEM((4, NCH, 8, 128), F32),
            pltpu.VMEM((4, NCH, 8, 128), F32),
            pltpu.VMEM((2, 2, 8, 128), F32),
            pltpu.VMEM((NCH, 2, 8, 128), F32),
            pltpu.VMEM((8, 128), U32),
            pltpu.VMEM((B, E), BF16),
            pltpu.VMEM((C,), BF16),
            pltpu.VMEM((C,), BF16),
            pltpu.VMEM((C,), BF16),
            pltpu.VMEM((C,), BF16),
            pltpu.SemaphoreType.DMA((NSEM + NCH * NP + 5,)),
        ],
        compiler_params=pltpu.CompilerParams(vmem_limit_bytes=110 * 1024 * 1024),
    )(xn, t_emb, g1, be1, w1n, w_emb, g2, be2, w2n)
    return jnp.transpose(out, (0, 3, 1, 2))
```

```python
import jax
import jax.numpy as jnp
from jax import lax
from jax.experimental import pallas as pl
from jax.experimental.pallas import tpu as pltpu

B, C, H, W, E = 2, 512, 64, 64, 1152
EPS = 1e-5
NCH = C // 128
WT = W // 2
T = 8
RU = 4 * T
NS = RU + 2
NU = H // RU
M = T * 16
ORD = (1, 2, 3, 4, 0, 5)

F32 = jnp.float32
BF16 = jnp.bfloat16
U32 = jnp.uint32

PA_ = 0.65
PB_ = 1.0 / PA_
A2, B2 = PA_ * PA_, PB_ * PB_
A3, B3 = A2 * PA_, B2 * PB_
C1 = 1.0 / (2.0 * A2 * (A2 - B2))
C2 = 1.0 / (2.0 * B2 * (B2 - A2))

ENDA = 29.0
ENDB = 35.9
HLAG = 2
HPRI = 3.0
WAHEAD = 4.0
FILL = 360.0
NACC = 2
STOP = ''
DM = [0, 0]
REP = 1
HPQ = [2, 3]
FREE = 0
FTAU = 200
SKIP = ''
WPAD = 8
UPAD = 16
PPAD = 1
XR = 8
RR = 33
TR = 8
WR = 8
NP = 4
NSEM = 17 + B * NU * NCH
ZP = 3
PACEH = 1


COST = {'r': 110.0, 'h': 44.0, 'w0': 36.0, 'w5': 36.0, 'w1': 116.0, 'w3': 116.0, 'x': 81.0}


def _schedule(extra=(), k=0):
    base = [48.0] * 36
    for g, j in enumerate(ORD):
        p = 6 * g
        base[p + 1] += 32
        base[p + 3] += 160
        base[p + 4] += 16
        base[p + 5] += 16
        fin = 16 * (0 if k == 0 else 2) * 4
        w = {1: 0, 2: 128, 3: 0, 4: 640 + 2 * fin, 0: 64 + fin + 64, 5: 64 + fin + 64}[j]
        if p + 6 < 36:
            base[p + 4] += w * 0.25
            base[p + 5] += w * 0.5
            base[p + 6] += w * 0.25
        else:
            base[p + 4] += w * 0.5
            base[p + 5] += w * 0.5
    nA = int(ENDA * 16)
    nB = int(ENDB * 16)
    cap = [max(FILL - base[t // 16], 24.0) / 16.0 for t in range(36 * 16)]
    A = [('r', s) for s in range(NS)]
    xs = [it for it in extra if it[0] == 'x']
    ws = [it for it in extra if it[0] != 'x']
    if xs:
        mer = []
        ne = 0
        for q, it in enumerate(A):
            mer.append(it)
            while ne < len(xs) and (ne + 0.5) / len(xs) <= (q + 1.0) / len(A):
                mer.append(xs[ne])
                ne += 1
        A = mer + xs[ne:]
    hs = [('h', t, j) for t in range(T) for j in range(6)]

    def sim(lam):
        out = []
        credit = 0.0
        totA = sum(COST[i[0]] for i in A)
        capA = sum(cap[:nA])
        ia = ih = iw = 0
        accA = 0.0
        cumcap = 0.0
        rowrel = {}
        for t in range(nB):
            cumcap += cap[t]
            credit += lam * cap[t]
            while ia < len(A) and (t >= nA - 1 or accA <= totA * cumcap / capA * (nA - 1.0) / nA):
                it = A[ia]
                out.append((it, t))
                accA += COST[it[0]]
                credit -= COST[it[0]]
                if it[0] == 'r':
                    rowrel[it[1]] = t
                ia += 1
            while credit > 0:
                it = None
                hok = ih < len(hs) and (4 * hs[ih][1] + 5) in rowrel and rowrel[4 * hs[ih][1] + 5] + HLAG <= t
                wok = iw < len(ws)
                if hok and wok:
                    it = hs[ih] if ih * len(ws) <= iw * len(hs) + HPRI * len(ws) else ws[iw]
                elif hok:
                    it = hs[ih]
                elif wok and iw * len(hs) <= (ih + WAHEAD) * len(ws):
                    it = ws[iw]
                if it is None:
                    break
                if it[0] == 'h':
                    ih += 1
                else:
                    iw += 1
                out.append((it, t))
                credit -= COST[it[0]]
            credit = min(credit, 60.0)
        return out, (ih == len(hs) and iw == len(ws) and ia == len(A))
    lo, hi = 0.05, 4.0
    for _ in range(30):
        mid = 0.5 * (lo + hi)
        if sim(mid)[1]:
            hi = mid
        else:
            lo = mid
    out, ok = sim(hi)
    assert ok
    q = 0
    while out[q][1] < FTAU:
        q += 1
    out.insert(q, (('f',), FTAU))
    return out


def _sl(hh, p):
    return pl.ds(16 * hh + p, 8, stride=2)


def _unpack(w):
    e = pltpu.unpack_elementwise(w, index=0, packed_dtype=BF16, unpacked_dtype=F32)
    o = pltpu.unpack_elementwise(w, index=1, packed_dtype=BF16, unpacked_dtype=F32)
    return e, o


def _bt6(d):
    d0, d1, d2, d3, d4, d5 = d
    p = A2 * d2
    q = B2 * d2
    ea = d4 - q
    eb = d4 - p
    e0 = (ea - p) + d0
    p3 = A2 * d3
    q3 = B2 * d3
    wa = p3 - d1
    wb = q3 - d1
    oi = (d5 - wa) - q3
    ta = PB_ * wa
    tb = PA_ * wb
    return [e0, ea + ta, ea - ta, eb + tb, eb - tb, oi]


def _g6(g0, g1, g2, c1=C1, c2=C2):
    ea = c1 * g0 + (C1 * A2) * g2
    oa = (C1 * PA_) * g1
    eb = c2 * g0 + (C2 * B2) * g2
    ob = (C2 * PB_) * g1
    return [g0, ea + oa, ea - oa, eb + ob, eb - ob, g2]


class _AT:
    def __init__(self):
        self.v = {}
        self.z = [None] * 4

    def feed(self, i, m):
        v = self.v
        if i in (1, 3):
            v[i] = m
        elif i == 2:
            v['sa'] = v[1] + m
            v['da'] = v[1] - m
        elif i == 4:
            sb = v[3] + m
            db = v[3] - m
            v['p0'] = v['sa'] + sb
            self.z[1] = PA_ * v['da'] + PB_ * db
            self.z[2] = A2 * v['sa'] + B2 * sb
            v['p3'] = A3 * v['da'] + B3 * db
        elif i == 0:
            self.z[0] = v['p0'] + m
        else:
            self.z[3] = v['p3'] + m


def _kernel(x_hbm, temb_hbm, g1_hbm, be1_hbm, w1_hbm, wemb_hbm, g2_hbm, be2_hbm, w2_hbm,
            out_hbm,
            zs, S, wraw, wt1, wt2, wembs, Wp, UA, UB, st, gb, off, scs, scp, temb_ref, g1_ref, be1_ref, g2_ref, be2_ref, sems):
    wt = (wt1, wt2)

    def x_copy(b, c):
        return pltpu.make_async_copy(
            x_hbm.at[b, :, :, pl.ds(pl.multiple_of(c * 128, 128), 128)], S.bitcast(BF16).at[b, c],
            sems.at[b * NCH + c])

    def w_copy(k, c):
        src = w1_hbm if k == 0 else w2_hbm
        return pltpu.make_async_copy(src.at[:, :, pl.ds(c * 128, 128)], wraw.bitcast(BF16).at[k, c],
                                     sems.at[8 + k * NCH + c])

    def w1_piece(c, h):
        return pltpu.make_async_copy(w1_hbm.at[:, pl.ds(h * (C // NP), C // NP), pl.ds(c * 128, 128)],
                                     wraw.bitcast(BF16).at[0, c, :, pl.ds(h * (C // NP), C // NP)],
                                     sems.at[NSEM + c * NP + h])

    def wemb_copy():
        return pltpu.make_async_copy(wemb_hbm, wembs, sems.at[16])

    def out_copy(b, u, c):
        r0 = pl.multiple_of(u * RU, RU)
        return pltpu.make_async_copy(
            S.bitcast(BF16).at[b, c, pl.ds(r0, RU)],
            out_hbm.at[b, pl.ds(r0, RU), :, pl.ds(pl.multiple_of(c * 128, 128), 128)],
            sems.at[17 + (b * NU + u) * NCH + c])

    x_copy(0, 0).start()
    small = [pltpu.make_async_copy(src, dst, sems.at[NSEM + NCH * NP + q]) for q, (src, dst) in enumerate(
        ((g1_hbm, g1_ref), (be1_hbm, be1_ref), (g2_hbm, g2_ref), (be2_hbm, be2_ref), (temb_hbm, temb_ref)))]
    for cp in small:
        cp.start()
    for c in range(1, NCH):
        x_copy(0, c).start()
    for c in range(NCH):
        for h in range(NP):
            w1_piece(c, h).start()
    def start_rest(stage):
        if STOP == 'pro0':
            return
        if stage == DM[0]:
            for c in range(NCH):
                x_copy(1, c).start()
        if stage == DM[1]:
            for c in range(NCH):
                w_copy(1, c).start()
            wemb_copy().start()

    start_rest(0)
    for cp in small:
        cp.wait()
    zero8 = jnp.zeros((8, 128), F32)
    zs[pl.ds(0, 8), :] = jnp.zeros((8, 128), U32)
    for c in range(NCH):
        sl = pl.ds(c * 128, 128)
        for q, r in enumerate((g1_ref, be1_ref, g2_ref, be2_ref)):
            gb[q, c] = jnp.broadcast_to(r[sl].astype(F32).reshape(1, 128), (8, 128))
        off[0, c] = zero8
        off[1, c] = zero8
    sub = lax.broadcasted_iota(jnp.int32, (8, 128), 0)

    def acc_stats(vals, piv, s1, s2):
        for q, v in enumerate(vals):
            d = v - piv
            k_ = q % len(s1)
            s1[k_] = s1[k_] + d
            s2[k_] = s2[k_] + d * d

    def put_stats(slot, c, u, piv, s1, s2):
        t1 = s1[0]
        t2 = s2[0]
        for q in range(1, len(s1)):
            t1 = t1 + s1[q]
            t2 = t2 + s2[q]
        st[slot, c, u, 0] = piv
        st[slot, c, u, 1] = t1
        st[slot, c, u, 2] = t2

    def x_stats_rolled(b, c):
        for u in range(NU):
            w0 = S[b, c, u * RU, pl.ds(0, 8), :]
            piv = jnp.broadcast_to(_unpack(w0)[0][0:1, :], (8, 128))

            def body(r, carry):
                s1 = list(carry[0])
                s2 = list(carry[1])
                vals = []
                for rr in range(XR):
                    for q in range(4):
                        vals += list(_unpack(S[b, c, u * RU + r * XR + rr, pl.ds(q * 8, 8), :]))
                acc_stats(vals, piv, s1, s2)
                return tuple(s1), tuple(s2)
            if XR == RU:
                s1, s2 = body(0, ((zero8,) * 4, (zero8,) * 4))
            else:
                s1, s2 = lax.fori_loop(0, RU // XR, body, ((zero8,) * 4, (zero8,) * 4))
            put_stats(b, c, u, piv, list(s1), list(s2))

    def finalize(kn, c, z=None):
        n = float(RU * W)
        kg = (kn // 2) * 2
        gam = gb[kg, c]
        bet = gb[kg + 1, c]
        of = off[kn, c]
        means = []
        m2s = []
        for u in range(NU):
            piv = st[kn, c, u, 0]
            t1 = st[kn, c, u, 1]
            t2 = st[kn, c, u, 2]
            if z is not None:
                t1 = z(t1)
                t2 = z(t2)
            s1 = jnp.sum(t1, axis=0, keepdims=True)
            s2 = jnp.sum(t2, axis=0, keepdims=True)
            means.append(piv[0:1] + s1 * (1.0 / n) + of[0:1])
            m2s.append(s2 - s1 * s1 * (1.0 / n))
        tot = means[0]
        for u in range(1, NU):
            tot = tot + means[u]
        gmean = jnp.sum(tot, axis=1, keepdims=True) * (1.0 / (NU * 128))
        acc = jnp.zeros((1, 128), F32)
        for u in range(NU):
            dm = means[u] - gmean
            acc = acc + m2s[u] + n * dm * dm
        var = jnp.sum(acc, axis=1, keepdims=True) * (1.0 / (NU * 128 * n))
        rstd = lax.rsqrt(var + EPS)
        sc = 0.5 * gam * rstd
        sh = 0.5 * bet + (of - gmean) * sc
        return sc, sh

    def w_row(kn, un, c, s, sc, sh, edge):
        h = un * RU - 1 + s
        if edge:
            valid = jnp.logical_and(h >= 0, h < H)
            h = jnp.clip(h, 0, H - 1)
        col = [[None] * 4 for _ in range(2)]
        for hh in range(2):
            for p in range(2):
                w = S[kn, c, h, _sl(hh, p), :]
                for e, v in enumerate(_unpack(w)):
                    uu = v * sc + sh
                    a = uu + uu * jnp.tanh(uu)
                    if edge:
                        a = jnp.where(valid, a, 0.0)
                    col[hh][2 * p + e] = a
        r0 = pltpu.roll(col[0][3], 1, 0)
        r1 = pltpu.roll(col[1][3], 1, 0)
        d0 = [jnp.where(sub == 0, 0.0, r0), jnp.where(sub == 0, r0, r1)]
        l0 = pltpu.roll(col[0][0], 7, 0)
        l1 = pltpu.roll(col[1][0], 7, 0)
        d5 = [jnp.where(sub == 7, l1, l0), jnp.where(sub == 7, 0.0, l1)]
        for hh in range(2):
            r = _bt6([d0[hh]] + col[hh] + [d5[hh]])
            for j in range(6):
                Wp[s, 2 * j + hh] = r[j]

    def h_tile(Ud, c, t, j, z=None):
        r = []
        for hh in range(2):
            d = [Wp[4 * t + q, 2 * j + hh] for q in range(6)]
            if z is not None:
                for q in HPQ:
                    d[q] = z(d[q])
            r.append(_bt6(d))
        r0 = t * 16 if isinstance(t, int) else pl.multiple_of(t * 16, 16)
        for i in range(6):
            Ud[i * 6 + j, c, pl.ds(r0, 16), :] = jnp.concatenate([r[0][i], r[1][i]], axis=0).astype(BF16)

    def produce_rolled(Ud, c):
        sc, sh = finalize(0, c)
        scp[c, 0] = sc
        scp[c, 1] = sh
        for q in range(12):
            Wp[0, q] = zero8

        def rbody(s, _):
            for rr in range(RR):
                w_row(0, 0, c, 1 + s * RR + rr, sc, sh, False)
            return 0
        if RR == NS - 1:
            rbody(0, 0)
        else:
            lax.fori_loop(0, (NS - 1) // RR, rbody, 0)

        def tbody(t, _):
            for tt in range(TR):
                for j in range(6):
                    h_tile(Ud, c, t * TR + tt, j)
            return 0
        if TR == T:
            tbody(0, 0)
        else:
            lax.fori_loop(0, T // TR, tbody, 0)

    def w_part(ksrc, kdst, c, r0, part, z=None):
        def tap(kh, kw):
            return wraw[ksrc, c, kh * 3 + kw, pl.ds(r0, 8), :]

        def cst(v):
            return v if z is None else z(jnp.full((8, 128), v, F32))
        if part in (0, 5):
            j = part
            w = [tap(kh, 0 if part == 0 else 2) for kh in range(3)]
            g = [_unpack(w[kh]) for kh in range(3)]
            c1, c2 = cst(C1), cst(C2)
            r = [_g6(g[0][h], g[1][h], g[2][h], c1, c2) for h in range(2)]
            wt[kdst][j, c, pl.ds(r0, 8), :] = w[0]
            wt[kdst][30 + j, c, pl.ds(r0, 8), :] = w[2]
            for i in range(1, 5):
                wt[kdst][i * 6 + j, c, pl.ds(r0, 8), :] = pltpu.pack_elementwise(
                    [r[0][i], r[1][i]], packed_dtype=BF16)
            return
        cc, pp = (C1, PA_) if part == 1 else (C2, PB_)
        ccv = cst(cc)
        tp = [[None] * 3 for _ in range(2)]
        tm = [[None] * 3 for _ in range(2)]
        for kh in range(3):
            g = [_unpack(tap(kh, kw)) for kw in range(3)]
            for h in range(2):
                e = ccv * g[0][h] + (cc * pp * pp) * g[2][h]
                o = (cc * pp) * g[1][h]
                tp[h][kh] = e + o
                tm[h][kh] = e - o
        for j, t in ((part, tp), (part + 1, tm)):
            r = [_g6(*t[h]) for h in range(2)]
            for i in range(6):
                wt[kdst][i * 6 + j, c, pl.ds(r0, 8), :] = pltpu.pack_elementwise(
                    [r[0][i], r[1][i]], packed_dtype=BF16)

    def w_block(k, c, r0):
        w = [[wraw[k, c, kh * 3 + kw, pl.ds(r0, 8), :] for kw in range(3)] for kh in range(3)]
        g = [[_unpack(w[kh][kw]) for kw in range(3)] for kh in range(3)]
        res = []
        for h in range(2):
            t = [_g6(g[kh][0][h], g[kh][1][h], g[kh][2][h]) for kh in range(3)]
            res.append([_g6(t[0][j], t[1][j], t[2][j]) for j in range(6)])
        for j in range(6):
            for i in range(6):
                if i in (0, 5) and j in (0, 5):
                    v = w[0 if i == 0 else 2][0 if j == 0 else 2]
                else:
                    v = pltpu.pack_elementwise([res[0][j][i], res[1][j][i]], packed_dtype=BF16)
                wt[k][i * 6 + j, c, pl.ds(r0, 8), :] = v

    def w_transform(k, c):
        def body(rb, _):
            w_block(k, c, pl.multiple_of(rb * 8, 8))
            return 0
        lax.fori_loop(0, C // 16, body, 0, unroll=2)

    def conv_body(k, nu, n, Uc, Un, extra):
        b = (nu // NU) % B
        u = nu % NU
        nn = jnp.minimum(nu + 1, 4 * NU - 1)
        kn = nn // NU
        un = nn % NU
        fmask = zs[pl.ds(0, 8), :] != 0
        n64 = pl.multiple_of(n * 64, 64)

        ms = []
        col = [_AT() for _ in range(4)]
        fin = [[None] * 4 for _ in range(4)]

        def where(a, t, hh, p):
            return u * RU + 4 * t + a, _sl(hh, p)

        def finish(a, bc):
            y = col[a].z[bc]
            vs = []
            for t in range(T):
                for hh in range(2):
                    q = (2 * t + hh) * 8
                    v = y[q:q + 8]
                    if k == 1:
                        row, dst = where(a, t, hh, bc // 2)
                        v = v + pltpu.unpack_elementwise(S[b, n, row, dst, :], index=bc % 2,
                                                         packed_dtype=BF16, unpacked_dtype=F32)
                    vs.append(v)
            fin[a][bc] = vs

        anchor = pltpu.bitcast(wt[k][ORD[0] * 6 + ORD[0], 0, pl.ds(n64, 8), :], F32)
        for j in ORD:
            at = _AT()
            for i in ORD:
                L = jnp.concatenate(
                    [pltpu.bitcast(Uc.bitcast(U32)[i * 6 + j, c, pl.ds(0, M // 2), :], BF16) for c in range(NCH)], axis=1)
                Wm = jnp.concatenate(
                    [pltpu.bitcast(wt[k][i * 6 + j, c, pl.ds(n64, 64), :], BF16) for c in range(NCH)], axis=1)
                m = lax.dot_general(L, Wm, (((1,), (1,)), ((), ())), preferred_element_type=F32)
                ms.append(m)
                at.feed(i, m)
            for a in (1, 2, 0, 3):
                col[a].feed(j, at.z[a])
                if j == 4:
                    finish(a, 1)
                    finish(a, 2)
                elif j == 0:
                    finish(a, 0)
                elif j == 5:
                    finish(a, 3)

        def pacer(tau):
            ph, q = tau // 16, tau % 16
            mv = ms[ph][q * 8:q * 8 + 8, :]
            return lambda v: jnp.where(fmask, mv, v)

        par = n % 2
        sc = scs[par, 0]
        sh = scs[par, 1]
        nu2 = jnp.where(n == NCH - 1, nu + 1, nu)
        kn2 = jnp.minimum(nu2 + 1, 4 * NU - 1) // NU
        n2 = (n + 1) % NCH
        if extra == 'w':
            items = [('w%d' % part, q) for q in range(16) for part in (1, 0, 3, 5)]
            wc = nu - 1 + n // 2
            wr = (n % 2) * 128
        elif extra == 'x':
            items = [('x', q) for q in range(RU)]
            xsrc = jnp.minimum(nu // 2 + 1, 3)
            xdst = jnp.where(nu == 6, 4, xsrc)
            xs1 = [zero8] * 2
            xs2 = [zero8] * 2
            xpiv = [None, None]
        else:
            items = []
        for it, tau in _schedule(items, k):
            z = pacer(tau)
            if tau < FREE:
                z = lambda v: jnp.where(fmask, anchor, v)
            if it[0] == 'f':
                fsc, fsh = finalize(kn2, n2, z)
                scs[1 - par, 0] = fsc
                scs[1 - par, 1] = fsh
            elif it[0] == 'r':
                s = it[1]
                w_row(kn, un, n, s, z(sc), sh, s == 0 or s == NS - 1)
            elif it[0] == 'h':
                h_tile(Un, n, it[1], it[2], z if PACEH else None)
            elif it[0][0] == 'w':
                w_part(1, 1, wc, pl.multiple_of(wr + it[1] * 8, 8), int(it[0][1]), z)
            else:
                uu, r0 = it[1] // (RU // 2), (it[1] % (RU // 2)) * 2
                if xpiv[uu] is None:
                    xpiv[uu] = jnp.broadcast_to(_unpack(S[xsrc, n, uu * RU, pl.ds(0, 8), :])[0][0:1, :], (8, 128))
                    xs1 = [zero8] * 2
                    xs2 = [zero8] * 2
                pv = z(xpiv[uu])
                vals = []
                for r in range(2):
                    for q in range(4):
                        vals += list(_unpack(S[xsrc, n, uu * RU + r0 + r, pl.ds(q * 8, 8), :]))
                acc_stats(vals, pv, xs1, xs2)
                if r0 == RU - 2:
                    put_stats(xdst, n, uu, xpiv[uu], xs1, xs2)

        for p in range(2):
            for a in (1, 2, 0, 3):
                for t in range(T):
                    for hh in range(2):
                        row, dst = where(a, t, hh, p)
                        S[(2 + b) if k == 0 else b, n, row, dst, :] = pltpu.pack_elementwise(
                            [fin[a][2 * p][2 * t + hh], fin[a][2 * p + 1][2 * t + hh]], packed_dtype=BF16)
        if k == 1:
            out_copy(b, u, n).start()

    def emb_rows():
        te = temb_ref[...].astype(F32)
        th = 0.5 * te
        sil = th + th * jnp.tanh(th)
        return jnp.dot(sil.astype(BF16), wembs[...], preferred_element_type=F32)

    def pro(c, _):
        x_copy(0, c).wait()
        if 's' not in SKIP:
            x_stats_rolled(0, c)
        if 'u' not in SKIP:
            produce_rolled(UA, c)
        return 0
    lax.fori_loop(0, NCH, pro, 0)
    start_rest(1)
    scs[0, 0] = scp[0, 0]
    scs[0, 1] = scp[0, 1]
    def wpro(q, _):
        c = q // NP
        h = q % NP
        pltpu.make_async_copy(w1_hbm.at[:, pl.ds(0, C // NP), pl.ds(0, 128)],
                              wraw.bitcast(BF16).at[0, c, :, pl.ds(pl.multiple_of(h * (C // NP), C // NP), C // NP)],
                              sems.at[NSEM + q]).wait()

        def body(rb, _):
            for q2 in range(WR):
                w_block(0, c, pl.multiple_of(h * (C // 2 // NP) + (rb * WR + q2) * 8, 8))
            return 0
        lax.fori_loop(0, C // 16 // NP // WR, body, 0)
        return 0
    if 2 in DM:
        lax.fori_loop(0, NCH * NP // 2, wpro, 0)
        start_rest(2)
        lax.fori_loop(NCH * NP // 2, NCH * NP, wpro, 0)
    else:
        lax.fori_loop(0, NCH * NP, wpro, 0)
    start_rest(3)

    def emb_block():
        wemb_copy().wait()
        emb = emb_rows()
        for bb in range(B):
            for c in range(NCH):
                off[2 + bb, c] = jnp.broadcast_to(emb[bb:bb + 1, c * 128:(c + 1) * 128], (8, 128))

    def pair(k):
        def f(p, _):
            nu = 2 * p

            def fa(n, _):
                if k == 0 and 'x' not in SKIP:
                    @pl.when(p == 0)
                    def _():
                        x_copy(1, n).wait()
                conv_body(k, nu, n, UA, UB, 'x')
                return 0

            def fb(n, _):
                conv_body(k, nu + 1, n, UB, UA, 'w' if k == 0 else None)
                return 0
            if k == 0:
                @pl.when(p == 1)
                def _():
                    emb_block()
            lax.fori_loop(0, NCH, fa, 0)
            if k == 0:
                @pl.when(p == 0)
                def _():
                    if 'x' in SKIP:
                        for c in range(NCH):
                            x_copy(1, c).wait()
                    w_copy(1, 0).wait()
                    w_copy(1, 1).wait()

                @pl.when(p == 1)
                def _():
                    w_copy(1, 2).wait()
                    w_copy(1, 3).wait()
            lax.fori_loop(0, NCH, fb, 0)
            return 0
        return f
    if STOP == 'pro0':
        return
    if STOP == 'pro':
        for c in range(NCH):
            x_copy(1, c).wait()
            w_copy(1, c).wait()
        wemb_copy().wait()
        return
    lax.fori_loop(0, NU, pair(0), 0)
    if STOP == 'c1':
        return
    def rep(_, __):
        lax.fori_loop(NU, 2 * NU, pair(1), 0)
        for b in range(B):
            for u in range(NU):
                for c in range(NCH):
                    out_copy(b, u, c).wait()
        return 0
    if REP > 1:
        lax.fori_loop(0, REP, rep, 0)
    else:
        rep(0, 0)


@jax.jit
def pallas_standalone__adm_resblock__diffusion_kernel(x, t_emb, g1, be1, w1, w_emb, g2, be2, w2):
    xn = jnp.transpose(x, (0, 2, 3, 1))
    w1n = jnp.transpose(w1, (2, 3, 0, 1)).reshape(9, C, C)
    w2n = jnp.transpose(w2, (2, 3, 0, 1)).reshape(9, C, C)
    vm = pl.BlockSpec(memory_space=pltpu.VMEM)
    hbm = pl.BlockSpec(memory_space=pl.ANY)
    out = pl.pallas_call(
        _kernel,
        out_shape=jax.ShapeDtypeStruct((B, H, W, C), BF16),
        in_specs=[hbm] * 9,
        out_specs=hbm,
        scratch_shapes=[
            pltpu.VMEM((ZP * 8, 128), U32),
            pltpu.VMEM((4, NCH, H, WT, 128), U32),
            pltpu.VMEM((2, NCH, 9, C // 2, 128), U32),
            pltpu.VMEM((36, NCH, C // 2 + WPAD, 128), U32),
            pltpu.VMEM((36, NCH, C // 2 + WPAD, 128), U32),
            pltpu.VMEM((E, C), BF16),
            pltpu.VMEM((NS, 12 + PPAD, 8, 128), F32),
            pltpu.VMEM((36, NCH, M + UPAD, 128), BF16),
            pltpu.VMEM((36, NCH, M + UPAD, 128), BF16),
            pltpu.VMEM((5, NCH, NU, 3, 8, 128), F32),
            pltpu.VMEM((4, NCH, 8, 128), F32),
            pltpu.VMEM((4, NCH, 8, 128), F32),
            pltpu.VMEM((2, 2, 8, 128), F32),
            pltpu.VMEM((NCH, 2, 8, 128), F32),
            pltpu.VMEM((B, E), BF16),
            pltpu.VMEM((C,), BF16),
            pltpu.VMEM((C,), BF16),
            pltpu.VMEM((C,), BF16),
            pltpu.VMEM((C,), BF16),
            pltpu.SemaphoreType.DMA((NSEM + NCH * NP + 5,)),
        ],
        compiler_params=pltpu.CompilerParams(vmem_limit_bytes=110 * 1024 * 1024),
    )(xn, t_emb, g1, be1, w1n, w_emb, g2, be2, w2n)
    return jnp.transpose(out, (0, 3, 1, 2))
```

```python
import jax
import jax.numpy as jnp
from jax import lax
from jax.experimental import pallas as pl
from jax.experimental.pallas import tpu as pltpu

B, C, H, W, E = 2, 512, 64, 64, 1152
EPS = 1e-5
NCH = C // 128
WT = W // 2
T = 8
RU = 4 * T
NS = RU + 2
NU = H // RU
M = T * 16
ORD = (1, 2, 3, 4, 0, 5)

F32 = jnp.float32
BF16 = jnp.bfloat16
U32 = jnp.uint32

PA_ = 0.65
PB_ = 1.0 / PA_
A2, B2 = PA_ * PA_, PB_ * PB_
A3, B3 = A2 * PA_, B2 * PB_
C1 = 1.0 / (2.0 * A2 * (A2 - B2))
C2 = 1.0 / (2.0 * B2 * (B2 - A2))

ENDA = 29.0
ENDB = 35.9
HLAG = 2
HPRI = 3.0
WAHEAD = 4.0
FILL = 360.0
NACC = 2
STOP = ''
DM = [0, 0]
REP = 1
HPQ = [2, 3]
FREE = 0
FTAU = 200
SKIP = ''
WPAD = 8
UPAD = 16
PPAD = 1
XR = 8
RR = 33
TR = 8
WR = 8
NP = 4
NSEM = 17 + B * NU * NCH
WHINT = 1
UNRS = [1, 2, 2, 2]
CP0 = 0
CPS = 12
ZP = 3
PACEH = 1


COST = {'r': 110.0, 'h': 44.0, 'w0': 36.0, 'w5': 36.0, 'w1': 116.0, 'w3': 116.0, 'x': 81.0}


def _schedule(extra=(), k=0):
    base = [48.0] * 36
    for g, j in enumerate(ORD):
        p = 6 * g
        base[p + 1] += 32
        base[p + 3] += 160
        base[p + 4] += 16
        base[p + 5] += 16
        fin = 16 * (0 if k == 0 else 2) * 4
        w = {1: 0, 2: 128, 3: 0, 4: 640 + 2 * fin, 0: 64 + fin + 64, 5: 64 + fin + 64}[j]
        if j == 4 and CP0 >= 0:
            for q in range(4):
                t0 = 16 * 24 + CP0 + CPS * q
                for tt in range(t0, t0 + 16):
                    base[min(tt // 16, 35)] += w / 64.0
        elif p + 6 < 36:
            base[p + 4] += w * 0.25
            base[p + 5] += w * 0.5
            base[p + 6] += w * 0.25
        else:
            base[p + 4] += w * 0.5
            base[p + 5] += w * 0.5
    nA = int(ENDA * 16)
    nB = int(ENDB * 16)
    cap = [max(FILL - base[t // 16], 24.0) / 16.0 for t in range(36 * 16)]
    A = [('r', s) for s in range(NS)]
    xs = [it for it in extra if it[0] == 'x']
    ws = [it for it in extra if it[0] != 'x']
    if xs:
        mer = []
        ne = 0
        for q, it in enumerate(A):
            mer.append(it)
            while ne < len(xs) and (ne + 0.5) / len(xs) <= (q + 1.0) / len(A):
                mer.append(xs[ne])
                ne += 1
        A = mer + xs[ne:]
    hs = [('h', t, j) for t in range(T) for j in range(6)]

    def sim(lam):
        out = []
        credit = 0.0
        totA = sum(COST[i[0]] for i in A)
        capA = sum(cap[:nA])
        ia = ih = iw = 0
        accA = 0.0
        cumcap = 0.0
        rowrel = {}
        for t in range(nB):
            cumcap += cap[t]
            credit += lam * cap[t]
            while ia < len(A) and (t >= nA - 1 or accA <= totA * cumcap / capA * (nA - 1.0) / nA):
                it = A[ia]
                out.append((it, t))
                accA += COST[it[0]]
                credit -= COST[it[0]]
                if it[0] == 'r':
                    rowrel[it[1]] = t
                ia += 1
            while credit > 0:
                it = None
                hok = ih < len(hs) and (4 * hs[ih][1] + 5) in rowrel and rowrel[4 * hs[ih][1] + 5] + HLAG <= t
                wok = iw < len(ws)
                if hok and wok:
                    it = hs[ih] if ih * len(ws) <= iw * len(hs) + HPRI * len(ws) else ws[iw]
                elif hok:
                    it = hs[ih]
                elif wok and iw * len(hs) <= (ih + WAHEAD) * len(ws):
                    it = ws[iw]
                if it is None:
                    break
                if it[0] == 'h':
                    ih += 1
                else:
                    iw += 1
                out.append((it, t))
                credit -= COST[it[0]]
            credit = min(credit, 60.0)
        return out, (ih == len(hs) and iw == len(ws) and ia == len(A))
    lo, hi = 0.05, 4.0
    for _ in range(30):
        mid = 0.5 * (lo + hi)
        if sim(mid)[1]:
            hi = mid
        else:
            lo = mid
    out, ok = sim(hi)
    assert ok
    q = 0
    while out[q][1] < FTAU:
        q += 1
    out.insert(q, (('f',), FTAU))
    return out


def _sl(hh, p):
    return pl.ds(16 * hh + p, 8, stride=2)


def _unpack(w):
    e = pltpu.unpack_elementwise(w, index=0, packed_dtype=BF16, unpacked_dtype=F32)
    o = pltpu.unpack_elementwise(w, index=1, packed_dtype=BF16, unpacked_dtype=F32)
    return e, o


def _bt6(d):
    d0, d1, d2, d3, d4, d5 = d
    p = A2 * d2
    q = B2 * d2
    ea = d4 - q
    eb = d4 - p
    e0 = (ea - p) + d0
    p3 = A2 * d3
    q3 = B2 * d3
    wa = p3 - d1
    wb = q3 - d1
    oi = (d5 - wa) - q3
    ta = PB_ * wa
    tb = PA_ * wb
    return [e0, ea + ta, ea - ta, eb + tb, eb - tb, oi]


def _g6(g0, g1, g2, c1=C1, c2=C2):
    ea = c1 * g0 + (C1 * A2) * g2
    oa = (C1 * PA_) * g1
    eb = c2 * g0 + (C2 * B2) * g2
    ob = (C2 * PB_) * g1
    return [g0, ea + oa, ea - oa, eb + ob, eb - ob, g2]


class _AT:
    def __init__(self):
        self.v = {}
        self.z = [None] * 4

    def feed(self, i, m):
        v = self.v
        if i in (1, 3):
            v[i] = m
        elif i == 2:
            v['sa'] = v[1] + m
            v['da'] = v[1] - m
        elif i == 4:
            sb = v[3] + m
            db = v[3] - m
            v['p0'] = v['sa'] + sb
            self.z[1] = PA_ * v['da'] + PB_ * db
            self.z[2] = A2 * v['sa'] + B2 * sb
            v['p3'] = A3 * v['da'] + B3 * db
        elif i == 0:
            self.z[0] = v['p0'] + m
        else:
            self.z[3] = v['p3'] + m


def _kernel(x_hbm, temb_hbm, g1_hbm, be1_hbm, w1_hbm, wemb_hbm, g2_hbm, be2_hbm, w2_hbm,
            out_hbm,
            zs, S, wraw, wt1, wt2, wembs, Wp, UA, UB, st, gb, off, scs, scp, temb_ref, g1_ref, be1_ref, g2_ref, be2_ref, sems):
    wt = (wt1, wt2)

    def x_copy(b, c):
        return pltpu.make_async_copy(
            x_hbm.at[b, :, :, pl.ds(pl.multiple_of(c * 128, 128), 128)], S.bitcast(BF16).at[b, c],
            sems.at[b * NCH + c])

    def w_copy(k, c):
        src = w1_hbm if k == 0 else w2_hbm
        return pltpu.make_async_copy(src.at[:, :, pl.ds(c * 128, 128)], wraw.bitcast(BF16).at[k, c],
                                     sems.at[8 + k * NCH + c])

    def w1_piece(c, h):
        return pltpu.make_async_copy(w1_hbm.at[:, pl.ds(h * (C // NP), C // NP), pl.ds(c * 128, 128)],
                                     wraw.bitcast(BF16).at[0, c, :, pl.ds(h * (C // NP), C // NP)],
                                     sems.at[NSEM + c * NP + h])

    def wemb_copy():
        return pltpu.make_async_copy(wemb_hbm, wembs, sems.at[16])

    def out_copy(b, u, c):
        r0 = pl.multiple_of(u * RU, RU)
        return pltpu.make_async_copy(
            S.bitcast(BF16).at[b, c, pl.ds(r0, RU)],
            out_hbm.at[b, pl.ds(r0, RU), :, pl.ds(pl.multiple_of(c * 128, 128), 128)],
            sems.at[17 + (b * NU + u) * NCH + c])

    x_copy(0, 0).start()
    small = [pltpu.make_async_copy(src, dst, sems.at[NSEM + NCH * NP + q]) for q, (src, dst) in enumerate(
        ((g1_hbm, g1_ref), (be1_hbm, be1_ref), (g2_hbm, g2_ref), (be2_hbm, be2_ref), (temb_hbm, temb_ref)))]
    for cp in small:
        cp.start()
    for c in range(1, NCH):
        x_copy(0, c).start()
    for c in range(NCH):
        for h in range(NP):
            w1_piece(c, h).start()
    def start_rest(stage):
        if STOP == 'pro0':
            return
        if stage == DM[0]:
            for c in range(NCH):
                x_copy(1, c).start()
        if stage == DM[1]:
            for c in range(NCH):
                w_copy(1, c).start()
            wemb_copy().start()

    start_rest(0)
    for cp in small:
        cp.wait()
    zero8 = jnp.zeros((8, 128), F32)
    zs[pl.ds(0, 8), :] = jnp.zeros((8, 128), U32)
    for c in range(NCH):
        sl = pl.ds(c * 128, 128)
        for q, r in enumerate((g1_ref, be1_ref, g2_ref, be2_ref)):
            gb[q, c] = jnp.broadcast_to(r[sl].astype(F32).reshape(1, 128), (8, 128))
        off[0, c] = zero8
        off[1, c] = zero8
    sub = lax.broadcasted_iota(jnp.int32, (8, 128), 0)

    def acc_stats(vals, piv, s1, s2):
        for q, v in enumerate(vals):
            d = v - piv
            k_ = q % len(s1)
            s1[k_] = s1[k_] + d
            s2[k_] = s2[k_] + d * d

    def put_stats(slot, c, u, piv, s1, s2):
        t1 = s1[0]
        t2 = s2[0]
        for q in range(1, len(s1)):
            t1 = t1 + s1[q]
            t2 = t2 + s2[q]
        st[slot, c, u, 0] = piv
        st[slot, c, u, 1] = t1
        st[slot, c, u, 2] = t2

    def x_stats_rolled(b, c):
        for u in range(NU):
            w0 = S[b, c, u * RU, pl.ds(0, 8), :]
            piv = jnp.broadcast_to(_unpack(w0)[0][0:1, :], (8, 128))

            def body(r, carry):
                s1 = list(carry[0])
                s2 = list(carry[1])
                vals = []
                for rr in range(XR):
                    for q in range(4):
                        vals += list(_unpack(S[b, c, u * RU + r * XR + rr, pl.ds(q * 8, 8), :]))
                acc_stats(vals, piv, s1, s2)
                return tuple(s1), tuple(s2)
            if XR == RU:
                s1, s2 = body(0, ((zero8,) * 4, (zero8,) * 4))
            else:
                s1, s2 = lax.fori_loop(0, RU // XR, body, ((zero8,) * 4, (zero8,) * 4))
            put_stats(b, c, u, piv, list(s1), list(s2))

    def finalize(kn, c, z=None):
        n = float(RU * W)
        kg = (kn // 2) * 2
        gam = gb[kg, c]
        bet = gb[kg + 1, c]
        of = off[kn, c]
        means = []
        m2s = []
        for u in range(NU):
            piv = st[kn, c, u, 0]
            t1 = st[kn, c, u, 1]
            t2 = st[kn, c, u, 2]
            if z is not None:
                t1 = z(t1)
                t2 = z(t2)
            s1 = jnp.sum(t1, axis=0, keepdims=True)
            s2 = jnp.sum(t2, axis=0, keepdims=True)
            means.append(piv[0:1] + s1 * (1.0 / n) + of[0:1])
            m2s.append(s2 - s1 * s1 * (1.0 / n))
        tot = means[0]
        for u in range(1, NU):
            tot = tot + means[u]
        gmean = jnp.sum(tot, axis=1, keepdims=True) * (1.0 / (NU * 128))
        acc = jnp.zeros((1, 128), F32)
        for u in range(NU):
            dm = means[u] - gmean
            acc = acc + m2s[u] + n * dm * dm
        var = jnp.sum(acc, axis=1, keepdims=True) * (1.0 / (NU * 128 * n))
        rstd = lax.rsqrt(var + EPS)
        sc = 0.5 * gam * rstd
        sh = 0.5 * bet + (of - gmean) * sc
        return sc, sh

    def w_row(kn, un, c, s, sc, sh, edge):
        h = un * RU - 1 + s
        if edge:
            valid = jnp.logical_and(h >= 0, h < H)
            h = jnp.clip(h, 0, H - 1)
        col = [[None] * 4 for _ in range(2)]
        for hh in range(2):
            for p in range(2):
                w = S[kn, c, h, _sl(hh, p), :]
                for e, v in enumerate(_unpack(w)):
                    uu = v * sc + sh
                    a = uu + uu * jnp.tanh(uu)
                    if edge:
                        a = jnp.where(valid, a, 0.0)
                    col[hh][2 * p + e] = a
        r0 = pltpu.roll(col[0][3], 1, 0)
        r1 = pltpu.roll(col[1][3], 1, 0)
        d0 = [jnp.where(sub == 0, 0.0, r0), jnp.where(sub == 0, r0, r1)]
        l0 = pltpu.roll(col[0][0], 7, 0)
        l1 = pltpu.roll(col[1][0], 7, 0)
        d5 = [jnp.where(sub == 7, l1, l0), jnp.where(sub == 7, 0.0, l1)]
        for hh in range(2):
            r = _bt6([d0[hh]] + col[hh] + [d5[hh]])
            for j in range(6):
                Wp[s, 2 * j + hh] = r[j]

    def h_tile(Ud, c, t, j, z=None):
        r = []
        for hh in range(2):
            d = [Wp[4 * t + q, 2 * j + hh] for q in range(6)]
            if z is not None:
                for q in HPQ:
                    d[q] = z(d[q])
            r.append(_bt6(d))
        r0 = t * 16 if isinstance(t, int) else pl.multiple_of(t * 16, 16)
        for i in range(6):
            Ud[i * 6 + j, c, pl.ds(r0, 16), :] = jnp.concatenate([r[0][i], r[1][i]], axis=0).astype(BF16)

    def produce_rolled(Ud, c):
        sc, sh = finalize(0, c)
        scp[c, 0] = sc
        scp[c, 1] = sh
        for q in range(12):
            Wp[0, q] = zero8

        def rbody(s, _):
            for rr in range(RR):
                w_row(0, 0, c, 1 + s * RR + rr, sc, sh, False)
            return 0
        if RR == NS - 1:
            rbody(0, 0)
        else:
            lax.fori_loop(0, (NS - 1) // RR, rbody, 0)

        def tbody(t, _):
            for tt in range(TR):
                for j in range(6):
                    h_tile(Ud, c, t * TR + tt, j)
            return 0
        if TR == T:
            tbody(0, 0)
        else:
            lax.fori_loop(0, T // TR, tbody, 0)

    def w_part(ksrc, kdst, c, r0, part, z=None):
        def tap(kh, kw):
            return wraw[ksrc, c, kh * 3 + kw, pl.ds(r0, 8), :]

        def cst(v):
            return v if z is None else z(jnp.full((8, 128), v, F32))
        if part in (0, 5):
            j = part
            w = [tap(kh, 0 if part == 0 else 2) for kh in range(3)]
            g = [_unpack(w[kh]) for kh in range(3)]
            c1, c2 = cst(C1), cst(C2)
            r = [_g6(g[0][h], g[1][h], g[2][h], c1, c2) for h in range(2)]
            wt[kdst][j, c, pl.ds(r0, 8), :] = w[0]
            wt[kdst][30 + j, c, pl.ds(r0, 8), :] = w[2]
            for i in range(1, 5):
                wt[kdst][i * 6 + j, c, pl.ds(r0, 8), :] = pltpu.pack_elementwise(
                    [r[0][i], r[1][i]], packed_dtype=BF16)
            return
        cc, pp = (C1, PA_) if part == 1 else (C2, PB_)
        ccv = cst(cc)
        tp = [[None] * 3 for _ in range(2)]
        tm = [[None] * 3 for _ in range(2)]
        for kh in range(3):
            g = [_unpack(tap(kh, kw)) for kw in range(3)]
            for h in range(2):
                e = ccv * g[0][h] + (cc * pp * pp) * g[2][h]
                o = (cc * pp) * g[1][h]
                tp[h][kh] = e + o
                tm[h][kh] = e - o
        for j, t in ((part, tp), (part + 1, tm)):
            r = [_g6(*t[h]) for h in range(2)]
            for i in range(6):
                wt[kdst][i * 6 + j, c, pl.ds(r0, 8), :] = pltpu.pack_elementwise(
                    [r[0][i], r[1][i]], packed_dtype=BF16)

    def w_block(k, c, r0):
        w = [[wraw[k, c, kh * 3 + kw, pl.ds(r0, 8), :] for kw in range(3)] for kh in range(3)]
        g = [[_unpack(w[kh][kw]) for kw in range(3)] for kh in range(3)]
        res = []
        for h in range(2):
            t = [_g6(g[kh][0][h], g[kh][1][h], g[kh][2][h]) for kh in range(3)]
            res.append([_g6(t[0][j], t[1][j], t[2][j]) for j in range(6)])
        for j in range(6):
            for i in range(6):
                if i in (0, 5) and j in (0, 5):
                    v = w[0 if i == 0 else 2][0 if j == 0 else 2]
                else:
                    v = pltpu.pack_elementwise([res[0][j][i], res[1][j][i]], packed_dtype=BF16)
                wt[k][i * 6 + j, c, pl.ds(r0, 8), :] = v

    def w_transform(k, c):
        def body(rb, _):
            w_block(k, c, pl.multiple_of(rb * 8, 8))
            return 0
        lax.fori_loop(0, C // 16, body, 0, unroll=2)

    def conv_body(k, nu, n, Uc, Un, extra):
        b = (nu // NU) % B
        u = nu % NU
        nn = jnp.minimum(nu + 1, 4 * NU - 1)
        kn = nn // NU
        un = nn % NU
        fmask = zs[pl.ds(0, 8), :] != 0
        n64 = pl.multiple_of(n * 64, 64)

        ms = []
        col = [_AT() for _ in range(4)]
        fin = [[None] * 4 for _ in range(4)]

        def where(a, t, hh, p):
            return u * RU + 4 * t + a, _sl(hh, p)

        def finish(a, bc):
            y = col[a].z[bc]
            vs = []
            for t in range(T):
                for hh in range(2):
                    q = (2 * t + hh) * 8
                    v = y[q:q + 8]
                    if k == 1:
                        row, dst = where(a, t, hh, bc // 2)
                        v = v + pltpu.unpack_elementwise(S[b, n, row, dst, :], index=bc % 2,
                                                         packed_dtype=BF16, unpacked_dtype=F32)
                    vs.append(v)
            fin[a][bc] = vs

        anchor = pltpu.bitcast(wt[k][ORD[0] * 6 + ORD[0], 0, pl.ds(n64, 8), :], F32)
        pend = []

        def col_feed(j, zz, zf=None):
            for q, a in enumerate((1, 2, 0, 3)):
                za = zz[a]
                if zf is not None:
                    z = zf(q)
                    za = jnp.concatenate([z(za[r * 8:r * 8 + 8]) for r in range(M // 8)], axis=0)
                col[a].feed(j, za)
                if j == 4:
                    finish(a, 1)
                    finish(a, 2)
                elif j == 0:
                    finish(a, 0)
                elif j == 5:
                    finish(a, 3)

        for j in ORD:
            at = _AT()
            for i in ORD:
                L = jnp.concatenate(
                    [pltpu.bitcast(Uc.bitcast(U32)[i * 6 + j, c, pl.ds(0, M // 2), :], BF16) for c in range(NCH)], axis=1)
                Wm = jnp.concatenate(
                    [pltpu.bitcast(wt[k][i * 6 + j, c, pl.ds(n64, 64), :], BF16) for c in range(NCH)], axis=1)
                m = lax.dot_general(L, Wm, (((1,), (1,)), ((), ())), preferred_element_type=F32)
                ms.append(m)
                at.feed(i, m)
            pend.append((j, at.z))
            if CP0 < 0 or j in (1, 2, 3):
                col_feed(*pend.pop(0))

        def pacer(tau):
            ph, q = tau // 16, tau % 16
            mv = ms[ph][q * 8:q * 8 + 8, :]
            return lambda v: jnp.where(fmask, mv, v)

        while pend:
            jj, zz = pend.pop(0)
            col_feed(jj, zz, (lambda q: pacer(16 * 24 + CP0 + CPS * q)) if jj == 4 else None)

        par = n % 2
        sc = scs[par, 0]
        sh = scs[par, 1]
        nu2 = jnp.where(n == NCH - 1, nu + 1, nu)
        kn2 = jnp.minimum(nu2 + 1, 4 * NU - 1) // NU
        n2 = (n + 1) % NCH
        if extra == 'w':
            items = [('w%d' % part, q) for q in range(16) for part in (1, 0, 3, 5)]
            wc = nu - 1 + n // 2
            wr = pl.multiple_of((n % 2) * 128, 128)
        elif extra == 'x':
            items = [('x', q) for q in range(RU)]
            xsrc = jnp.minimum(nu // 2 + 1, 3)
            xdst = jnp.where(nu == 6, 4, xsrc)
            xs1 = [zero8] * 2
            xs2 = [zero8] * 2
            xpiv = [None, None]
        else:
            items = []
        for it, tau in _schedule(items, k):
            z = pacer(tau)
            if tau < FREE:
                z = lambda v: jnp.where(fmask, anchor, v)
            if it[0] == 'f':
                fsc, fsh = finalize(kn2, n2, z)
                scs[1 - par, 0] = fsc
                scs[1 - par, 1] = fsh
            elif it[0] == 'r':
                s = it[1]
                w_row(kn, un, n, s, z(sc), sh, s == 0 or s == NS - 1)
            elif it[0] == 'h':
                h_tile(Un, n, it[1], it[2], z if PACEH else None)
            elif it[0][0] == 'w':
                w_part(1, 1, wc, (wr + it[1] * 8) if WHINT else pl.multiple_of(wr + it[1] * 8, 8), int(it[0][1]), z)
            else:
                uu, r0 = it[1] // (RU // 2), (it[1] % (RU // 2)) * 2
                if xpiv[uu] is None:
                    xpiv[uu] = jnp.broadcast_to(_unpack(S[xsrc, n, uu * RU, pl.ds(0, 8), :])[0][0:1, :], (8, 128))
                    xs1 = [zero8] * 2
                    xs2 = [zero8] * 2
                pv = z(xpiv[uu])
                vals = []
                for r in range(2):
                    for q in range(4):
                        vals += list(_unpack(S[xsrc, n, uu * RU + r0 + r, pl.ds(q * 8, 8), :]))
                acc_stats(vals, pv, xs1, xs2)
                if r0 == RU - 2:
                    put_stats(xdst, n, uu, xpiv[uu], xs1, xs2)

        for p in range(2):
            for a in (1, 2, 0, 3):
                for t in range(T):
                    for hh in range(2):
                        row, dst = where(a, t, hh, p)
                        S[(2 + b) if k == 0 else b, n, row, dst, :] = pltpu.pack_elementwise(
                            [fin[a][2 * p][2 * t + hh], fin[a][2 * p + 1][2 * t + hh]], packed_dtype=BF16)
        if k == 1:
            out_copy(b, u, n).start()

    def emb_rows():
        te = temb_ref[...].astype(F32)
        th = 0.5 * te
        sil = th + th * jnp.tanh(th)
        return jnp.dot(sil.astype(BF16), wembs[...], preferred_element_type=F32)

    def pro(c, _):
        x_copy(0, c).wait()
        if 's' not in SKIP:
            x_stats_rolled(0, c)
        if 'u' not in SKIP:
            produce_rolled(UA, c)
        return 0
    lax.fori_loop(0, NCH, pro, 0)
    start_rest(1)
    scs[0, 0] = scp[0, 0]
    scs[0, 1] = scp[0, 1]
    def wpro(q, _):
        c = q // NP
        h = q % NP
        pltpu.make_async_copy(w1_hbm.at[:, pl.ds(0, C // NP), pl.ds(0, 128)],
                              wraw.bitcast(BF16).at[0, c, :, pl.ds(pl.multiple_of(h * (C // NP), C // NP), C // NP)],
                              sems.at[NSEM + q]).wait()

        def body(rb, _):
            for q2 in range(WR):
                w_block(0, c, pl.multiple_of(h * (C // 2 // NP) + (rb * WR + q2) * 8, 8))
            return 0
        lax.fori_loop(0, C // 16 // NP // WR, body, 0)
        return 0
    if 2 in DM:
        lax.fori_loop(0, NCH * NP // 2, wpro, 0)
        start_rest(2)
        lax.fori_loop(NCH * NP // 2, NCH * NP, wpro, 0)
    else:
        lax.fori_loop(0, NCH * NP, wpro, 0)
    start_rest(3)

    def emb_block():
        wemb_copy().wait()
        emb = emb_rows()
        for bb in range(B):
            for c in range(NCH):
                off[2 + bb, c] = jnp.broadcast_to(emb[bb:bb + 1, c * 128:(c + 1) * 128], (8, 128))

    def pair(k):
        def f(p, _):
            nu = 2 * p

            ua = UNRS[0] if k == 0 else UNRS[2]
            ub = UNRS[1] if k == 0 else UNRS[3]

            def fa(n2, _):
                if k == 0 and 'x' not in SKIP:
                    @pl.when(p == 0)
                    def _():
                        for h in range(ua):
                            x_copy(1, n2 * ua + h).wait()
                for h in range(ua):
                    conv_body(k, nu, n2 * ua + h, UA, UB, 'x')
                return 0

            def fb(n2, _):
                for h in range(ub):
                    conv_body(k, nu + 1, n2 * ub + h, UB, UA, 'w' if k == 0 else None)
                return 0
            if k == 0:
                @pl.when(p == 1)
                def _():
                    emb_block()
            lax.fori_loop(0, NCH // ua, fa, 0)
            if k == 0:
                @pl.when(p == 0)
                def _():
                    if 'x' in SKIP:
                        for c in range(NCH):
                            x_copy(1, c).wait()
                    w_copy(1, 0).wait()
                    w_copy(1, 1).wait()

                @pl.when(p == 1)
                def _():
                    w_copy(1, 2).wait()
                    w_copy(1, 3).wait()
            lax.fori_loop(0, NCH // ub, fb, 0)
            return 0
        return f
    if STOP == 'pro0':
        return
    if STOP == 'pro':
        for c in range(NCH):
            x_copy(1, c).wait()
            w_copy(1, c).wait()
        wemb_copy().wait()
        return
    lax.fori_loop(0, NU, pair(0), 0)
    if STOP == 'c1':
        return
    def rep(_, __):
        lax.fori_loop(NU, 2 * NU, pair(1), 0)
        for b in range(B):
            for u in range(NU):
                for c in range(NCH):
                    out_copy(b, u, c).wait()
        return 0
    if REP > 1:
        lax.fori_loop(0, REP, rep, 0)
    else:
        rep(0, 0)


@jax.jit
def pallas_standalone__adm_resblock__diffusion_kernel(x, t_emb, g1, be1, w1, w_emb, g2, be2, w2):
    xn = jnp.transpose(x, (0, 2, 3, 1))
    w1n = jnp.transpose(w1, (2, 3, 0, 1)).reshape(9, C, C)
    w2n = jnp.transpose(w2, (2, 3, 0, 1)).reshape(9, C, C)
    vm = pl.BlockSpec(memory_space=pltpu.VMEM)
    hbm = pl.BlockSpec(memory_space=pl.ANY)
    out = pl.pallas_call(
        _kernel,
        out_shape=jax.ShapeDtypeStruct((B, H, W, C), BF16),
        in_specs=[hbm] * 9,
        out_specs=hbm,
        scratch_shapes=[
            pltpu.VMEM((ZP * 8, 128), U32),
            pltpu.VMEM((4, NCH, H, WT, 128), U32),
            pltpu.VMEM((2, NCH, 9, C // 2, 128), U32),
            pltpu.VMEM((36, NCH, C // 2 + WPAD, 128), U32),
            pltpu.VMEM((36, NCH, C // 2 + WPAD, 128), U32),
            pltpu.VMEM((E, C), BF16),
            pltpu.VMEM((NS, 12 + PPAD, 8, 128), F32),
            pltpu.VMEM((36, NCH, M + UPAD, 128), BF16),
            pltpu.VMEM((36, NCH, M + UPAD, 128), BF16),
            pltpu.VMEM((5, NCH, NU, 3, 8, 128), F32),
            pltpu.VMEM((4, NCH, 8, 128), F32),
            pltpu.VMEM((4, NCH, 8, 128), F32),
            pltpu.VMEM((2, 2, 8, 128), F32),
            pltpu.VMEM((NCH, 2, 8, 128), F32),
            pltpu.VMEM((B, E), BF16),
            pltpu.VMEM((C,), BF16),
            pltpu.VMEM((C,), BF16),
            pltpu.VMEM((C,), BF16),
            pltpu.VMEM((C,), BF16),
            pltpu.SemaphoreType.DMA((NSEM + NCH * NP + 5,)),
        ],
        compiler_params=pltpu.CompilerParams(vmem_limit_bytes=110 * 1024 * 1024),
    )(xn, t_emb, g1, be1, w1n, w_emb, g2, be2, w2n)
    return jnp.transpose(out, (0, 3, 1, 2))
```

```python
import jax
import jax.numpy as jnp
from jax import lax
from jax.experimental import pallas as pl
from jax.experimental.pallas import tpu as pltpu

B, C, H, W, E = 2, 512, 64, 64, 1152
EPS = 1e-5
NCH = C // 128
WT = W // 2
T = 8
RU = 4 * T
NS = RU + 2
NU = H // RU
M = T * 16
ORD = (1, 2, 3, 4, 0, 5)

F32 = jnp.float32
BF16 = jnp.bfloat16
U32 = jnp.uint32

PA_ = 0.65
PB_ = 1.0 / PA_
A2, B2 = PA_ * PA_, PB_ * PB_
A3, B3 = A2 * PA_, B2 * PB_
C1 = 1.0 / (2.0 * A2 * (A2 - B2))
C2 = 1.0 / (2.0 * B2 * (B2 - A2))

ENDA = [28.5, 28.5, 29.0, 29.0, 29.0, 29.0, 29.5, 29.5]
ENDB = [35.6, 35.6, 35.9, 35.9, 35.9, 35.9, 35.9, 35.0]
HLAG = [1, 4, 2, 2, 2, 2, 2, 6]
HPRI = [6.0, 6.0, 3.0, 3.0, 3.0, 3.0, 3.0, 3.0]
WAHEAD = [4.0, 4.0, 4.0, 4.0, 4.0, 2.0, 4.0, 4.0]
FILL = [347.0, 347.0, 360.0, 360.0, 360.0, 360.0, 360.0, 363.0]
NACC = 2
STOP = ''
DM = [0, 0]
REP = 1
HPQ = [2, 3]
FREE = 0
FTAU = [180, 180, 200, 200, 180, 180, 150, 260]
SKIP = ''
WPAD = 8
UPAD = 16
PPAD = 1
XR = 8
RR = 33
TR = 8
WR = 8
NP = 4
NSEM = 17 + B * NU * NCH
WHINT = 1
UNRS = [1, 2, 2, 2]
CP0 = [0, 0, 0, 0, 0, -1, 4, 4]
CPS = [12, 12, 12, 12, 12, 14, 12, 12]
ZP = 3
PACEH = 1


CR = [110.0, 110.0, 110.0, 110.0, 110.0, 120.0, 110.0, 110.0]
CH = [44.0, 44.0, 44.0, 44.0, 44.0, 44.0, 44.0, 44.0]
CX = [1.0, 1.0, 1.0, 1.0, 1.0, 1.0, 1.0, 1.0]


def _schedule(extra=(), k=0, bi=0):
    COST = {'r': CR[bi], 'h': CH[bi], 'w0': 36.0 * CX[bi], 'w5': 36.0 * CX[bi], 'w1': 116.0 * CX[bi], 'w3': 116.0 * CX[bi], 'x': 81.0 * CX[bi]}
    base = [48.0] * 36
    for g, j in enumerate(ORD):
        p = 6 * g
        base[p + 1] += 32
        base[p + 3] += 160
        base[p + 4] += 16
        base[p + 5] += 16
        fin = 16 * (0 if k == 0 else 2) * 4
        w = {1: 0, 2: 128, 3: 0, 4: 640 + 2 * fin, 0: 64 + fin + 64, 5: 64 + fin + 64}[j]
        if j == 4 and CP0[bi] >= 0:
            for q in range(4):
                t0 = 16 * 24 + CP0[bi] + CPS[bi] * q
                for tt in range(t0, t0 + 16):
                    base[min(tt // 16, 35)] += w / 64.0
        elif p + 6 < 36:
            base[p + 4] += w * 0.25
            base[p + 5] += w * 0.5
            base[p + 6] += w * 0.25
        else:
            base[p + 4] += w * 0.5
            base[p + 5] += w * 0.5
    nA = int(ENDA[bi] * 16)
    nB = int(ENDB[bi] * 16)
    cap = [max(FILL[bi] - base[t // 16], 24.0) / 16.0 for t in range(36 * 16)]
    A = [('r', s) for s in range(NS)]
    xs = [it for it in extra if it[0] == 'x']
    ws = [it for it in extra if it[0] != 'x']
    if xs:
        mer = []
        ne = 0
        for q, it in enumerate(A):
            mer.append(it)
            while ne < len(xs) and (ne + 0.5) / len(xs) <= (q + 1.0) / len(A):
                mer.append(xs[ne])
                ne += 1
        A = mer + xs[ne:]
    hs = [('h', t, j) for t in range(T) for j in range(6)]

    def sim(lam):
        out = []
        credit = 0.0
        totA = sum(COST[i[0]] for i in A)
        capA = sum(cap[:nA])
        ia = ih = iw = 0
        accA = 0.0
        cumcap = 0.0
        rowrel = {}
        for t in range(nB):
            cumcap += cap[t]
            credit += lam * cap[t]
            while ia < len(A) and (t >= nA - 1 or accA <= totA * cumcap / capA * (nA - 1.0) / nA):
                it = A[ia]
                out.append((it, t))
                accA += COST[it[0]]
                credit -= COST[it[0]]
                if it[0] == 'r':
                    rowrel[it[1]] = t
                ia += 1
            while credit > 0:
                it = None
                hok = ih < len(hs) and (4 * hs[ih][1] + 5) in rowrel and rowrel[4 * hs[ih][1] + 5] + HLAG[bi] <= t
                wok = iw < len(ws)
                if hok and wok:
                    it = hs[ih] if ih * len(ws) <= iw * len(hs) + HPRI[bi] * len(ws) else ws[iw]
                elif hok:
                    it = hs[ih]
                elif wok and iw * len(hs) <= (ih + WAHEAD[bi]) * len(ws):
                    it = ws[iw]
                if it is None:
                    break
                if it[0] == 'h':
                    ih += 1
                else:
                    iw += 1
                out.append((it, t))
                credit -= COST[it[0]]
            credit = min(credit, 60.0)
        return out, (ih == len(hs) and iw == len(ws) and ia == len(A))
    lo, hi = 0.05, 4.0
    for _ in range(30):
        mid = 0.5 * (lo + hi)
        if sim(mid)[1]:
            hi = mid
        else:
            lo = mid
    out, ok = sim(hi)
    assert ok
    q = 0
    while out[q][1] < FTAU[bi]:
        q += 1
    out.insert(q, (('f',), FTAU[bi]))
    return out


def _sl(hh, p):
    return pl.ds(16 * hh + p, 8, stride=2)


def _unpack(w):
    e = pltpu.unpack_elementwise(w, index=0, packed_dtype=BF16, unpacked_dtype=F32)
    o = pltpu.unpack_elementwise(w, index=1, packed_dtype=BF16, unpacked_dtype=F32)
    return e, o


def _bt6(d):
    d0, d1, d2, d3, d4, d5 = d
    p = A2 * d2
    q = B2 * d2
    ea = d4 - q
    eb = d4 - p
    e0 = (ea - p) + d0
    p3 = A2 * d3
    q3 = B2 * d3
    wa = p3 - d1
    wb = q3 - d1
    oi = (d5 - wa) - q3
    ta = PB_ * wa
    tb = PA_ * wb
    return [e0, ea + ta, ea - ta, eb + tb, eb - tb, oi]


def _g6(g0, g1, g2, c1=C1, c2=C2):
    ea = c1 * g0 + (C1 * A2) * g2
    oa = (C1 * PA_) * g1
    eb = c2 * g0 + (C2 * B2) * g2
    ob = (C2 * PB_) * g1
    return [g0, ea + oa, ea - oa, eb + ob, eb - ob, g2]


class _AT:
    def __init__(self):
        self.v = {}
        self.z = [None] * 4

    def feed(self, i, m):
        v = self.v
        if i in (1, 3):
            v[i] = m
        elif i == 2:
            v['sa'] = v[1] + m
            v['da'] = v[1] - m
        elif i == 4:
            sb = v[3] + m
            db = v[3] - m
            v['p0'] = v['sa'] + sb
            self.z[1] = PA_ * v['da'] + PB_ * db
            self.z[2] = A2 * v['sa'] + B2 * sb
            v['p3'] = A3 * v['da'] + B3 * db
        elif i == 0:
            self.z[0] = v['p0'] + m
        else:
            self.z[3] = v['p3'] + m


def _kernel(x_hbm, temb_hbm, g1_hbm, be1_hbm, w1_hbm, wemb_hbm, g2_hbm, be2_hbm, w2_hbm,
            out_hbm,
            zs, S, wraw, wt1, wt2, wembs, Wp, UA, UB, st, gb, off, scs, scp, temb_ref, g1_ref, be1_ref, g2_ref, be2_ref, sems):
    wt = (wt1, wt2)

    def x_copy(b, c):
        return pltpu.make_async_copy(
            x_hbm.at[b, :, :, pl.ds(pl.multiple_of(c * 128, 128), 128)], S.bitcast(BF16).at[b, c],
            sems.at[b * NCH + c])

    def w_copy(k, c):
        src = w1_hbm if k == 0 else w2_hbm
        return pltpu.make_async_copy(src.at[:, :, pl.ds(c * 128, 128)], wraw.bitcast(BF16).at[k, c],
                                     sems.at[8 + k * NCH + c])

    def w1_piece(c, h):
        return pltpu.make_async_copy(w1_hbm.at[:, pl.ds(h * (C // NP), C // NP), pl.ds(c * 128, 128)],
                                     wraw.bitcast(BF16).at[0, c, :, pl.ds(h * (C // NP), C // NP)],
                                     sems.at[NSEM + c * NP + h])

    def wemb_copy():
        return pltpu.make_async_copy(wemb_hbm, wembs, sems.at[16])

    def out_copy(b, u, c):
        r0 = pl.multiple_of(u * RU, RU)
        return pltpu.make_async_copy(
            S.bitcast(BF16).at[b, c, pl.ds(r0, RU)],
            out_hbm.at[b, pl.ds(r0, RU), :, pl.ds(pl.multiple_of(c * 128, 128), 128)],
            sems.at[17 + (b * NU + u) * NCH + c])

    x_copy(0, 0).start()
    small = [pltpu.make_async_copy(src, dst, sems.at[NSEM + NCH * NP + q]) for q, (src, dst) in enumerate(
        ((g1_hbm, g1_ref), (be1_hbm, be1_ref), (g2_hbm, g2_ref), (be2_hbm, be2_ref), (temb_hbm, temb_ref)))]
    for cp in small:
        cp.start()
    for c in range(1, NCH):
        x_copy(0, c).start()
    for c in range(NCH):
        for h in range(NP):
            w1_piece(c, h).start()
    def start_rest(stage):
        if STOP == 'pro0':
            return
        if stage == DM[0]:
            for c in range(NCH):
                x_copy(1, c).start()
        if stage == DM[1]:
            for c in range(NCH):
                w_copy(1, c).start()
            wemb_copy().start()

    start_rest(0)
    for cp in small:
        cp.wait()
    zero8 = jnp.zeros((8, 128), F32)
    zs[pl.ds(0, 8), :] = jnp.zeros((8, 128), U32)
    for c in range(NCH):
        sl = pl.ds(c * 128, 128)
        for q, r in enumerate((g1_ref, be1_ref, g2_ref, be2_ref)):
            gb[q, c] = jnp.broadcast_to(r[sl].astype(F32).reshape(1, 128), (8, 128))
        off[0, c] = zero8
        off[1, c] = zero8
    sub = lax.broadcasted_iota(jnp.int32, (8, 128), 0)

    def acc_stats(vals, piv, s1, s2):
        for q, v in enumerate(vals):
            d = v - piv
            k_ = q % len(s1)
            s1[k_] = s1[k_] + d
            s2[k_] = s2[k_] + d * d

    def put_stats(slot, c, u, piv, s1, s2):
        t1 = s1[0]
        t2 = s2[0]
        for q in range(1, len(s1)):
            t1 = t1 + s1[q]
            t2 = t2 + s2[q]
        st[slot, c, u, 0] = piv
        st[slot, c, u, 1] = t1
        st[slot, c, u, 2] = t2

    def x_stats_rolled(b, c):
        for u in range(NU):
            w0 = S[b, c, u * RU, pl.ds(0, 8), :]
            piv = jnp.broadcast_to(_unpack(w0)[0][0:1, :], (8, 128))

            def body(r, carry):
                s1 = list(carry[0])
                s2 = list(carry[1])
                vals = []
                for rr in range(XR):
                    for q in range(4):
                        vals += list(_unpack(S[b, c, u * RU + r * XR + rr, pl.ds(q * 8, 8), :]))
                acc_stats(vals, piv, s1, s2)
                return tuple(s1), tuple(s2)
            if XR == RU:
                s1, s2 = body(0, ((zero8,) * 4, (zero8,) * 4))
            else:
                s1, s2 = lax.fori_loop(0, RU // XR, body, ((zero8,) * 4, (zero8,) * 4))
            put_stats(b, c, u, piv, list(s1), list(s2))

    def finalize(kn, c, z=None):
        n = float(RU * W)
        kg = (kn // 2) * 2
        gam = gb[kg, c]
        bet = gb[kg + 1, c]
        of = off[kn, c]
        means = []
        m2s = []
        for u in range(NU):
            piv = st[kn, c, u, 0]
            t1 = st[kn, c, u, 1]
            t2 = st[kn, c, u, 2]
            if z is not None:
                t1 = z(t1)
                t2 = z(t2)
            s1 = jnp.sum(t1, axis=0, keepdims=True)
            s2 = jnp.sum(t2, axis=0, keepdims=True)
            means.append(piv[0:1] + s1 * (1.0 / n) + of[0:1])
            m2s.append(s2 - s1 * s1 * (1.0 / n))
        tot = means[0]
        for u in range(1, NU):
            tot = tot + means[u]
        gmean = jnp.sum(tot, axis=1, keepdims=True) * (1.0 / (NU * 128))
        acc = jnp.zeros((1, 128), F32)
        for u in range(NU):
            dm = means[u] - gmean
            acc = acc + m2s[u] + n * dm * dm
        var = jnp.sum(acc, axis=1, keepdims=True) * (1.0 / (NU * 128 * n))
        rstd = lax.rsqrt(var + EPS)
        sc = 0.5 * gam * rstd
        sh = 0.5 * bet + (of - gmean) * sc
        return sc, sh

    def w_row(kn, un, c, s, sc, sh, edge):
        h = un * RU - 1 + s
        if edge:
            valid = jnp.logical_and(h >= 0, h < H)
            h = jnp.clip(h, 0, H - 1)
        col = [[None] * 4 for _ in range(2)]
        for hh in range(2):
            for p in range(2):
                w = S[kn, c, h, _sl(hh, p), :]
                for e, v in enumerate(_unpack(w)):
                    uu = v * sc + sh
                    a = uu + uu * jnp.tanh(uu)
                    if edge:
                        a = jnp.where(valid, a, 0.0)
                    col[hh][2 * p + e] = a
        r0 = pltpu.roll(col[0][3], 1, 0)
        r1 = pltpu.roll(col[1][3], 1, 0)
        d0 = [jnp.where(sub == 0, 0.0, r0), jnp.where(sub == 0, r0, r1)]
        l0 = pltpu.roll(col[0][0], 7, 0)
        l1 = pltpu.roll(col[1][0], 7, 0)
        d5 = [jnp.where(sub == 7, l1, l0), jnp.where(sub == 7, 0.0, l1)]
        for hh in range(2):
            r = _bt6([d0[hh]] + col[hh] + [d5[hh]])
            for j in range(6):
                Wp[s, 2 * j + hh] = r[j]

    def h_tile(Ud, c, t, j, z=None):
        r = []
        for hh in range(2):
            d = [Wp[4 * t + q, 2 * j + hh] for q in range(6)]
            if z is not None:
                for q in HPQ:
                    d[q] = z(d[q])
            r.append(_bt6(d))
        r0 = t * 16 if isinstance(t, int) else pl.multiple_of(t * 16, 16)
        for i in range(6):
            Ud[i * 6 + j, c, pl.ds(r0, 16), :] = jnp.concatenate([r[0][i], r[1][i]], axis=0).astype(BF16)

    def produce_rolled(Ud, c):
        sc, sh = finalize(0, c)
        scp[c, 0] = sc
        scp[c, 1] = sh
        for q in range(12):
            Wp[0, q] = zero8

        def rbody(s, _):
            for rr in range(RR):
                w_row(0, 0, c, 1 + s * RR + rr, sc, sh, False)
            return 0
        if RR == NS - 1:
            rbody(0, 0)
        else:
            lax.fori_loop(0, (NS - 1) // RR, rbody, 0)

        def tbody(t, _):
            for tt in range(TR):
                for j in range(6):
                    h_tile(Ud, c, t * TR + tt, j)
            return 0
        if TR == T:
            tbody(0, 0)
        else:
            lax.fori_loop(0, T // TR, tbody, 0)

    def w_part(ksrc, kdst, c, r0, part, z=None):
        def tap(kh, kw):
            return wraw[ksrc, c, kh * 3 + kw, pl.ds(r0, 8), :]

        def cst(v):
            return v if z is None else z(jnp.full((8, 128), v, F32))
        if part in (0, 5):
            j = part
            w = [tap(kh, 0 if part == 0 else 2) for kh in range(3)]
            g = [_unpack(w[kh]) for kh in range(3)]
            c1, c2 = cst(C1), cst(C2)
            r = [_g6(g[0][h], g[1][h], g[2][h], c1, c2) for h in range(2)]
            wt[kdst][j, c, pl.ds(r0, 8), :] = w[0]
            wt[kdst][30 + j, c, pl.ds(r0, 8), :] = w[2]
            for i in range(1, 5):
                wt[kdst][i * 6 + j, c, pl.ds(r0, 8), :] = pltpu.pack_elementwise(
                    [r[0][i], r[1][i]], packed_dtype=BF16)
            return
        cc, pp = (C1, PA_) if part == 1 else (C2, PB_)
        ccv = cst(cc)
        tp = [[None] * 3 for _ in range(2)]
        tm = [[None] * 3 for _ in range(2)]
        for kh in range(3):
            g = [_unpack(tap(kh, kw)) for kw in range(3)]
            for h in range(2):
                e = ccv * g[0][h] + (cc * pp * pp) * g[2][h]
                o = (cc * pp) * g[1][h]
                tp[h][kh] = e + o
                tm[h][kh] = e - o
        for j, t in ((part, tp), (part + 1, tm)):
            r = [_g6(*t[h]) for h in range(2)]
            for i in range(6):
                wt[kdst][i * 6 + j, c, pl.ds(r0, 8), :] = pltpu.pack_elementwise(
                    [r[0][i], r[1][i]], packed_dtype=BF16)

    def w_block(k, c, r0):
        w = [[wraw[k, c, kh * 3 + kw, pl.ds(r0, 8), :] for kw in range(3)] for kh in range(3)]
        g = [[_unpack(w[kh][kw]) for kw in range(3)] for kh in range(3)]
        res = []
        for h in range(2):
            t = [_g6(g[kh][0][h], g[kh][1][h], g[kh][2][h]) for kh in range(3)]
            res.append([_g6(t[0][j], t[1][j], t[2][j]) for j in range(6)])
        for j in range(6):
            for i in range(6):
                if i in (0, 5) and j in (0, 5):
                    v = w[0 if i == 0 else 2][0 if j == 0 else 2]
                else:
                    v = pltpu.pack_elementwise([res[0][j][i], res[1][j][i]], packed_dtype=BF16)
                wt[k][i * 6 + j, c, pl.ds(r0, 8), :] = v

    def w_transform(k, c):
        def body(rb, _):
            w_block(k, c, pl.multiple_of(rb * 8, 8))
            return 0
        lax.fori_loop(0, C // 16, body, 0, unroll=2)

    def conv_body(k, nu, n, Uc, Un, extra, half=0):
        b = (nu // NU) % B
        u = nu % NU
        nn = jnp.minimum(nu + 1, 4 * NU - 1)
        kn = nn // NU
        un = nn % NU
        fmask = zs[pl.ds(0, 8), :] != 0
        n64 = pl.multiple_of(n * 64, 64)

        ms = []
        col = [_AT() for _ in range(4)]
        fin = [[None] * 4 for _ in range(4)]

        def where(a, t, hh, p):
            return u * RU + 4 * t + a, _sl(hh, p)

        def finish(a, bc):
            y = col[a].z[bc]
            vs = []
            for t in range(T):
                for hh in range(2):
                    q = (2 * t + hh) * 8
                    v = y[q:q + 8]
                    if k == 1:
                        row, dst = where(a, t, hh, bc // 2)
                        v = v + pltpu.unpack_elementwise(S[b, n, row, dst, :], index=bc % 2,
                                                         packed_dtype=BF16, unpacked_dtype=F32)
                    vs.append(v)
            fin[a][bc] = vs

        bi = 2 * (2 * k + (0 if extra == 'x' else 1)) + half
        anchor = pltpu.bitcast(wt[k][ORD[0] * 6 + ORD[0], 0, pl.ds(n64, 8), :], F32)
        pend = []

        def col_feed(j, zz, zf=None):
            for q, a in enumerate((1, 2, 0, 3)):
                za = zz[a]
                if zf is not None:
                    z = zf(q)
                    za = jnp.concatenate([z(za[r * 8:r * 8 + 8]) for r in range(M // 8)], axis=0)
                col[a].feed(j, za)
                if j == 4:
                    finish(a, 1)
                    finish(a, 2)
                elif j == 0:
                    finish(a, 0)
                elif j == 5:
                    finish(a, 3)

        for j in ORD:
            at = _AT()
            for i in ORD:
                L = jnp.concatenate(
                    [pltpu.bitcast(Uc.bitcast(U32)[i * 6 + j, c, pl.ds(0, M // 2), :], BF16) for c in range(NCH)], axis=1)
                Wm = jnp.concatenate(
                    [pltpu.bitcast(wt[k][i * 6 + j, c, pl.ds(n64, 64), :], BF16) for c in range(NCH)], axis=1)
                m = lax.dot_general(L, Wm, (((1,), (1,)), ((), ())), preferred_element_type=F32)
                ms.append(m)
                at.feed(i, m)
            pend.append((j, at.z))
            if CP0[bi] < 0 or j in (1, 2, 3):
                col_feed(*pend.pop(0))

        def pacer(tau):
            ph, q = tau // 16, tau % 16
            mv = ms[ph][q * 8:q * 8 + 8, :]
            return lambda v: jnp.where(fmask, mv, v)

        while pend:
            jj, zz = pend.pop(0)
            col_feed(jj, zz, (lambda q: pacer(16 * 24 + CP0[bi] + CPS[bi] * q)) if jj == 4 else None)

        par = n % 2
        sc = scs[par, 0]
        sh = scs[par, 1]
        nu2 = jnp.where(n == NCH - 1, nu + 1, nu)
        kn2 = jnp.minimum(nu2 + 1, 4 * NU - 1) // NU
        n2 = (n + 1) % NCH
        if extra == 'w':
            items = [('w%d' % part, q) for q in range(16) for part in (1, 0, 3, 5)]
            wc = nu - 1 + n // 2
            wr = pl.multiple_of((n % 2) * 128, 128)
        elif extra == 'x':
            items = [('x', q) for q in range(RU)]
            xsrc = jnp.minimum(nu // 2 + 1, 3)
            xdst = jnp.where(nu == 6, 4, xsrc)
            xs1 = [zero8] * 2
            xs2 = [zero8] * 2
            xpiv = [None, None]
        else:
            items = []
        for it, tau in _schedule(items, k, bi):
            z = pacer(tau)
            if tau < FREE:
                z = lambda v: jnp.where(fmask, anchor, v)
            if it[0] == 'f':
                fsc, fsh = finalize(kn2, n2, z)
                scs[1 - par, 0] = fsc
                scs[1 - par, 1] = fsh
            elif it[0] == 'r':
                s = it[1]
                w_row(kn, un, n, s, z(sc), sh, s == 0 or s == NS - 1)
            elif it[0] == 'h':
                h_tile(Un, n, it[1], it[2], z if PACEH else None)
            elif it[0][0] == 'w':
                w_part(1, 1, wc, (wr + it[1] * 8) if WHINT else pl.multiple_of(wr + it[1] * 8, 8), int(it[0][1]), z)
            else:
                uu, r0 = it[1] // (RU // 2), (it[1] % (RU // 2)) * 2
                if xpiv[uu] is None:
                    xpiv[uu] = jnp.broadcast_to(_unpack(S[xsrc, n, uu * RU, pl.ds(0, 8), :])[0][0:1, :], (8, 128))
                    xs1 = [zero8] * 2
                    xs2 = [zero8] * 2
                pv = z(xpiv[uu])
                vals = []
                for r in range(2):
                    for q in range(4):
                        vals += list(_unpack(S[xsrc, n, uu * RU + r0 + r, pl.ds(q * 8, 8), :]))
                acc_stats(vals, pv, xs1, xs2)
                if r0 == RU - 2:
                    put_stats(xdst, n, uu, xpiv[uu], xs1, xs2)

        for p in range(2):
            for a in (1, 2, 0, 3):
                for t in range(T):
                    for hh in range(2):
                        row, dst = where(a, t, hh, p)
                        S[(2 + b) if k == 0 else b, n, row, dst, :] = pltpu.pack_elementwise(
                            [fin[a][2 * p][2 * t + hh], fin[a][2 * p + 1][2 * t + hh]], packed_dtype=BF16)
        if k == 1:
            out_copy(b, u, n).start()

    def emb_rows():
        te = temb_ref[...].astype(F32)
        th = 0.5 * te
        sil = th + th * jnp.tanh(th)
        return jnp.dot(sil.astype(BF16), wembs[...], preferred_element_type=F32)

    def pro(c, _):
        x_copy(0, c).wait()
        if 's' not in SKIP:
            x_stats_rolled(0, c)
        if 'u' not in SKIP:
            produce_rolled(UA, c)
        return 0
    lax.fori_loop(0, NCH, pro, 0)
    start_rest(1)
    scs[0, 0] = scp[0, 0]
    scs[0, 1] = scp[0, 1]
    def wpro(q, _):
        c = q // NP
        h = q % NP
        pltpu.make_async_copy(w1_hbm.at[:, pl.ds(0, C // NP), pl.ds(0, 128)],
                              wraw.bitcast(BF16).at[0, c, :, pl.ds(pl.multiple_of(h * (C // NP), C // NP), C // NP)],
                              sems.at[NSEM + q]).wait()

        def body(rb, _):
            for q2 in range(WR):
                w_block(0, c, pl.multiple_of(h * (C // 2 // NP) + (rb * WR + q2) * 8, 8))
            return 0
        lax.fori_loop(0, C // 16 // NP // WR, body, 0)
        return 0
    if 2 in DM:
        lax.fori_loop(0, NCH * NP // 2, wpro, 0)
        start_rest(2)
        lax.fori_loop(NCH * NP // 2, NCH * NP, wpro, 0)
    else:
        lax.fori_loop(0, NCH * NP, wpro, 0)
    start_rest(3)

    def emb_block():
        wemb_copy().wait()
        emb = emb_rows()
        for bb in range(B):
            for c in range(NCH):
                off[2 + bb, c] = jnp.broadcast_to(emb[bb:bb + 1, c * 128:(c + 1) * 128], (8, 128))

    def pair(k):
        def f(p, _):
            nu = 2 * p

            ua = UNRS[0] if k == 0 else UNRS[2]
            ub = UNRS[1] if k == 0 else UNRS[3]

            def fa(n2, _):
                for h in range(ua):
                    if k == 0 and 'x' not in SKIP:
                        @pl.when(p == 0)
                        def _():
                            x_copy(1, n2 * ua + h).wait()
                    conv_body(k, nu, n2 * ua + h, UA, UB, 'x', h)
                return 0

            def fb(n2, _):
                for h in range(ub):
                    conv_body(k, nu + 1, n2 * ub + h, UB, UA, 'w' if k == 0 else None, h)
                return 0
            if k == 0:
                @pl.when(p == 1)
                def _():
                    emb_block()
            lax.fori_loop(0, NCH // ua, fa, 0)
            if k == 0:
                @pl.when(p == 0)
                def _():
                    if 'x' in SKIP:
                        for c in range(NCH):
                            x_copy(1, c).wait()
                    w_copy(1, 0).wait()
                    w_copy(1, 1).wait()

                @pl.when(p == 1)
                def _():
                    w_copy(1, 2).wait()
                    w_copy(1, 3).wait()
            lax.fori_loop(0, NCH // ub, fb, 0)
            return 0
        return f
    if STOP == 'pro0':
        return
    if STOP == 'pro':
        for c in range(NCH):
            x_copy(1, c).wait()
            w_copy(1, c).wait()
        wemb_copy().wait()
        return
    lax.fori_loop(0, NU, pair(0), 0)
    if STOP == 'c1':
        return
    def rep(_, __):
        lax.fori_loop(NU, 2 * NU, pair(1), 0)
        for b in range(B):
            for u in range(NU):
                for c in range(NCH):
                    out_copy(b, u, c).wait()
        return 0
    if REP > 1:
        lax.fori_loop(0, REP, rep, 0)
    else:
        rep(0, 0)


@jax.jit
def pallas_standalone__adm_resblock__diffusion_kernel(x, t_emb, g1, be1, w1, w_emb, g2, be2, w2):
    xn = jnp.transpose(x, (0, 2, 3, 1))
    w1n = jnp.transpose(w1, (2, 3, 0, 1)).reshape(9, C, C)
    w2n = jnp.transpose(w2, (2, 3, 0, 1)).reshape(9, C, C)
    vm = pl.BlockSpec(memory_space=pltpu.VMEM)
    hbm = pl.BlockSpec(memory_space=pl.ANY)
    out = pl.pallas_call(
        _kernel,
        out_shape=jax.ShapeDtypeStruct((B, H, W, C), BF16),
        in_specs=[hbm] * 9,
        out_specs=hbm,
        scratch_shapes=[
            pltpu.VMEM((ZP * 8, 128), U32),
            pltpu.VMEM((4, NCH, H, WT, 128), U32),
            pltpu.VMEM((2, NCH, 9, C // 2, 128), U32),
            pltpu.VMEM((36, NCH, C // 2 + WPAD, 128), U32),
            pltpu.VMEM((36, NCH, C // 2 + WPAD, 128), U32),
            pltpu.VMEM((E, C), BF16),
            pltpu.VMEM((NS, 12 + PPAD, 8, 128), F32),
            pltpu.VMEM((36, NCH, M + UPAD, 128), BF16),
            pltpu.VMEM((36, NCH, M + UPAD, 128), BF16),
            pltpu.VMEM((5, NCH, NU, 3, 8, 128), F32),
            pltpu.VMEM((4, NCH, 8, 128), F32),
            pltpu.VMEM((4, NCH, 8, 128), F32),
            pltpu.VMEM((2, 2, 8, 128), F32),
            pltpu.VMEM((NCH, 2, 8, 128), F32),
            pltpu.VMEM((B, E), BF16),
            pltpu.VMEM((C,), BF16),
            pltpu.VMEM((C,), BF16),
            pltpu.VMEM((C,), BF16),
            pltpu.VMEM((C,), BF16),
            pltpu.SemaphoreType.DMA((NSEM + NCH * NP + 5,)),
        ],
        compiler_params=pltpu.CompilerParams(vmem_limit_bytes=110 * 1024 * 1024),
    )(xn, t_emb, g1, be1, w1n, w_emb, g2, be2, w2n)
    return jnp.transpose(out, (0, 3, 1, 2))
```

```python
import jax
import jax.numpy as jnp
from jax import lax
from jax.experimental import pallas as pl
from jax.experimental.pallas import tpu as pltpu

B, C, H, W, E = 2, 512, 64, 64, 1152
EPS = 1e-5
NCH = C // 128
WT = W // 2
T = 8
RU = 4 * T
NS = RU + 2
NU = H // RU
M = T * 16
ORD = (1, 2, 3, 4, 0, 5)

F32 = jnp.float32
BF16 = jnp.bfloat16
U32 = jnp.uint32

PA_ = 0.65
PB_ = 1.0 / PA_
A2, B2 = PA_ * PA_, PB_ * PB_
A3, B3 = A2 * PA_, B2 * PB_
C1 = 1.0 / (2.0 * A2 * (A2 - B2))
C2 = 1.0 / (2.0 * B2 * (B2 - A2))

ENDA = [28.5, 28.5, 29.0, 29.0, 29.0, 28.5, 29.5, 29.5]
ENDB = [35.6, 35.6, 35.9, 35.9, 35.9, 35.3, 35.9, 35.0]
HLAG = [1, 4, 2, 2, 2, 2, 2, 6]
HPRI = [6.0, 6.0, 3.0, 3.0, 3.0, 3.0, 3.0, 3.0]
WAHEAD = [4.0, 4.0, 4.0, 4.0, 4.0, 2.0, 4.0, 4.0]
FILL = [347.0, 347.0, 360.0, 360.0, 360.0, 360.0, 360.0, 363.0]
NACC = 2
STOP = ''
DM = [0, 0]
REP = 1
HPQ = [2, 3]
FREE = 0
FTAU = [180, 180, 200, 200, 180, 180, 150, 260]
SKIP = ''
WPAD = 8
UPAD = 16
PPAD = 1
XR = 8
RR = 33
TR = 8
WR = 8
NP = 1
NSEM = 17 + B * NU * NCH
WHINT = 1
UNRS = [1, 2, 2, 2]
CP0 = [0, 0, 0, 0, 0, -1, 4, 4]
CPS = [12, 12, 12, 12, 12, 12, 12, 12]
ZP = 3
PACEH = 1


WORDS = [(1, 0, 3, 5), (1, 3, 0, 5), (0, 1, 5, 3), (1, 0, 5, 3), (0, 5, 1, 3), (3, 0, 1, 5), (0, 1, 3, 5), (1, 5, 3, 0)]
WORD = [0, 0, 0, 0, 0, 0, 0, 0]
HPQS = [(2, 3), (0, 5), (1, 4), (2,), (3,), (1, 2), (3, 4), (0, 2, 4)]
HPK = [0, 0, 0, 0, 0, 0, 0, 0]
CR = [110.0, 110.0, 110.0, 110.0, 110.0, 130.0, 110.0, 110.0]
CH = [44.0, 44.0, 44.0, 44.0, 44.0, 44.0, 44.0, 44.0]
CX = [1.0, 1.0, 1.0, 1.0, 1.0, 1.0, 1.0, 1.0]


def _schedule(extra=(), k=0, bi=0):
    COST = {'r': CR[bi], 'h': CH[bi], 'w0': 36.0 * CX[bi], 'w5': 36.0 * CX[bi], 'w1': 116.0 * CX[bi], 'w3': 116.0 * CX[bi], 'x': 81.0 * CX[bi]}
    base = [48.0] * 36
    for g, j in enumerate(ORD):
        p = 6 * g
        base[p + 1] += 32
        base[p + 3] += 160
        base[p + 4] += 16
        base[p + 5] += 16
        fin = 16 * (0 if k == 0 else 2) * 4
        w = {1: 0, 2: 128, 3: 0, 4: 640 + 2 * fin, 0: 64 + fin + 64, 5: 64 + fin + 64}[j]
        if j == 4 and CP0[bi] >= 0:
            for q in range(4):
                t0 = 16 * 24 + CP0[bi] + CPS[bi] * q
                for tt in range(t0, t0 + 16):
                    base[min(tt // 16, 35)] += w / 64.0
        elif p + 6 < 36:
            base[p + 4] += w * 0.25
            base[p + 5] += w * 0.5
            base[p + 6] += w * 0.25
        else:
            base[p + 4] += w * 0.5
            base[p + 5] += w * 0.5
    nA = int(ENDA[bi] * 16)
    nB = int(ENDB[bi] * 16)
    cap = [max(FILL[bi] - base[t // 16], 24.0) / 16.0 for t in range(36 * 16)]
    A = [('r', s) for s in range(NS)]
    xs = [it for it in extra if it[0] == 'x']
    ws = [it for it in extra if it[0] != 'x']
    if xs:
        mer = []
        ne = 0
        for q, it in enumerate(A):
            mer.append(it)
            while ne < len(xs) and (ne + 0.5) / len(xs) <= (q + 1.0) / len(A):
                mer.append(xs[ne])
                ne += 1
        A = mer + xs[ne:]
    hs = [('h', t, j) for t in range(T) for j in range(6)]

    def sim(lam):
        out = []
        credit = 0.0
        totA = sum(COST[i[0]] for i in A)
        capA = sum(cap[:nA])
        ia = ih = iw = 0
        accA = 0.0
        cumcap = 0.0
        rowrel = {}
        for t in range(nB):
            cumcap += cap[t]
            credit += lam * cap[t]
            while ia < len(A) and (t >= nA - 1 or accA <= totA * cumcap / capA * (nA - 1.0) / nA):
                it = A[ia]
                out.append((it, t))
                accA += COST[it[0]]
                credit -= COST[it[0]]
                if it[0] == 'r':
                    rowrel[it[1]] = t
                ia += 1
            while credit > 0:
                it = None
                hok = ih < len(hs) and (4 * hs[ih][1] + 5) in rowrel and rowrel[4 * hs[ih][1] + 5] + HLAG[bi] <= t
                wok = iw < len(ws)
                if hok and wok:
                    it = hs[ih] if ih * len(ws) <= iw * len(hs) + HPRI[bi] * len(ws) else ws[iw]
                elif hok:
                    it = hs[ih]
                elif wok and iw * len(hs) <= (ih + WAHEAD[bi]) * len(ws):
                    it = ws[iw]
                if it is None:
                    break
                if it[0] == 'h':
                    ih += 1
                else:
                    iw += 1
                out.append((it, t))
                credit -= COST[it[0]]
            credit = min(credit, 60.0)
        return out, (ih == len(hs) and iw == len(ws) and ia == len(A))
    lo, hi = 0.05, 4.0
    for _ in range(30):
        mid = 0.5 * (lo + hi)
        if sim(mid)[1]:
            hi = mid
        else:
            lo = mid
    out, ok = sim(hi)
    assert ok
    q = 0
    while out[q][1] < FTAU[bi]:
        q += 1
    out.insert(q, (('f',), FTAU[bi]))
    return out


def _sl(hh, p):
    return pl.ds(16 * hh + p, 8, stride=2)


def _unpack(w):
    e = pltpu.unpack_elementwise(w, index=0, packed_dtype=BF16, unpacked_dtype=F32)
    o = pltpu.unpack_elementwise(w, index=1, packed_dtype=BF16, unpacked_dtype=F32)
    return e, o


def _bt6(d):
    d0, d1, d2, d3, d4, d5 = d
    p = A2 * d2
    q = B2 * d2
    ea = d4 - q
    eb = d4 - p
    e0 = (ea - p) + d0
    p3 = A2 * d3
    q3 = B2 * d3
    wa = p3 - d1
    wb = q3 - d1
    oi = (d5 - wa) - q3
    ta = PB_ * wa
    tb = PA_ * wb
    return [e0, ea + ta, ea - ta, eb + tb, eb - tb, oi]


def _g6(g0, g1, g2, c1=C1, c2=C2):
    ea = c1 * g0 + (C1 * A2) * g2
    oa = (C1 * PA_) * g1
    eb = c2 * g0 + (C2 * B2) * g2
    ob = (C2 * PB_) * g1
    return [g0, ea + oa, ea - oa, eb + ob, eb - ob, g2]


class _AT:
    def __init__(self):
        self.v = {}
        self.z = [None] * 4

    def feed(self, i, m):
        v = self.v
        if i in (1, 3):
            v[i] = m
        elif i == 2:
            v['sa'] = v[1] + m
            v['da'] = v[1] - m
        elif i == 4:
            sb = v[3] + m
            db = v[3] - m
            v['p0'] = v['sa'] + sb
            self.z[1] = PA_ * v['da'] + PB_ * db
            self.z[2] = A2 * v['sa'] + B2 * sb
            v['p3'] = A3 * v['da'] + B3 * db
        elif i == 0:
            self.z[0] = v['p0'] + m
        else:
            self.z[3] = v['p3'] + m


def _kernel(x_hbm, temb_hbm, g1_hbm, be1_hbm, w1_hbm, wemb_hbm, g2_hbm, be2_hbm, w2_hbm,
            out_hbm,
            zs, S, wraw, wt1, wt2, wembs, Wp, UA, UB, st, gb, off, scs, scp, temb_ref, g1_ref, be1_ref, g2_ref, be2_ref, sems):
    wt = (wt1, wt2)

    def x_copy(b, c):
        return pltpu.make_async_copy(
            x_hbm.at[b, :, :, pl.ds(pl.multiple_of(c * 128, 128), 128)], S.bitcast(BF16).at[b, c],
            sems.at[b * NCH + c])

    def w_copy(k, c):
        src = w1_hbm if k == 0 else w2_hbm
        return pltpu.make_async_copy(src.at[:, :, pl.ds(c * 128, 128)], wraw.bitcast(BF16).at[k, c],
                                     sems.at[8 + k * NCH + c])

    def w1_piece(c, h):
        return pltpu.make_async_copy(w1_hbm.at[:, pl.ds(h * (C // NP), C // NP), pl.ds(c * 128, 128)],
                                     wraw.bitcast(BF16).at[0, c, :, pl.ds(h * (C // NP), C // NP)],
                                     sems.at[NSEM + c * NP + h])

    def wemb_copy():
        return pltpu.make_async_copy(wemb_hbm, wembs, sems.at[16])

    def out_copy(b, u, c):
        r0 = pl.multiple_of(u * RU, RU)
        return pltpu.make_async_copy(
            S.bitcast(BF16).at[b, c, pl.ds(r0, RU)],
            out_hbm.at[b, pl.ds(r0, RU), :, pl.ds(pl.multiple_of(c * 128, 128), 128)],
            sems.at[17 + (b * NU + u) * NCH + c])

    x_copy(0, 0).start()
    small = [pltpu.make_async_copy(src, dst, sems.at[NSEM + NCH * NP + q]) for q, (src, dst) in enumerate(
        ((g1_hbm, g1_ref), (be1_hbm, be1_ref), (g2_hbm, g2_ref), (be2_hbm, be2_ref), (temb_hbm, temb_ref)))]
    for cp in small:
        cp.start()
    for c in range(1, NCH):
        x_copy(0, c).start()
    for c in range(NCH):
        for h in range(NP):
            w1_piece(c, h).start()
    def start_rest(stage):
        if STOP == 'pro0':
            return
        if stage == DM[0]:
            for c in range(NCH):
                x_copy(1, c).start()
        if stage == DM[1]:
            for c in range(NCH):
                w_copy(1, c).start()
            wemb_copy().start()

    start_rest(0)
    for cp in small:
        cp.wait()
    zero8 = jnp.zeros((8, 128), F32)
    zs[pl.ds(0, 8), :] = jnp.zeros((8, 128), U32)
    for c in range(NCH):
        sl = pl.ds(c * 128, 128)
        for q, r in enumerate((g1_ref, be1_ref, g2_ref, be2_ref)):
            gb[q, c] = jnp.broadcast_to(r[sl].astype(F32).reshape(1, 128), (8, 128))
        off[0, c] = zero8
        off[1, c] = zero8
    sub = lax.broadcasted_iota(jnp.int32, (8, 128), 0)

    def acc_stats(vals, piv, s1, s2):
        for q, v in enumerate(vals):
            d = v - piv
            k_ = q % len(s1)
            s1[k_] = s1[k_] + d
            s2[k_] = s2[k_] + d * d

    def put_stats(slot, c, u, piv, s1, s2):
        t1 = s1[0]
        t2 = s2[0]
        for q in range(1, len(s1)):
            t1 = t1 + s1[q]
            t2 = t2 + s2[q]
        st[slot, c, u, 0] = piv
        st[slot, c, u, 1] = t1
        st[slot, c, u, 2] = t2

    def x_stats_rolled(b, c):
        for u in range(NU):
            w0 = S[b, c, u * RU, pl.ds(0, 8), :]
            piv = jnp.broadcast_to(_unpack(w0)[0][0:1, :], (8, 128))

            def body(r, carry):
                s1 = list(carry[0])
                s2 = list(carry[1])
                vals = []
                for rr in range(XR):
                    for q in range(4):
                        vals += list(_unpack(S[b, c, u * RU + r * XR + rr, pl.ds(q * 8, 8), :]))
                acc_stats(vals, piv, s1, s2)
                return tuple(s1), tuple(s2)
            if XR == RU:
                s1, s2 = body(0, ((zero8,) * 4, (zero8,) * 4))
            else:
                s1, s2 = lax.fori_loop(0, RU // XR, body, ((zero8,) * 4, (zero8,) * 4))
            put_stats(b, c, u, piv, list(s1), list(s2))

    def finalize(kn, c, z=None):
        n = float(RU * W)
        kg = (kn // 2) * 2
        gam = gb[kg, c]
        bet = gb[kg + 1, c]
        of = off[kn, c]
        means = []
        m2s = []
        for u in range(NU):
            piv = st[kn, c, u, 0]
            t1 = st[kn, c, u, 1]
            t2 = st[kn, c, u, 2]
            if z is not None:
                t1 = z(t1)
                t2 = z(t2)
            s1 = jnp.sum(t1, axis=0, keepdims=True)
            s2 = jnp.sum(t2, axis=0, keepdims=True)
            means.append(piv[0:1] + s1 * (1.0 / n) + of[0:1])
            m2s.append(s2 - s1 * s1 * (1.0 / n))
        tot = means[0]
        for u in range(1, NU):
            tot = tot + means[u]
        gmean = jnp.sum(tot, axis=1, keepdims=True) * (1.0 / (NU * 128))
        acc = jnp.zeros((1, 128), F32)
        for u in range(NU):
            dm = means[u] - gmean
            acc = acc + m2s[u] + n * dm * dm
        var = jnp.sum(acc, axis=1, keepdims=True) * (1.0 / (NU * 128 * n))
        rstd = lax.rsqrt(var + EPS)
        sc = 0.5 * gam * rstd
        sh = 0.5 * bet + (of - gmean) * sc
        return sc, sh

    def w_row(kn, un, c, s, sc, sh, edge):
        h = un * RU - 1 + s
        if edge:
            valid = jnp.logical_and(h >= 0, h < H)
            h = jnp.clip(h, 0, H - 1)
        col = [[None] * 4 for _ in range(2)]
        for hh in range(2):
            for p in range(2):
                w = S[kn, c, h, _sl(hh, p), :]
                for e, v in enumerate(_unpack(w)):
                    uu = v * sc + sh
                    a = uu + uu * jnp.tanh(uu)
                    if edge:
                        a = jnp.where(valid, a, 0.0)
                    col[hh][2 * p + e] = a
        r0 = pltpu.roll(col[0][3], 1, 0)
        r1 = pltpu.roll(col[1][3], 1, 0)
        d0 = [jnp.where(sub == 0, 0.0, r0), jnp.where(sub == 0, r0, r1)]
        l0 = pltpu.roll(col[0][0], 7, 0)
        l1 = pltpu.roll(col[1][0], 7, 0)
        d5 = [jnp.where(sub == 7, l1, l0), jnp.where(sub == 7, 0.0, l1)]
        for hh in range(2):
            r = _bt6([d0[hh]] + col[hh] + [d5[hh]])
            for j in range(6):
                Wp[s, 2 * j + hh] = r[j]

    def h_tile(Ud, c, t, j, z=None, hpq=()):
        r = []
        for hh in range(2):
            d = [Wp[4 * t + q, 2 * j + hh] for q in range(6)]
            if z is not None:
                for q in hpq:
                    d[q] = z(d[q])
            r.append(_bt6(d))
        r0 = t * 16 if isinstance(t, int) else pl.multiple_of(t * 16, 16)
        for i in range(6):
            Ud[i * 6 + j, c, pl.ds(r0, 16), :] = jnp.concatenate([r[0][i], r[1][i]], axis=0).astype(BF16)

    def produce_rolled(Ud, c):
        sc, sh = finalize(0, c)
        scp[c, 0] = sc
        scp[c, 1] = sh
        for q in range(12):
            Wp[0, q] = zero8

        def rbody(s, _):
            for rr in range(RR):
                w_row(0, 0, c, 1 + s * RR + rr, sc, sh, False)
            return 0
        if RR == NS - 1:
            rbody(0, 0)
        else:
            lax.fori_loop(0, (NS - 1) // RR, rbody, 0)

        def tbody(t, _):
            for tt in range(TR):
                for j in range(6):
                    h_tile(Ud, c, t * TR + tt, j)
            return 0
        if TR == T:
            tbody(0, 0)
        else:
            lax.fori_loop(0, T // TR, tbody, 0)

    def w_part(ksrc, kdst, c, r0, part, z=None):
        def tap(kh, kw):
            return wraw[ksrc, c, kh * 3 + kw, pl.ds(r0, 8), :]

        def cst(v):
            return v if z is None else z(jnp.full((8, 128), v, F32))
        if part in (0, 5):
            j = part
            w = [tap(kh, 0 if part == 0 else 2) for kh in range(3)]
            g = [_unpack(w[kh]) for kh in range(3)]
            c1, c2 = cst(C1), cst(C2)
            r = [_g6(g[0][h], g[1][h], g[2][h], c1, c2) for h in range(2)]
            wt[kdst][j, c, pl.ds(r0, 8), :] = w[0]
            wt[kdst][30 + j, c, pl.ds(r0, 8), :] = w[2]
            for i in range(1, 5):
                wt[kdst][i * 6 + j, c, pl.ds(r0, 8), :] = pltpu.pack_elementwise(
                    [r[0][i], r[1][i]], packed_dtype=BF16)
            return
        cc, pp = (C1, PA_) if part == 1 else (C2, PB_)
        ccv = cst(cc)
        tp = [[None] * 3 for _ in range(2)]
        tm = [[None] * 3 for _ in range(2)]
        for kh in range(3):
            g = [_unpack(tap(kh, kw)) for kw in range(3)]
            for h in range(2):
                e = ccv * g[0][h] + (cc * pp * pp) * g[2][h]
                o = (cc * pp) * g[1][h]
                tp[h][kh] = e + o
                tm[h][kh] = e - o
        for j, t in ((part, tp), (part + 1, tm)):
            r = [_g6(*t[h]) for h in range(2)]
            for i in range(6):
                wt[kdst][i * 6 + j, c, pl.ds(r0, 8), :] = pltpu.pack_elementwise(
                    [r[0][i], r[1][i]], packed_dtype=BF16)

    def w_block(k, c, r0):
        w = [[wraw[k, c, kh * 3 + kw, pl.ds(r0, 8), :] for kw in range(3)] for kh in range(3)]
        g = [[_unpack(w[kh][kw]) for kw in range(3)] for kh in range(3)]
        res = []
        for h in range(2):
            t = [_g6(g[kh][0][h], g[kh][1][h], g[kh][2][h]) for kh in range(3)]
            res.append([_g6(t[0][j], t[1][j], t[2][j]) for j in range(6)])
        for j in range(6):
            for i in range(6):
                if i in (0, 5) and j in (0, 5):
                    v = w[0 if i == 0 else 2][0 if j == 0 else 2]
                else:
                    v = pltpu.pack_elementwise([res[0][j][i], res[1][j][i]], packed_dtype=BF16)
                wt[k][i * 6 + j, c, pl.ds(r0, 8), :] = v

    def w_transform(k, c):
        def body(rb, _):
            w_block(k, c, pl.multiple_of(rb * 8, 8))
            return 0
        lax.fori_loop(0, C // 16, body, 0, unroll=2)

    def conv_body(k, nu, n, Uc, Un, extra, half=0):
        b = (nu // NU) % B
        u = nu % NU
        nn = jnp.minimum(nu + 1, 4 * NU - 1)
        kn = nn // NU
        un = nn % NU
        fmask = zs[pl.ds(0, 8), :] != 0
        n64 = pl.multiple_of(n * 64, 64)

        ms = []
        col = [_AT() for _ in range(4)]
        fin = [[None] * 4 for _ in range(4)]

        def where(a, t, hh, p):
            return u * RU + 4 * t + a, _sl(hh, p)

        def finish(a, bc):
            y = col[a].z[bc]
            vs = []
            for t in range(T):
                for hh in range(2):
                    q = (2 * t + hh) * 8
                    v = y[q:q + 8]
                    if k == 1:
                        row, dst = where(a, t, hh, bc // 2)
                        v = v + pltpu.unpack_elementwise(S[b, n, row, dst, :], index=bc % 2,
                                                         packed_dtype=BF16, unpacked_dtype=F32)
                    vs.append(v)
            fin[a][bc] = vs

        bi = 2 * (2 * k + (0 if extra == 'x' else 1)) + half
        anchor = pltpu.bitcast(wt[k][ORD[0] * 6 + ORD[0], 0, pl.ds(n64, 8), :], F32)
        pend = []

        def col_feed(j, zz, zf=None):
            for q, a in enumerate((1, 2, 0, 3)):
                za = zz[a]
                if zf is not None:
                    z = zf(q)
                    za = jnp.concatenate([z(za[r * 8:r * 8 + 8]) for r in range(M // 8)], axis=0)
                col[a].feed(j, za)
                if j == 4:
                    finish(a, 1)
                    finish(a, 2)
                elif j == 0:
                    finish(a, 0)
                elif j == 5:
                    finish(a, 3)

        for j in ORD:
            at = _AT()
            for i in ORD:
                L = jnp.concatenate(
                    [pltpu.bitcast(Uc.bitcast(U32)[i * 6 + j, c, pl.ds(0, M // 2), :], BF16) for c in range(NCH)], axis=1)
                Wm = jnp.concatenate(
                    [pltpu.bitcast(wt[k][i * 6 + j, c, pl.ds(n64, 64), :], BF16) for c in range(NCH)], axis=1)
                m = lax.dot_general(L, Wm, (((1,), (1,)), ((), ())), preferred_element_type=F32)
                ms.append(m)
                at.feed(i, m)
            pend.append((j, at.z))
            if CP0[bi] < 0 or j in (1, 2, 3):
                col_feed(*pend.pop(0))

        def pacer(tau):
            ph, q = tau // 16, tau % 16
            mv = ms[ph][q * 8:q * 8 + 8, :]
            return lambda v: jnp.where(fmask, mv, v)

        while pend:
            jj, zz = pend.pop(0)
            col_feed(jj, zz, (lambda q: pacer(16 * 24 + CP0[bi] + CPS[bi] * q)) if jj == 4 else None)

        par = n % 2
        sc = scs[par, 0]
        sh = scs[par, 1]
        nu2 = jnp.where(n == NCH - 1, nu + 1, nu)
        kn2 = jnp.minimum(nu2 + 1, 4 * NU - 1) // NU
        n2 = (n + 1) % NCH
        if extra == 'w':
            items = [('w%d' % part, q) for q in range(16) for part in WORDS[WORD[bi]]]
            wc = nu - 1 + n // 2
            wr = pl.multiple_of((n % 2) * 128, 128)
        elif extra == 'x':
            items = [('x', q) for q in range(RU)]
            xsrc = jnp.minimum(nu // 2 + 1, 3)
            xdst = jnp.where(nu == 6, 4, xsrc)
            xs1 = [zero8] * 2
            xs2 = [zero8] * 2
            xpiv = [None, None]
        else:
            items = []
        for it, tau in _schedule(items, k, bi):
            z = pacer(tau)
            if tau < FREE:
                z = lambda v: jnp.where(fmask, anchor, v)
            if it[0] == 'f':
                fsc, fsh = finalize(kn2, n2, z)
                scs[1 - par, 0] = fsc
                scs[1 - par, 1] = fsh
            elif it[0] == 'r':
                s = it[1]
                w_row(kn, un, n, s, z(sc), sh, s == 0 or s == NS - 1)
            elif it[0] == 'h':
                h_tile(Un, n, it[1], it[2], z if PACEH else None, HPQS[HPK[bi]])
            elif it[0][0] == 'w':
                w_part(1, 1, wc, (wr + it[1] * 8) if WHINT else pl.multiple_of(wr + it[1] * 8, 8), int(it[0][1]), z)
            else:
                uu, r0 = it[1] // (RU // 2), (it[1] % (RU // 2)) * 2
                if xpiv[uu] is None:
                    xpiv[uu] = jnp.broadcast_to(_unpack(S[xsrc, n, uu * RU, pl.ds(0, 8), :])[0][0:1, :], (8, 128))
                    xs1 = [zero8] * 2
                    xs2 = [zero8] * 2
                pv = z(xpiv[uu])
                vals = []
                for r in range(2):
                    for q in range(4):
                        vals += list(_unpack(S[xsrc, n, uu * RU + r0 + r, pl.ds(q * 8, 8), :]))
                acc_stats(vals, pv, xs1, xs2)
                if r0 == RU - 2:
                    put_stats(xdst, n, uu, xpiv[uu], xs1, xs2)

        for p in range(2):
            for a in (1, 2, 0, 3):
                for t in range(T):
                    for hh in range(2):
                        row, dst = where(a, t, hh, p)
                        S[(2 + b) if k == 0 else b, n, row, dst, :] = pltpu.pack_elementwise(
                            [fin[a][2 * p][2 * t + hh], fin[a][2 * p + 1][2 * t + hh]], packed_dtype=BF16)
        if k == 1:
            out_copy(b, u, n).start()

    def emb_rows():
        te = temb_ref[...].astype(F32)
        th = 0.5 * te
        sil = th + th * jnp.tanh(th)
        return jnp.dot(sil.astype(BF16), wembs[...], preferred_element_type=F32)

    def pro(c, _):
        x_copy(0, c).wait()
        if 's' not in SKIP:
            x_stats_rolled(0, c)
        if 'u' not in SKIP:
            produce_rolled(UA, c)
        return 0
    lax.fori_loop(0, NCH, pro, 0)
    start_rest(1)
    scs[0, 0] = scp[0, 0]
    scs[0, 1] = scp[0, 1]
    def wpro(q, _):
        c = q // NP
        h = q % NP
        pltpu.make_async_copy(w1_hbm.at[:, pl.ds(0, C // NP), pl.ds(0, 128)],
                              wraw.bitcast(BF16).at[0, c, :, pl.ds(pl.multiple_of(h * (C // NP), C // NP), C // NP)],
                              sems.at[NSEM + q]).wait()

        def body(rb, _):
            for q2 in range(WR):
                w_block(0, c, pl.multiple_of(h * (C // 2 // NP) + (rb * WR + q2) * 8, 8))
            return 0
        lax.fori_loop(0, C // 16 // NP // WR, body, 0)
        return 0
    if 2 in DM:
        lax.fori_loop(0, NCH * NP // 2, wpro, 0)
        start_rest(2)
        lax.fori_loop(NCH * NP // 2, NCH * NP, wpro, 0)
    else:
        lax.fori_loop(0, NCH * NP, wpro, 0)
    start_rest(3)

    def emb_block():
        wemb_copy().wait()
        emb = emb_rows()
        for bb in range(B):
            for c in range(NCH):
                off[2 + bb, c] = jnp.broadcast_to(emb[bb:bb + 1, c * 128:(c + 1) * 128], (8, 128))

    def pair(k):
        def f(p, _):
            nu = 2 * p

            ua = UNRS[0] if k == 0 else UNRS[2]
            ub = UNRS[1] if k == 0 else UNRS[3]

            def fa(n2, _):
                for h in range(ua):
                    if k == 0 and 'x' not in SKIP:
                        @pl.when(p == 0)
                        def _():
                            x_copy(1, n2 * ua + h).wait()
                    conv_body(k, nu, n2 * ua + h, UA, UB, 'x', h)
                return 0

            def fb(n2, _):
                for h in range(ub):
                    conv_body(k, nu + 1, n2 * ub + h, UB, UA, 'w' if k == 0 else None, h)
                return 0
            if k == 0:
                @pl.when(p == 1)
                def _():
                    emb_block()
            lax.fori_loop(0, NCH // ua, fa, 0)
            if k == 0:
                @pl.when(p == 0)
                def _():
                    if 'x' in SKIP:
                        for c in range(NCH):
                            x_copy(1, c).wait()
                    w_copy(1, 0).wait()
                    w_copy(1, 1).wait()

                @pl.when(p == 1)
                def _():
                    w_copy(1, 2).wait()
                    w_copy(1, 3).wait()
            lax.fori_loop(0, NCH // ub, fb, 0)
            return 0
        return f
    if STOP == 'pro0':
        return
    if STOP == 'pro':
        for c in range(NCH):
            x_copy(1, c).wait()
            w_copy(1, c).wait()
        wemb_copy().wait()
        return
    lax.fori_loop(0, NU, pair(0), 0)
    if STOP == 'c1':
        return
    def rep(_, __):
        lax.fori_loop(NU, 2 * NU, pair(1), 0)
        for b in range(B):
            for u in range(NU):
                for c in range(NCH):
                    out_copy(b, u, c).wait()
        return 0
    if REP > 1:
        lax.fori_loop(0, REP, rep, 0)
    else:
        rep(0, 0)


@jax.jit
def pallas_standalone__adm_resblock__diffusion_kernel(x, t_emb, g1, be1, w1, w_emb, g2, be2, w2):
    xn = jnp.transpose(x, (0, 2, 3, 1))
    w1n = jnp.transpose(w1, (2, 3, 0, 1)).reshape(9, C, C)
    w2n = jnp.transpose(w2, (2, 3, 0, 1)).reshape(9, C, C)
    vm = pl.BlockSpec(memory_space=pltpu.VMEM)
    hbm = pl.BlockSpec(memory_space=pl.ANY)
    out = pl.pallas_call(
        _kernel,
        out_shape=jax.ShapeDtypeStruct((B, H, W, C), BF16),
        in_specs=[hbm] * 9,
        out_specs=hbm,
        scratch_shapes=[
            pltpu.VMEM((ZP * 8, 128), U32),
            pltpu.VMEM((4, NCH, H, WT, 128), U32),
            pltpu.VMEM((2, NCH, 9, C // 2, 128), U32),
            pltpu.VMEM((36, NCH, C // 2 + WPAD, 128), U32),
            pltpu.VMEM((36, NCH, C // 2 + WPAD, 128), U32),
            pltpu.VMEM((E, C), BF16),
            pltpu.VMEM((NS, 12 + PPAD, 8, 128), F32),
            pltpu.VMEM((36, NCH, M + UPAD, 128), BF16),
            pltpu.VMEM((36, NCH, M + UPAD, 128), BF16),
            pltpu.VMEM((5, NCH, NU, 3, 8, 128), F32),
            pltpu.VMEM((4, NCH, 8, 128), F32),
            pltpu.VMEM((4, NCH, 8, 128), F32),
            pltpu.VMEM((2, 2, 8, 128), F32),
            pltpu.VMEM((NCH, 2, 8, 128), F32),
            pltpu.VMEM((B, E), BF16),
            pltpu.VMEM((C,), BF16),
            pltpu.VMEM((C,), BF16),
            pltpu.VMEM((C,), BF16),
            pltpu.VMEM((C,), BF16),
            pltpu.SemaphoreType.DMA((NSEM + NCH * NP + 5,)),
        ],
        compiler_params=pltpu.CompilerParams(vmem_limit_bytes=110 * 1024 * 1024),
    )(xn, t_emb, g1, be1, w1n, w_emb, g2, be2, w2n)
    return jnp.transpose(out, (0, 3, 1, 2))
```

```python
import jax
import jax.numpy as jnp
from jax import lax
from jax.experimental import pallas as pl
from jax.experimental.pallas import tpu as pltpu

B, C, H, W, E = 2, 512, 64, 64, 1152
EPS = 1e-5
NCH = C // 128
WT = W // 2
T = 8
RU = 4 * T
NS = RU + 2
NU = H // RU
M = T * 16
ORD = (1, 2, 3, 4, 0, 5)

F32 = jnp.float32
BF16 = jnp.bfloat16
U32 = jnp.uint32

PA_ = 0.65
PB_ = 1.0 / PA_
A2, B2 = PA_ * PA_, PB_ * PB_
A3, B3 = A2 * PA_, B2 * PB_
C1 = 1.0 / (2.0 * A2 * (A2 - B2))
C2 = 1.0 / (2.0 * B2 * (B2 - A2))

ENDA = [28.5, 28.5, 29.0, 29.0, 29.0, 28.5, 29.5, 28.5]
ENDB = [35.6, 35.6, 35.9, 35.9, 35.9, 35.3, 35.9, 35.0]
HLAG = [1, 4, 1, 2, 2, 2, 0, 6]
HPRI = [6.0, 6.0, 3.0, 3.0, 3.0, 3.0, 3.0, 3.0]
WAHEAD = [4.0, 4.0, 4.0, 4.0, 4.0, 2.0, 4.0, 3.0]
FILL = [347.0, 347.0, 360.0, 360.0, 360.0, 360.0, 360.0, 363.0]
NACC = 2
STOP = ''
DM = [0, 0]
REP = 1
HPQ = [2, 3]
FREE = 0
FTAU = [180, 180, 260, 200, 200, 180, 230, 180]
SKIP = ''
WPAD = 8
UPAD = 16
PPAD = 1
XR = 8
RR = 33
TR = 8
WR = 8
NP = 1
NSEM = 17 + B * NU * NCH
WHINT = 1
UNRS = [1, 2, 2, 2]
CP0 = [0, 0, 0, 0, 0, -1, 4, 4]
CPS = [12, 12, 12, 12, 12, 12, 12, 12]
ZP = 3
PACEH = 1


WORDS = [(1, 0, 3, 5), (1, 3, 0, 5), (0, 1, 5, 3), (1, 0, 5, 3), (0, 5, 1, 3), (3, 0, 1, 5), (0, 1, 3, 5), (1, 5, 3, 0)]
WORD = [0, 0, 0, 0, 0, 0, 0, 0]
HPQS = [(2, 3), (0, 5), (1, 4), (2,), (3,), (1, 2), (3, 4), (0, 2, 4)]
HPK = [0, 0, 0, 0, 0, 0, 0, 5]
CR = [110.0, 110.0, 110.0, 110.0, 110.0, 120.0, 105.0, 110.0]
CH = [44.0, 44.0, 44.0, 44.0, 44.0, 47.0, 44.0, 44.0]
CX = [1.0, 1.0, 1.0, 1.0, 1.0, 1.0, 0.9, 1.05]


def _schedule(extra=(), k=0, bi=0):
    COST = {'r': CR[bi], 'h': CH[bi], 'w0': 36.0 * CX[bi], 'w5': 36.0 * CX[bi], 'w1': 116.0 * CX[bi], 'w3': 116.0 * CX[bi], 'x': 81.0 * CX[bi]}
    base = [48.0] * 36
    for g, j in enumerate(ORD):
        p = 6 * g
        base[p + 1] += 32
        base[p + 3] += 160
        base[p + 4] += 16
        base[p + 5] += 16
        fin = 16 * (0 if k == 0 else 2) * 4
        w = {1: 0, 2: 128, 3: 0, 4: 640 + 2 * fin, 0: 64 + fin + 64, 5: 64 + fin + 64}[j]
        if j == 4 and CP0[bi] >= 0:
            for q in range(4):
                t0 = 16 * 24 + CP0[bi] + CPS[bi] * q
                for tt in range(t0, t0 + 16):
                    base[min(tt // 16, 35)] += w / 64.0
        elif p + 6 < 36:
            base[p + 4] += w * 0.25
            base[p + 5] += w * 0.5
            base[p + 6] += w * 0.25
        else:
            base[p + 4] += w * 0.5
            base[p + 5] += w * 0.5
    nA = int(ENDA[bi] * 16)
    nB = int(ENDB[bi] * 16)
    cap = [max(FILL[bi] - base[t // 16], 24.0) / 16.0 for t in range(36 * 16)]
    A = [('r', s) for s in range(NS)]
    xs = [it for it in extra if it[0] == 'x']
    ws = [it for it in extra if it[0] != 'x']
    if xs:
        mer = []
        ne = 0
        for q, it in enumerate(A):
            mer.append(it)
            while ne < len(xs) and (ne + 0.5) / len(xs) <= (q + 1.0) / len(A):
                mer.append(xs[ne])
                ne += 1
        A = mer + xs[ne:]
    hs = [('h', t, j) for t in range(T) for j in range(6)]

    def sim(lam):
        out = []
        credit = 0.0
        totA = sum(COST[i[0]] for i in A)
        capA = sum(cap[:nA])
        ia = ih = iw = 0
        accA = 0.0
        cumcap = 0.0
        rowrel = {}
        for t in range(nB):
            cumcap += cap[t]
            credit += lam * cap[t]
            while ia < len(A) and (t >= nA - 1 or accA <= totA * cumcap / capA * (nA - 1.0) / nA):
                it = A[ia]
                out.append((it, t))
                accA += COST[it[0]]
                credit -= COST[it[0]]
                if it[0] == 'r':
                    rowrel[it[1]] = t
                ia += 1
            while credit > 0:
                it = None
                hok = ih < len(hs) and (4 * hs[ih][1] + 5) in rowrel and rowrel[4 * hs[ih][1] + 5] + HLAG[bi] <= t
                wok = iw < len(ws)
                if hok and wok:
                    it = hs[ih] if ih * len(ws) <= iw * len(hs) + HPRI[bi] * len(ws) else ws[iw]
                elif hok:
                    it = hs[ih]
                elif wok and iw * len(hs) <= (ih + WAHEAD[bi]) * len(ws):
                    it = ws[iw]
                if it is None:
                    break
                if it[0] == 'h':
                    ih += 1
                else:
                    iw += 1
                out.append((it, t))
                credit -= COST[it[0]]
            credit = min(credit, 60.0)
        return out, (ih == len(hs) and iw == len(ws) and ia == len(A))
    lo, hi = 0.05, 4.0
    for _ in range(30):
        mid = 0.5 * (lo + hi)
        if sim(mid)[1]:
            hi = mid
        else:
            lo = mid
    out, ok = sim(hi)
    assert ok
    q = 0
    while out[q][1] < FTAU[bi]:
        q += 1
    out.insert(q, (('f',), FTAU[bi]))
    return out


def _sl(hh, p):
    return pl.ds(16 * hh + p, 8, stride=2)


def _unpack(w):
    e = pltpu.unpack_elementwise(w, index=0, packed_dtype=BF16, unpacked_dtype=F32)
    o = pltpu.unpack_elementwise(w, index=1, packed_dtype=BF16, unpacked_dtype=F32)
    return e, o


def _bt6(d):
    d0, d1, d2, d3, d4, d5 = d
    p = A2 * d2
    q = B2 * d2
    ea = d4 - q
    eb = d4 - p
    e0 = (ea - p) + d0
    p3 = A2 * d3
    q3 = B2 * d3
    wa = p3 - d1
    wb = q3 - d1
    oi = (d5 - wa) - q3
    ta = PB_ * wa
    tb = PA_ * wb
    return [e0, ea + ta, ea - ta, eb + tb, eb - tb, oi]


def _g6(g0, g1, g2, c1=C1, c2=C2):
    ea = c1 * g0 + (C1 * A2) * g2
    oa = (C1 * PA_) * g1
    eb = c2 * g0 + (C2 * B2) * g2
    ob = (C2 * PB_) * g1
    return [g0, ea + oa, ea - oa, eb + ob, eb - ob, g2]


class _AT:
    def __init__(self):
        self.v = {}
        self.z = [None] * 4

    def feed(self, i, m):
        v = self.v
        if i in (1, 3):
            v[i] = m
        elif i == 2:
            v['sa'] = v[1] + m
            v['da'] = v[1] - m
        elif i == 4:
            sb = v[3] + m
            db = v[3] - m
            v['p0'] = v['sa'] + sb
            self.z[1] = PA_ * v['da'] + PB_ * db
            self.z[2] = A2 * v['sa'] + B2 * sb
            v['p3'] = A3 * v['da'] + B3 * db
        elif i == 0:
            self.z[0] = v['p0'] + m
        else:
            self.z[3] = v['p3'] + m


def _kernel(x_hbm, temb_hbm, g1_hbm, be1_hbm, w1_hbm, wemb_hbm, g2_hbm, be2_hbm, w2_hbm,
            out_hbm,
            zs, S, wraw, wt1, wt2, wembs, Wp, UA, UB, st, gb, off, scs, scp, temb_ref, g1_ref, be1_ref, g2_ref, be2_ref, sems):
    wt = (wt1, wt2)

    def x_copy(b, c):
        return pltpu.make_async_copy(
            x_hbm.at[b, :, :, pl.ds(pl.multiple_of(c * 128, 128), 128)], S.bitcast(BF16).at[b, c],
            sems.at[b * NCH + c])

    def w_copy(k, c):
        src = w1_hbm if k == 0 else w2_hbm
        return pltpu.make_async_copy(src.at[:, :, pl.ds(c * 128, 128)], wraw.bitcast(BF16).at[k, c],
                                     sems.at[8 + k * NCH + c])

    def w1_piece(c, h):
        return pltpu.make_async_copy(w1_hbm.at[:, pl.ds(h * (C // NP), C // NP), pl.ds(c * 128, 128)],
                                     wraw.bitcast(BF16).at[0, c, :, pl.ds(h * (C // NP), C // NP)],
                                     sems.at[NSEM + c * NP + h])

    def wemb_copy():
        return pltpu.make_async_copy(wemb_hbm, wembs, sems.at[16])

    def out_copy(b, u, c):
        r0 = pl.multiple_of(u * RU, RU)
        return pltpu.make_async_copy(
            S.bitcast(BF16).at[b, c, pl.ds(r0, RU)],
            out_hbm.at[b, pl.ds(r0, RU), :, pl.ds(pl.multiple_of(c * 128, 128), 128)],
            sems.at[17 + (b * NU + u) * NCH + c])

    x_copy(0, 0).start()
    small = [pltpu.make_async_copy(src, dst, sems.at[NSEM + NCH * NP + q]) for q, (src, dst) in enumerate(
        ((g1_hbm, g1_ref), (be1_hbm, be1_ref), (g2_hbm, g2_ref), (be2_hbm, be2_ref), (temb_hbm, temb_ref)))]
    for cp in small:
        cp.start()
    for c in range(1, NCH):
        x_copy(0, c).start()
    for c in range(NCH):
        for h in range(NP):
            w1_piece(c, h).start()
    def start_rest(stage):
        if STOP == 'pro0':
            return
        if stage == DM[0]:
            for c in range(NCH):
                x_copy(1, c).start()
        if stage == DM[1]:
            for c in range(NCH):
                w_copy(1, c).start()
            wemb_copy().start()

    start_rest(0)
    for cp in small:
        cp.wait()
    zero8 = jnp.zeros((8, 128), F32)
    zs[pl.ds(0, 8), :] = jnp.zeros((8, 128), U32)
    for c in range(NCH):
        sl = pl.ds(c * 128, 128)
        for q, r in enumerate((g1_ref, be1_ref, g2_ref, be2_ref)):
            gb[q, c] = jnp.broadcast_to(r[sl].astype(F32).reshape(1, 128), (8, 128))
        off[0, c] = zero8
        off[1, c] = zero8
    sub = lax.broadcasted_iota(jnp.int32, (8, 128), 0)

    def acc_stats(vals, piv, s1, s2):
        for q, v in enumerate(vals):
            d = v - piv
            k_ = q % len(s1)
            s1[k_] = s1[k_] + d
            s2[k_] = s2[k_] + d * d

    def put_stats(slot, c, u, piv, s1, s2):
        t1 = s1[0]
        t2 = s2[0]
        for q in range(1, len(s1)):
            t1 = t1 + s1[q]
            t2 = t2 + s2[q]
        st[slot, c, u, 0] = piv
        st[slot, c, u, 1] = t1
        st[slot, c, u, 2] = t2

    def x_stats_rolled(b, c):
        for u in range(NU):
            w0 = S[b, c, u * RU, pl.ds(0, 8), :]
            piv = jnp.broadcast_to(_unpack(w0)[0][0:1, :], (8, 128))

            def body(r, carry):
                s1 = list(carry[0])
                s2 = list(carry[1])
                vals = []
                for rr in range(XR):
                    for q in range(4):
                        vals += list(_unpack(S[b, c, u * RU + r * XR + rr, pl.ds(q * 8, 8), :]))
                acc_stats(vals, piv, s1, s2)
                return tuple(s1), tuple(s2)
            if XR == RU:
                s1, s2 = body(0, ((zero8,) * 4, (zero8,) * 4))
            else:
                s1, s2 = lax.fori_loop(0, RU // XR, body, ((zero8,) * 4, (zero8,) * 4))
            put_stats(b, c, u, piv, list(s1), list(s2))

    def finalize(kn, c, z=None):
        n = float(RU * W)
        kg = (kn // 2) * 2
        gam = gb[kg, c]
        bet = gb[kg + 1, c]
        of = off[kn, c]
        means = []
        m2s = []
        for u in range(NU):
            piv = st[kn, c, u, 0]
            t1 = st[kn, c, u, 1]
            t2 = st[kn, c, u, 2]
            if z is not None:
                t1 = z(t1)
                t2 = z(t2)
            s1 = jnp.sum(t1, axis=0, keepdims=True)
            s2 = jnp.sum(t2, axis=0, keepdims=True)
            means.append(piv[0:1] + s1 * (1.0 / n) + of[0:1])
            m2s.append(s2 - s1 * s1 * (1.0 / n))
        tot = means[0]
        for u in range(1, NU):
            tot = tot + means[u]
        gmean = jnp.sum(tot, axis=1, keepdims=True) * (1.0 / (NU * 128))
        acc = jnp.zeros((1, 128), F32)
        for u in range(NU):
            dm = means[u] - gmean
            acc = acc + m2s[u] + n * dm * dm
        var = jnp.sum(acc, axis=1, keepdims=True) * (1.0 / (NU * 128 * n))
        rstd = lax.rsqrt(var + EPS)
        sc = 0.5 * gam * rstd
        sh = 0.5 * bet + (of - gmean) * sc
        return sc, sh

    def w_row(kn, un, c, s, sc, sh, edge):
        h = un * RU - 1 + s
        if edge:
            valid = jnp.logical_and(h >= 0, h < H)
            h = jnp.clip(h, 0, H - 1)
        col = [[None] * 4 for _ in range(2)]
        for hh in range(2):
            for p in range(2):
                w = S[kn, c, h, _sl(hh, p), :]
                for e, v in enumerate(_unpack(w)):
                    uu = v * sc + sh
                    a = uu + uu * jnp.tanh(uu)
                    if edge:
                        a = jnp.where(valid, a, 0.0)
                    col[hh][2 * p + e] = a
        r0 = pltpu.roll(col[0][3], 1, 0)
        r1 = pltpu.roll(col[1][3], 1, 0)
        d0 = [jnp.where(sub == 0, 0.0, r0), jnp.where(sub == 0, r0, r1)]
        l0 = pltpu.roll(col[0][0], 7, 0)
        l1 = pltpu.roll(col[1][0], 7, 0)
        d5 = [jnp.where(sub == 7, l1, l0), jnp.where(sub == 7, 0.0, l1)]
        for hh in range(2):
            r = _bt6([d0[hh]] + col[hh] + [d5[hh]])
            for j in range(6):
                Wp[s, 2 * j + hh] = r[j]

    def h_tile(Ud, c, t, j, z=None, hpq=()):
        r = []
        for hh in range(2):
            d = [Wp[4 * t + q, 2 * j + hh] for q in range(6)]
            if z is not None:
                for q in hpq:
                    d[q] = z(d[q])
            r.append(_bt6(d))
        r0 = t * 16 if isinstance(t, int) else pl.multiple_of(t * 16, 16)
        for i in range(6):
            Ud[i * 6 + j, c, pl.ds(r0, 16), :] = jnp.concatenate([r[0][i], r[1][i]], axis=0).astype(BF16)

    def produce_rolled(Ud, c):
        sc, sh = finalize(0, c)
        scp[c, 0] = sc
        scp[c, 1] = sh
        for q in range(12):
            Wp[0, q] = zero8

        def rbody(s, _):
            for rr in range(RR):
                w_row(0, 0, c, 1 + s * RR + rr, sc, sh, False)
            return 0
        if RR == NS - 1:
            rbody(0, 0)
        else:
            lax.fori_loop(0, (NS - 1) // RR, rbody, 0)

        def tbody(t, _):
            for tt in range(TR):
                for j in range(6):
                    h_tile(Ud, c, t * TR + tt, j)
            return 0
        if TR == T:
            tbody(0, 0)
        else:
            lax.fori_loop(0, T // TR, tbody, 0)

    def w_part(ksrc, kdst, c, r0, part, z=None):
        def tap(kh, kw):
            return wraw[ksrc, c, kh * 3 + kw, pl.ds(r0, 8), :]

        def cst(v):
            return v if z is None else z(jnp.full((8, 128), v, F32))
        if part in (0, 5):
            j = part
            w = [tap(kh, 0 if part == 0 else 2) for kh in range(3)]
            g = [_unpack(w[kh]) for kh in range(3)]
            c1, c2 = cst(C1), cst(C2)
            r = [_g6(g[0][h], g[1][h], g[2][h], c1, c2) for h in range(2)]
            wt[kdst][j, c, pl.ds(r0, 8), :] = w[0]
            wt[kdst][30 + j, c, pl.ds(r0, 8), :] = w[2]
            for i in range(1, 5):
                wt[kdst][i * 6 + j, c, pl.ds(r0, 8), :] = pltpu.pack_elementwise(
                    [r[0][i], r[1][i]], packed_dtype=BF16)
            return
        cc, pp = (C1, PA_) if part == 1 else (C2, PB_)
        ccv = cst(cc)
        tp = [[None] * 3 for _ in range(2)]
        tm = [[None] * 3 for _ in range(2)]
        for kh in range(3):
            g = [_unpack(tap(kh, kw)) for kw in range(3)]
            for h in range(2):
                e = ccv * g[0][h] + (cc * pp * pp) * g[2][h]
                o = (cc * pp) * g[1][h]
                tp[h][kh] = e + o
                tm[h][kh] = e - o
        for j, t in ((part, tp), (part + 1, tm)):
            r = [_g6(*t[h]) for h in range(2)]
            for i in range(6):
                wt[kdst][i * 6 + j, c, pl.ds(r0, 8), :] = pltpu.pack_elementwise(
                    [r[0][i], r[1][i]], packed_dtype=BF16)

    def w_block(k, c, r0):
        w = [[wraw[k, c, kh * 3 + kw, pl.ds(r0, 8), :] for kw in range(3)] for kh in range(3)]
        g = [[_unpack(w[kh][kw]) for kw in range(3)] for kh in range(3)]
        res = []
        for h in range(2):
            t = [_g6(g[kh][0][h], g[kh][1][h], g[kh][2][h]) for kh in range(3)]
            res.append([_g6(t[0][j], t[1][j], t[2][j]) for j in range(6)])
        for j in range(6):
            for i in range(6):
                if i in (0, 5) and j in (0, 5):
                    v = w[0 if i == 0 else 2][0 if j == 0 else 2]
                else:
                    v = pltpu.pack_elementwise([res[0][j][i], res[1][j][i]], packed_dtype=BF16)
                wt[k][i * 6 + j, c, pl.ds(r0, 8), :] = v

    def w_transform(k, c):
        def body(rb, _):
            w_block(k, c, pl.multiple_of(rb * 8, 8))
            return 0
        lax.fori_loop(0, C // 16, body, 0, unroll=2)

    def conv_body(k, nu, n, Uc, Un, extra, half=0):
        b = (nu // NU) % B
        u = nu % NU
        nn = jnp.minimum(nu + 1, 4 * NU - 1)
        kn = nn // NU
        un = nn % NU
        fmask = zs[pl.ds(0, 8), :] != 0
        n64 = pl.multiple_of(n * 64, 64)

        ms = []
        col = [_AT() for _ in range(4)]
        fin = [[None] * 4 for _ in range(4)]

        def where(a, t, hh, p):
            return u * RU + 4 * t + a, _sl(hh, p)

        def finish(a, bc):
            y = col[a].z[bc]
            vs = []
            for t in range(T):
                for hh in range(2):
                    q = (2 * t + hh) * 8
                    v = y[q:q + 8]
                    if k == 1:
                        row, dst = where(a, t, hh, bc // 2)
                        v = v + pltpu.unpack_elementwise(S[b, n, row, dst, :], index=bc % 2,
                                                         packed_dtype=BF16, unpacked_dtype=F32)
                    vs.append(v)
            fin[a][bc] = vs

        bi = 2 * (2 * k + (0 if extra == 'x' else 1)) + half
        anchor = pltpu.bitcast(wt[k][ORD[0] * 6 + ORD[0], 0, pl.ds(n64, 8), :], F32)
        pend = []

        def col_feed(j, zz, zf=None):
            for q, a in enumerate((1, 2, 0, 3)):
                za = zz[a]
                if zf is not None:
                    z = zf(q)
                    za = jnp.concatenate([z(za[r * 8:r * 8 + 8]) for r in range(M // 8)], axis=0)
                col[a].feed(j, za)
                if j == 4:
                    finish(a, 1)
                    finish(a, 2)
                elif j == 0:
                    finish(a, 0)
                elif j == 5:
                    finish(a, 3)

        for j in ORD:
            at = _AT()
            for i in ORD:
                L = jnp.concatenate(
                    [pltpu.bitcast(Uc.bitcast(U32)[i * 6 + j, c, pl.ds(0, M // 2), :], BF16) for c in range(NCH)], axis=1)
                Wm = jnp.concatenate(
                    [pltpu.bitcast(wt[k][i * 6 + j, c, pl.ds(n64, 64), :], BF16) for c in range(NCH)], axis=1)
                m = lax.dot_general(L, Wm, (((1,), (1,)), ((), ())), preferred_element_type=F32)
                ms.append(m)
                at.feed(i, m)
            pend.append((j, at.z))
            if CP0[bi] < 0 or j in (1, 2, 3):
                col_feed(*pend.pop(0))

        def pacer(tau):
            ph, q = tau // 16, tau % 16
            mv = ms[ph][q * 8:q * 8 + 8, :]
            return lambda v: jnp.where(fmask, mv, v)

        while pend:
            jj, zz = pend.pop(0)
            col_feed(jj, zz, (lambda q: pacer(16 * 24 + CP0[bi] + CPS[bi] * q)) if jj == 4 else None)

        par = n % 2
        sc = scs[par, 0]
        sh = scs[par, 1]
        nu2 = jnp.where(n == NCH - 1, nu + 1, nu)
        kn2 = jnp.minimum(nu2 + 1, 4 * NU - 1) // NU
        n2 = (n + 1) % NCH
        if extra == 'w':
            items = [('w%d' % part, q) for q in range(16) for part in WORDS[WORD[bi]]]
            wc = nu - 1 + n // 2
            wr = pl.multiple_of((n % 2) * 128, 128)
        elif extra == 'x':
            items = [('x', q) for q in range(RU)]
            xsrc = jnp.minimum(nu // 2 + 1, 3)
            xdst = jnp.where(nu == 6, 4, xsrc)
            xs1 = [zero8] * 2
            xs2 = [zero8] * 2
            xpiv = [None, None]
        else:
            items = []
        for it, tau in _schedule(items, k, bi):
            z = pacer(tau)
            if tau < FREE:
                z = lambda v: jnp.where(fmask, anchor, v)
            if it[0] == 'f':
                fsc, fsh = finalize(kn2, n2, z)
                scs[1 - par, 0] = fsc
                scs[1 - par, 1] = fsh
            elif it[0] == 'r':
                s = it[1]
                w_row(kn, un, n, s, z(sc), sh, s == 0 or s == NS - 1)
            elif it[0] == 'h':
                h_tile(Un, n, it[1], it[2], z if PACEH else None, HPQS[HPK[bi]])
            elif it[0][0] == 'w':
                w_part(1, 1, wc, (wr + it[1] * 8) if WHINT else pl.multiple_of(wr + it[1] * 8, 8), int(it[0][1]), z)
            else:
                uu, r0 = it[1] // (RU // 2), (it[1] % (RU // 2)) * 2
                if xpiv[uu] is None:
                    xpiv[uu] = jnp.broadcast_to(_unpack(S[xsrc, n, uu * RU, pl.ds(0, 8), :])[0][0:1, :], (8, 128))
                    xs1 = [zero8] * 2
                    xs2 = [zero8] * 2
                pv = z(xpiv[uu])
                vals = []
                for r in range(2):
                    for q in range(4):
                        vals += list(_unpack(S[xsrc, n, uu * RU + r0 + r, pl.ds(q * 8, 8), :]))
                acc_stats(vals, pv, xs1, xs2)
                if r0 == RU - 2:
                    put_stats(xdst, n, uu, xpiv[uu], xs1, xs2)

        for p in range(2):
            for a in (1, 2, 0, 3):
                for t in range(T):
                    for hh in range(2):
                        row, dst = where(a, t, hh, p)
                        S[(2 + b) if k == 0 else b, n, row, dst, :] = pltpu.pack_elementwise(
                            [fin[a][2 * p][2 * t + hh], fin[a][2 * p + 1][2 * t + hh]], packed_dtype=BF16)
        if k == 1:
            out_copy(b, u, n).start()

    def emb_rows():
        te = temb_ref[...].astype(F32)
        th = 0.5 * te
        sil = th + th * jnp.tanh(th)
        return jnp.dot(sil.astype(BF16), wembs[...], preferred_element_type=F32)

    def pro(c, _):
        x_copy(0, c).wait()
        if 's' not in SKIP:
            x_stats_rolled(0, c)
        if 'u' not in SKIP:
            produce_rolled(UA, c)
        return 0
    lax.fori_loop(0, NCH, pro, 0)
    start_rest(1)
    scs[0, 0] = scp[0, 0]
    scs[0, 1] = scp[0, 1]
    def wpro(q, _):
        c = q // NP
        h = q % NP
        pltpu.make_async_copy(w1_hbm.at[:, pl.ds(0, C // NP), pl.ds(0, 128)],
                              wraw.bitcast(BF16).at[0, c, :, pl.ds(pl.multiple_of(h * (C // NP), C // NP), C // NP)],
                              sems.at[NSEM + q]).wait()

        def body(rb, _):
            for q2 in range(WR):
                w_block(0, c, pl.multiple_of(h * (C // 2 // NP) + (rb * WR + q2) * 8, 8))
            return 0
        lax.fori_loop(0, C // 16 // NP // WR, body, 0)
        return 0
    if 2 in DM:
        lax.fori_loop(0, NCH * NP // 2, wpro, 0)
        start_rest(2)
        lax.fori_loop(NCH * NP // 2, NCH * NP, wpro, 0)
    else:
        lax.fori_loop(0, NCH * NP, wpro, 0)
    start_rest(3)

    def emb_block():
        wemb_copy().wait()
        emb = emb_rows()
        for bb in range(B):
            for c in range(NCH):
                off[2 + bb, c] = jnp.broadcast_to(emb[bb:bb + 1, c * 128:(c + 1) * 128], (8, 128))

    def pair(k):
        def f(p, _):
            nu = 2 * p

            ua = UNRS[0] if k == 0 else UNRS[2]
            ub = UNRS[1] if k == 0 else UNRS[3]

            def fa(n2, _):
                for h in range(ua):
                    if k == 0 and 'x' not in SKIP:
                        @pl.when(p == 0)
                        def _():
                            x_copy(1, n2 * ua + h).wait()
                    conv_body(k, nu, n2 * ua + h, UA, UB, 'x', h)
                return 0

            def fb(n2, _):
                for h in range(ub):
                    conv_body(k, nu + 1, n2 * ub + h, UB, UA, 'w' if k == 0 else None, h)
                return 0
            if k == 0:
                @pl.when(p == 1)
                def _():
                    emb_block()
            lax.fori_loop(0, NCH // ua, fa, 0)
            if k == 0:
                @pl.when(p == 0)
                def _():
                    if 'x' in SKIP:
                        for c in range(NCH):
                            x_copy(1, c).wait()
                    w_copy(1, 0).wait()
                    w_copy(1, 1).wait()

                @pl.when(p == 1)
                def _():
                    w_copy(1, 2).wait()
                    w_copy(1, 3).wait()
            lax.fori_loop(0, NCH // ub, fb, 0)
            return 0
        return f
    if STOP == 'pro0':
        return
    if STOP == 'pro':
        for c in range(NCH):
            x_copy(1, c).wait()
            w_copy(1, c).wait()
        wemb_copy().wait()
        return
    lax.fori_loop(0, NU, pair(0), 0)
    if STOP == 'c1':
        return
    def rep(_, __):
        lax.fori_loop(NU, 2 * NU, pair(1), 0)
        for b in range(B):
            for u in range(NU):
                for c in range(NCH):
                    out_copy(b, u, c).wait()
        return 0
    if REP > 1:
        lax.fori_loop(0, REP, rep, 0)
    else:
        rep(0, 0)


@jax.jit
def pallas_standalone__adm_resblock__diffusion_kernel(x, t_emb, g1, be1, w1, w_emb, g2, be2, w2):
    xn = jnp.transpose(x, (0, 2, 3, 1))
    w1n = jnp.transpose(w1, (2, 3, 0, 1)).reshape(9, C, C)
    w2n = jnp.transpose(w2, (2, 3, 0, 1)).reshape(9, C, C)
    vm = pl.BlockSpec(memory_space=pltpu.VMEM)
    hbm = pl.BlockSpec(memory_space=pl.ANY)
    out = pl.pallas_call(
        _kernel,
        out_shape=jax.ShapeDtypeStruct((B, H, W, C), BF16),
        in_specs=[hbm] * 9,
        out_specs=hbm,
        scratch_shapes=[
            pltpu.VMEM((ZP * 8, 128), U32),
            pltpu.VMEM((4, NCH, H, WT, 128), U32),
            pltpu.VMEM((2, NCH, 9, C // 2, 128), U32),
            pltpu.VMEM((36, NCH, C // 2 + WPAD, 128), U32),
            pltpu.VMEM((36, NCH, C // 2 + WPAD, 128), U32),
            pltpu.VMEM((E, C), BF16),
            pltpu.VMEM((NS, 12 + PPAD, 8, 128), F32),
            pltpu.VMEM((36, NCH, M + UPAD, 128), BF16),
            pltpu.VMEM((36, NCH, M + UPAD, 128), BF16),
            pltpu.VMEM((5, NCH, NU, 3, 8, 128), F32),
            pltpu.VMEM((4, NCH, 8, 128), F32),
            pltpu.VMEM((4, NCH, 8, 128), F32),
            pltpu.VMEM((2, 2, 8, 128), F32),
            pltpu.VMEM((NCH, 2, 8, 128), F32),
            pltpu.VMEM((B, E), BF16),
            pltpu.VMEM((C,), BF16),
            pltpu.VMEM((C,), BF16),
            pltpu.VMEM((C,), BF16),
            pltpu.VMEM((C,), BF16),
            pltpu.SemaphoreType.DMA((NSEM + NCH * NP + 5,)),
        ],
        compiler_params=pltpu.CompilerParams(vmem_limit_bytes=110 * 1024 * 1024),
    )(xn, t_emb, g1, be1, w1n, w_emb, g2, be2, w2n)
    return jnp.transpose(out, (0, 3, 1, 2))
```

```python
import jax
import jax.numpy as jnp
from jax import lax
from jax.experimental import pallas as pl
from jax.experimental.pallas import tpu as pltpu

B, C, H, W, E = 2, 512, 64, 64, 1152
EPS = 1e-5
NCH = C // 128
WT = W // 2
T = 8
RU = 4 * T
NS = RU + 2
NU = H // RU
M = T * 16
ORD = (1, 2, 3, 4, 0, 5)

F32 = jnp.float32
BF16 = jnp.bfloat16
U32 = jnp.uint32

PA_ = 0.65
PB_ = 1.0 / PA_
A2, B2 = PA_ * PA_, PB_ * PB_
A3, B3 = A2 * PA_, B2 * PB_
C1 = 1.0 / (2.0 * A2 * (A2 - B2))
C2 = 1.0 / (2.0 * B2 * (B2 - A2))

ENDA = [28.5, 28.5, 29.0, 28.75, 29.0, 28.5, 29.5, 28.5]
ENDB = [35.6, 35.6, 35.9, 35.9, 35.9, 35.3, 35.9, 35.0]
HLAG = [1, 4, 1, 2, 2, 2, 0, 6]
HPRI = [6.0, 6.0, 3.0, 2.0, 3.0, 3.0, 3.0, 3.0]
WAHEAD = [4.0, 4.0, 4.0, 4.0, 4.0, 8.0, 4.0, 3.0]
FILL = [347.0, 347.0, 360.0, 357.0, 360.0, 360.0, 360.0, 366.0]
NACC = 2
STOP = ''
DM = [0, 0]
REP = 1
HPQ = [2, 3]
FREE = 0
FTAU = [180, 180, 260, 200, 200, 180, 180, 200]
SKIP = ''
WPAD = 8
UPAD = 16
PPAD = 1
XR = 8
RR = 33
TR = 8
WR = 8
NP = 1
NSEM = 17 + B * NU * NCH
WHINT = 1
UNRS = [1, 2, 2, 2]
CP0 = [0, 0, 0, 8, 0, -1, 4, 4]
CPS = [12, 12, 12, 12, 12, 12, 10, 12]
ZP = 3
PACEH = 1


WORDS = [(1, 0, 3, 5), (1, 3, 0, 5), (0, 1, 5, 3), (1, 0, 5, 3), (0, 5, 1, 3), (3, 0, 1, 5), (0, 1, 3, 5), (1, 5, 3, 0)]
WORD = [0, 0, 0, 6, 0, 0, 0, 0]
HPQS = [(2, 3), (0, 5), (1, 4), (2,), (3,), (1, 2), (3, 4), (0, 2, 4)]
HPK = [0, 0, 5, 0, 0, 6, 0, 5]
CR = [110.0, 110.0, 110.0, 110.0, 110.0, 120.0, 105.0, 110.0]
CH = [44.0, 44.0, 44.0, 47.0, 44.0, 47.0, 44.0, 44.0]
CX = [1.0, 1.0, 1.0, 1.0, 1.0, 1.0, 0.8, 1.05]


def _schedule(extra=(), k=0, bi=0):
    COST = {'r': CR[bi], 'h': CH[bi], 'w0': 36.0 * CX[bi], 'w5': 36.0 * CX[bi], 'w1': 116.0 * CX[bi], 'w3': 116.0 * CX[bi], 'x': 81.0 * CX[bi]}
    base = [48.0] * 36
    for g, j in enumerate(ORD):
        p = 6 * g
        base[p + 1] += 32
        base[p + 3] += 160
        base[p + 4] += 16
        base[p + 5] += 16
        fin = 16 * (0 if k == 0 else 2) * 4
        w = {1: 0, 2: 128, 3: 0, 4: 640 + 2 * fin, 0: 64 + fin + 64, 5: 64 + fin + 64}[j]
        if j == 4 and CP0[bi] >= 0:
            for q in range(4):
                t0 = 16 * 24 + CP0[bi] + CPS[bi] * q
                for tt in range(t0, t0 + 16):
                    base[min(tt // 16, 35)] += w / 64.0
        elif p + 6 < 36:
            base[p + 4] += w * 0.25
            base[p + 5] += w * 0.5
            base[p + 6] += w * 0.25
        else:
            base[p + 4] += w * 0.5
            base[p + 5] += w * 0.5
    nA = int(ENDA[bi] * 16)
    nB = int(ENDB[bi] * 16)
    cap = [max(FILL[bi] - base[t // 16], 24.0) / 16.0 for t in range(36 * 16)]
    A = [('r', s) for s in range(NS)]
    xs = [it for it in extra if it[0] == 'x']
    ws = [it for it in extra if it[0] != 'x']
    if xs:
        mer = []
        ne = 0
        for q, it in enumerate(A):
            mer.append(it)
            while ne < len(xs) and (ne + 0.5) / len(xs) <= (q + 1.0) / len(A):
                mer.append(xs[ne])
                ne += 1
        A = mer + xs[ne:]
    hs = [('h', t, j) for t in range(T) for j in range(6)]

    def sim(lam):
        out = []
        credit = 0.0
        totA = sum(COST[i[0]] for i in A)
        capA = sum(cap[:nA])
        ia = ih = iw = 0
        accA = 0.0
        cumcap = 0.0
        rowrel = {}
        for t in range(nB):
            cumcap += cap[t]
            credit += lam * cap[t]
            while ia < len(A) and (t >= nA - 1 or accA <= totA * cumcap / capA * (nA - 1.0) / nA):
                it = A[ia]
                out.append((it, t))
                accA += COST[it[0]]
                credit -= COST[it[0]]
                if it[0] == 'r':
                    rowrel[it[1]] = t
                ia += 1
            while credit > 0:
                it = None
                hok = ih < len(hs) and (4 * hs[ih][1] + 5) in rowrel and rowrel[4 * hs[ih][1] + 5] + HLAG[bi] <= t
                wok = iw < len(ws)
                if hok and wok:
                    it = hs[ih] if ih * len(ws) <= iw * len(hs) + HPRI[bi] * len(ws) else ws[iw]
                elif hok:
                    it = hs[ih]
                elif wok and iw * len(hs) <= (ih + WAHEAD[bi]) * len(ws):
                    it = ws[iw]
                if it is None:
                    break
                if it[0] == 'h':
                    ih += 1
                else:
                    iw += 1
                out.append((it, t))
                credit -= COST[it[0]]
            credit = min(credit, 60.0)
        return out, (ih == len(hs) and iw == len(ws) and ia == len(A))
    lo, hi = 0.05, 4.0
    for _ in range(30):
        mid = 0.5 * (lo + hi)
        if sim(mid)[1]:
            hi = mid
        else:
            lo = mid
    out, ok = sim(hi)
    assert ok
    q = 0
    while out[q][1] < FTAU[bi]:
        q += 1
    out.insert(q, (('f',), FTAU[bi]))
    return out


def _sl(hh, p):
    return pl.ds(16 * hh + p, 8, stride=2)


def _unpack(w):
    e = pltpu.unpack_elementwise(w, index=0, packed_dtype=BF16, unpacked_dtype=F32)
    o = pltpu.unpack_elementwise(w, index=1, packed_dtype=BF16, unpacked_dtype=F32)
    return e, o


def _bt6(d):
    d0, d1, d2, d3, d4, d5 = d
    p = A2 * d2
    q = B2 * d2
    ea = d4 - q
    eb = d4 - p
    e0 = (ea - p) + d0
    p3 = A2 * d3
    q3 = B2 * d3
    wa = p3 - d1
    wb = q3 - d1
    oi = (d5 - wa) - q3
    ta = PB_ * wa
    tb = PA_ * wb
    return [e0, ea + ta, ea - ta, eb + tb, eb - tb, oi]


def _g6(g0, g1, g2, c1=C1, c2=C2):
    u = (C1 * A2) * g2
    ea = c1 * g0 + u
    oa = (C1 * PA_) * g1
    eb = c2 * g0 - u
    ob = (C2 * PB_) * g1
    return [g0, ea + oa, ea - oa, eb + ob, eb - ob, g2]


class _AT:
    def __init__(self):
        self.v = {}
        self.z = [None] * 4

    def feed(self, i, m):
        v = self.v
        if i in (1, 3):
            v[i] = m
        elif i == 2:
            v['sa'] = v[1] + m
            v['da'] = v[1] - m
        elif i == 4:
            sb = v[3] + m
            db = v[3] - m
            v['p0'] = v['sa'] + sb
            self.z[1] = PA_ * v['da'] + PB_ * db
            self.z[2] = A2 * v['sa'] + B2 * sb
            v['p3'] = A3 * v['da'] + B3 * db
        elif i == 0:
            self.z[0] = v['p0'] + m
        else:
            self.z[3] = v['p3'] + m


def _kernel(x_hbm, temb_hbm, g1_hbm, be1_hbm, w1_hbm, wemb_hbm, g2_hbm, be2_hbm, w2_hbm,
            out_hbm,
            zs, S, wraw, wt1, wt2, wembs, Wp, UA, UB, st, gb, off, scs, scp, temb_ref, g1_ref, be1_ref, g2_ref, be2_ref, sems):
    wt = (wt1, wt2)

    def x_copy(b, c):
        return pltpu.make_async_copy(
            x_hbm.at[b, :, :, pl.ds(pl.multiple_of(c * 128, 128), 128)], S.bitcast(BF16).at[b, c],
            sems.at[b * NCH + c])

    def w_copy(k, c):
        src = w1_hbm if k == 0 else w2_hbm
        return pltpu.make_async_copy(src.at[:, :, pl.ds(c * 128, 128)], wraw.bitcast(BF16).at[k, c],
                                     sems.at[8 + k * NCH + c])

    def w1_piece(c, h):
        return pltpu.make_async_copy(w1_hbm.at[:, pl.ds(h * (C // NP), C // NP), pl.ds(c * 128, 128)],
                                     wraw.bitcast(BF16).at[0, c, :, pl.ds(h * (C // NP), C // NP)],
                                     sems.at[NSEM + c * NP + h])

    def wemb_copy():
        return pltpu.make_async_copy(wemb_hbm, wembs, sems.at[16])

    def out_copy(b, u, c):
        r0 = pl.multiple_of(u * RU, RU)
        return pltpu.make_async_copy(
            S.bitcast(BF16).at[b, c, pl.ds(r0, RU)],
            out_hbm.at[b, pl.ds(r0, RU), :, pl.ds(pl.multiple_of(c * 128, 128), 128)],
            sems.at[17 + (b * NU + u) * NCH + c])

    x_copy(0, 0).start()
    small = [pltpu.make_async_copy(src, dst, sems.at[NSEM + NCH * NP + q]) for q, (src, dst) in enumerate(
        ((g1_hbm, g1_ref), (be1_hbm, be1_ref), (g2_hbm, g2_ref), (be2_hbm, be2_ref), (temb_hbm, temb_ref)))]
    for cp in small:
        cp.start()
    for c in range(1, NCH):
        x_copy(0, c).start()
    for c in range(NCH):
        for h in range(NP):
            w1_piece(c, h).start()
    def start_rest(stage):
        if STOP == 'pro0':
            return
        if stage == DM[0]:
            for c in range(NCH):
                x_copy(1, c).start()
        if stage == DM[1]:
            for c in range(NCH):
                w_copy(1, c).start()
            wemb_copy().start()

    start_rest(0)
    for cp in small:
        cp.wait()
    zero8 = jnp.zeros((8, 128), F32)
    zs[pl.ds(0, 8), :] = jnp.zeros((8, 128), U32)
    for c in range(NCH):
        sl = pl.ds(c * 128, 128)
        for q, r in enumerate((g1_ref, be1_ref, g2_ref, be2_ref)):
            gb[q, c] = jnp.broadcast_to(r[sl].astype(F32).reshape(1, 128), (8, 128))
        off[0, c] = zero8
        off[1, c] = zero8
    sub = lax.broadcasted_iota(jnp.int32, (8, 128), 0)

    def acc_stats(vals, piv, s1, s2):
        for q, v in enumerate(vals):
            d = v - piv
            k_ = q % len(s1)
            s1[k_] = s1[k_] + d
            s2[k_] = s2[k_] + d * d

    def put_stats(slot, c, u, piv, s1, s2):
        t1 = s1[0]
        t2 = s2[0]
        for q in range(1, len(s1)):
            t1 = t1 + s1[q]
            t2 = t2 + s2[q]
        st[slot, c, u, 0] = piv
        st[slot, c, u, 1] = t1
        st[slot, c, u, 2] = t2

    def x_stats_rolled(b, c):
        for u in range(NU):
            w0 = S[b, c, u * RU, pl.ds(0, 8), :]
            piv = jnp.broadcast_to(_unpack(w0)[0][0:1, :], (8, 128))

            def body(r, carry):
                s1 = list(carry[0])
                s2 = list(carry[1])
                vals = []
                for rr in range(XR):
                    for q in range(4):
                        vals += list(_unpack(S[b, c, u * RU + r * XR + rr, pl.ds(q * 8, 8), :]))
                acc_stats(vals, piv, s1, s2)
                return tuple(s1), tuple(s2)
            if XR == RU:
                s1, s2 = body(0, ((zero8,) * 4, (zero8,) * 4))
            else:
                s1, s2 = lax.fori_loop(0, RU // XR, body, ((zero8,) * 4, (zero8,) * 4))
            put_stats(b, c, u, piv, list(s1), list(s2))

    def finalize(kn, c, z=None):
        n = float(RU * W)
        kg = (kn // 2) * 2
        gam = gb[kg, c]
        bet = gb[kg + 1, c]
        of = off[kn, c]
        means = []
        m2s = []
        for u in range(NU):
            piv = st[kn, c, u, 0]
            t1 = st[kn, c, u, 1]
            t2 = st[kn, c, u, 2]
            if z is not None:
                t1 = z(t1)
                t2 = z(t2)
            s1 = jnp.sum(t1, axis=0, keepdims=True)
            s2 = jnp.sum(t2, axis=0, keepdims=True)
            means.append(piv[0:1] + s1 * (1.0 / n) + of[0:1])
            m2s.append(s2 - s1 * s1 * (1.0 / n))
        tot = means[0]
        for u in range(1, NU):
            tot = tot + means[u]
        gmean = jnp.sum(tot, axis=1, keepdims=True) * (1.0 / (NU * 128))
        acc = jnp.zeros((1, 128), F32)
        for u in range(NU):
            dm = means[u] - gmean
            acc = acc + m2s[u] + n * dm * dm
        var = jnp.sum(acc, axis=1, keepdims=True) * (1.0 / (NU * 128 * n))
        rstd = lax.rsqrt(var + EPS)
        sc = 0.5 * gam * rstd
        sh = 0.5 * bet + (of - gmean) * sc
        return sc, sh

    def w_row(kn, un, c, s, sc, sh, edge):
        h = un * RU - 1 + s
        if edge:
            valid = jnp.logical_and(h >= 0, h < H)
            h = jnp.clip(h, 0, H - 1)
        col = [[None] * 4 for _ in range(2)]
        for hh in range(2):
            for p in range(2):
                w = S[kn, c, h, _sl(hh, p), :]
                for e, v in enumerate(_unpack(w)):
                    uu = v * sc + sh
                    a = uu + uu * jnp.tanh(uu)
                    if edge:
                        a = jnp.where(valid, a, 0.0)
                    col[hh][2 * p + e] = a
        r0 = pltpu.roll(col[0][3], 1, 0)
        r1 = pltpu.roll(col[1][3], 1, 0)
        d0 = [jnp.where(sub == 0, 0.0, r0), jnp.where(sub == 0, r0, r1)]
        l0 = pltpu.roll(col[0][0], 7, 0)
        l1 = pltpu.roll(col[1][0], 7, 0)
        d5 = [jnp.where(sub == 7, l1, l0), jnp.where(sub == 7, 0.0, l1)]
        for hh in range(2):
            r = _bt6([d0[hh]] + col[hh] + [d5[hh]])
            for j in range(6):
                Wp[s, 2 * j + hh] = r[j]

    def h_tile(Ud, c, t, j, z=None, hpq=()):
        r = []
        for hh in range(2):
            d = [Wp[4 * t + q, 2 * j + hh] for q in range(6)]
            if z is not None:
                for q in hpq:
                    d[q] = z(d[q])
            r.append(_bt6(d))
        r0 = t * 16 if isinstance(t, int) else pl.multiple_of(t * 16, 16)
        for i in range(6):
            Ud[i * 6 + j, c, pl.ds(r0, 16), :] = jnp.concatenate([r[0][i], r[1][i]], axis=0).astype(BF16)

    def produce_rolled(Ud, c):
        sc, sh = finalize(0, c)
        scp[c, 0] = sc
        scp[c, 1] = sh
        for q in range(12):
            Wp[0, q] = zero8

        def rbody(s, _):
            for rr in range(RR):
                w_row(0, 0, c, 1 + s * RR + rr, sc, sh, False)
            return 0
        if RR == NS - 1:
            rbody(0, 0)
        else:
            lax.fori_loop(0, (NS - 1) // RR, rbody, 0)

        def tbody(t, _):
            for tt in range(TR):
                for j in range(6):
                    h_tile(Ud, c, t * TR + tt, j)
            return 0
        if TR == T:
            tbody(0, 0)
        else:
            lax.fori_loop(0, T // TR, tbody, 0)

    def w_part(ksrc, kdst, c, r0, part, z=None):
        def tap(kh, kw):
            return wraw[ksrc, c, kh * 3 + kw, pl.ds(r0, 8), :]

        def cst(v):
            return v if z is None else z(jnp.full((8, 128), v, F32))
        if part in (0, 5):
            j = part
            w = [tap(kh, 0 if part == 0 else 2) for kh in range(3)]
            g = [_unpack(w[kh]) for kh in range(3)]
            c1, c2 = cst(C1), cst(C2)
            r = [_g6(g[0][h], g[1][h], g[2][h], c1, c2) for h in range(2)]
            wt[kdst][j, c, pl.ds(r0, 8), :] = w[0]
            wt[kdst][30 + j, c, pl.ds(r0, 8), :] = w[2]
            for i in range(1, 5):
                wt[kdst][i * 6 + j, c, pl.ds(r0, 8), :] = pltpu.pack_elementwise(
                    [r[0][i], r[1][i]], packed_dtype=BF16)
            return
        cc, pp = (C1, PA_) if part == 1 else (C2, PB_)
        ccv = cst(cc)
        tp = [[None] * 3 for _ in range(2)]
        tm = [[None] * 3 for _ in range(2)]
        for kh in range(3):
            g = [_unpack(tap(kh, kw)) for kw in range(3)]
            for h in range(2):
                e = ccv * g[0][h] + (cc * pp * pp) * g[2][h]
                o = (cc * pp) * g[1][h]
                tp[h][kh] = e + o
                tm[h][kh] = e - o
        for j, t in ((part, tp), (part + 1, tm)):
            r = [_g6(*t[h]) for h in range(2)]
            for i in range(6):
                wt[kdst][i * 6 + j, c, pl.ds(r0, 8), :] = pltpu.pack_elementwise(
                    [r[0][i], r[1][i]], packed_dtype=BF16)

    def w_block(k, c, r0):
        w = [[wraw[k, c, kh * 3 + kw, pl.ds(r0, 8), :] for kw in range(3)] for kh in range(3)]
        g = [[_unpack(w[kh][kw]) for kw in range(3)] for kh in range(3)]
        res = []
        for h in range(2):
            t = [_g6(g[kh][0][h], g[kh][1][h], g[kh][2][h]) for kh in range(3)]
            res.append([_g6(t[0][j], t[1][j], t[2][j]) for j in range(6)])
        for j in range(6):
            for i in range(6):
                if i in (0, 5) and j in (0, 5):
                    v = w[0 if i == 0 else 2][0 if j == 0 else 2]
                else:
                    v = pltpu.pack_elementwise([res[0][j][i], res[1][j][i]], packed_dtype=BF16)
                wt[k][i * 6 + j, c, pl.ds(r0, 8), :] = v

    def w_transform(k, c):
        def body(rb, _):
            w_block(k, c, pl.multiple_of(rb * 8, 8))
            return 0
        lax.fori_loop(0, C // 16, body, 0, unroll=2)

    def conv_body(k, nu, n, Uc, Un, extra, half=0):
        b = (nu // NU) % B
        u = nu % NU
        nn = jnp.minimum(nu + 1, 4 * NU - 1)
        kn = nn // NU
        un = nn % NU
        fmask = zs[pl.ds(0, 8), :] != 0
        n64 = pl.multiple_of(n * 64, 64)

        ms = []
        col = [_AT() for _ in range(4)]
        fin = [[None] * 4 for _ in range(4)]

        def where(a, t, hh, p):
            return u * RU + 4 * t + a, _sl(hh, p)

        def finish(a, bc):
            y = col[a].z[bc]
            vs = []
            for t in range(T):
                for hh in range(2):
                    q = (2 * t + hh) * 8
                    v = y[q:q + 8]
                    if k == 1:
                        row, dst = where(a, t, hh, bc // 2)
                        v = v + pltpu.unpack_elementwise(S[b, n, row, dst, :], index=bc % 2,
                                                         packed_dtype=BF16, unpacked_dtype=F32)
                    vs.append(v)
            fin[a][bc] = vs

        bi = 2 * (2 * k + (0 if extra == 'x' else 1)) + half
        anchor = pltpu.bitcast(wt[k][ORD[0] * 6 + ORD[0], 0, pl.ds(n64, 8), :], F32)
        pend = []

        def col_feed(j, zz, zf=None):
            for q, a in enumerate((1, 2, 0, 3)):
                za = zz[a]
                if zf is not None:
                    z = zf(q)
                    za = jnp.concatenate([z(za[r * 8:r * 8 + 8]) for r in range(M // 8)], axis=0)
                col[a].feed(j, za)
                if j == 4:
                    finish(a, 1)
                    finish(a, 2)
                elif j == 0:
                    finish(a, 0)
                elif j == 5:
                    finish(a, 3)

        for j in ORD:
            at = _AT()
            for i in ORD:
                L = jnp.concatenate(
                    [pltpu.bitcast(Uc.bitcast(U32)[i * 6 + j, c, pl.ds(0, M // 2), :], BF16) for c in range(NCH)], axis=1)
                Wm = jnp.concatenate(
                    [pltpu.bitcast(wt[k][i * 6 + j, c, pl.ds(n64, 64), :], BF16) for c in range(NCH)], axis=1)
                m = lax.dot_general(L, Wm, (((1,), (1,)), ((), ())), preferred_element_type=F32)
                ms.append(m)
                at.feed(i, m)
            pend.append((j, at.z))
            if CP0[bi] < 0 or j in (1, 2, 3):
                col_feed(*pend.pop(0))

        def pacer(tau):
            ph, q = tau // 16, tau % 16
            mv = ms[ph][q * 8:q * 8 + 8, :]
            return lambda v: jnp.where(fmask, mv, v)

        while pend:
            jj, zz = pend.pop(0)
            col_feed(jj, zz, (lambda q: pacer(16 * 24 + CP0[bi] + CPS[bi] * q)) if jj == 4 else None)

        par = n % 2
        sc = scs[par, 0]
        sh = scs[par, 1]
        nu2 = jnp.where(n == NCH - 1, nu + 1, nu)
        kn2 = jnp.minimum(nu2 + 1, 4 * NU - 1) // NU
        n2 = (n + 1) % NCH
        if extra == 'w':
            items = [('w%d' % part, q) for q in range(16) for part in WORDS[WORD[bi]]]
            wc = nu - 1 + n // 2
            wr = pl.multiple_of((n % 2) * 128, 128)
        elif extra == 'x':
            items = [('x', q) for q in range(RU)]
            xsrc = jnp.minimum(nu // 2 + 1, 3)
            xdst = jnp.where(nu == 6, 4, xsrc)
            xs1 = [zero8] * 2
            xs2 = [zero8] * 2
            xpiv = [None, None]
        else:
            items = []
        for it, tau in _schedule(items, k, bi):
            z = pacer(tau)
            if tau < FREE:
                z = lambda v: jnp.where(fmask, anchor, v)
            if it[0] == 'f':
                fsc, fsh = finalize(kn2, n2, z)
                scs[1 - par, 0] = fsc
                scs[1 - par, 1] = fsh
            elif it[0] == 'r':
                s = it[1]
                w_row(kn, un, n, s, z(sc), sh, s == 0 or s == NS - 1)
            elif it[0] == 'h':
                h_tile(Un, n, it[1], it[2], z if PACEH else None, HPQS[HPK[bi]])
            elif it[0][0] == 'w':
                w_part(1, 1, wc, (wr + it[1] * 8) if WHINT else pl.multiple_of(wr + it[1] * 8, 8), int(it[0][1]), z)
            else:
                uu, r0 = it[1] // (RU // 2), (it[1] % (RU // 2)) * 2
                if xpiv[uu] is None:
                    xpiv[uu] = jnp.broadcast_to(_unpack(S[xsrc, n, uu * RU, pl.ds(0, 8), :])[0][0:1, :], (8, 128))
                    xs1 = [zero8] * 2
                    xs2 = [zero8] * 2
                pv = z(xpiv[uu])
                vals = []
                for r in range(2):
                    for q in range(4):
                        vals += list(_unpack(S[xsrc, n, uu * RU + r0 + r, pl.ds(q * 8, 8), :]))
                acc_stats(vals, pv, xs1, xs2)
                if r0 == RU - 2:
                    put_stats(xdst, n, uu, xpiv[uu], xs1, xs2)

        for p in range(2):
            for a in (1, 2, 0, 3):
                for t in range(T):
                    for hh in range(2):
                        row, dst = where(a, t, hh, p)
                        S[(2 + b) if k == 0 else b, n, row, dst, :] = pltpu.pack_elementwise(
                            [fin[a][2 * p][2 * t + hh], fin[a][2 * p + 1][2 * t + hh]], packed_dtype=BF16)
        if k == 1:
            out_copy(b, u, n).start()

    def emb_rows():
        te = temb_ref[...].astype(F32)
        th = 0.5 * te
        sil = th + th * jnp.tanh(th)
        return jnp.dot(sil.astype(BF16), wembs[...], preferred_element_type=F32)

    def pro(c, _):
        x_copy(0, c).wait()
        if 's' not in SKIP:
            x_stats_rolled(0, c)
        if 'u' not in SKIP:
            produce_rolled(UA, c)
        return 0
    lax.fori_loop(0, NCH, pro, 0)
    start_rest(1)
    scs[0, 0] = scp[0, 0]
    scs[0, 1] = scp[0, 1]
    def wpro(q, _):
        c = q // NP
        h = q % NP
        pltpu.make_async_copy(w1_hbm.at[:, pl.ds(0, C // NP), pl.ds(0, 128)],
                              wraw.bitcast(BF16).at[0, c, :, pl.ds(pl.multiple_of(h * (C // NP), C // NP), C // NP)],
                              sems.at[NSEM + q]).wait()

        def body(rb, _):
            for q2 in range(WR):
                w_block(0, c, pl.multiple_of(h * (C // 2 // NP) + (rb * WR + q2) * 8, 8))
            return 0
        lax.fori_loop(0, C // 16 // NP // WR, body, 0)
        return 0
    if 2 in DM:
        lax.fori_loop(0, NCH * NP // 2, wpro, 0)
        start_rest(2)
        lax.fori_loop(NCH * NP // 2, NCH * NP, wpro, 0)
    else:
        lax.fori_loop(0, NCH * NP, wpro, 0)
    start_rest(3)

    def emb_block():
        wemb_copy().wait()
        emb = emb_rows()
        for bb in range(B):
            for c in range(NCH):
                off[2 + bb, c] = jnp.broadcast_to(emb[bb:bb + 1, c * 128:(c + 1) * 128], (8, 128))

    def pair(k):
        def f(p, _):
            nu = 2 * p

            ua = UNRS[0] if k == 0 else UNRS[2]
            ub = UNRS[1] if k == 0 else UNRS[3]

            def fa(n2, _):
                for h in range(ua):
                    if k == 0 and 'x' not in SKIP:
                        @pl.when(p == 0)
                        def _():
                            x_copy(1, n2 * ua + h).wait()
                    conv_body(k, nu, n2 * ua + h, UA, UB, 'x', h)
                return 0

            def fb(n2, _):
                for h in range(ub):
                    conv_body(k, nu + 1, n2 * ub + h, UB, UA, 'w' if k == 0 else None, h)
                return 0
            if k == 0:
                @pl.when(p == 1)
                def _():
                    emb_block()
            lax.fori_loop(0, NCH // ua, fa, 0)
            if k == 0:
                @pl.when(p == 0)
                def _():
                    if 'x' in SKIP:
                        for c in range(NCH):
                            x_copy(1, c).wait()
                    w_copy(1, 0).wait()
                    w_copy(1, 1).wait()

                @pl.when(p == 1)
                def _():
                    w_copy(1, 2).wait()
                    w_copy(1, 3).wait()
            lax.fori_loop(0, NCH // ub, fb, 0)
            return 0
        return f
    if STOP == 'pro0':
        return
    if STOP == 'pro':
        for c in range(NCH):
            x_copy(1, c).wait()
            w_copy(1, c).wait()
        wemb_copy().wait()
        return
    lax.fori_loop(0, NU, pair(0), 0)
    if STOP == 'c1':
        return
    def rep(_, __):
        lax.fori_loop(NU, 2 * NU, pair(1), 0)
        for b in range(B):
            for u in range(NU):
                for c in range(NCH):
                    out_copy(b, u, c).wait()
        return 0
    if REP > 1:
        lax.fori_loop(0, REP, rep, 0)
    else:
        rep(0, 0)


@jax.jit
def pallas_standalone__adm_resblock__diffusion_kernel(x, t_emb, g1, be1, w1, w_emb, g2, be2, w2):
    xn = jnp.transpose(x, (0, 2, 3, 1))
    w1n = jnp.transpose(w1, (2, 3, 0, 1)).reshape(9, C, C)
    w2n = jnp.transpose(w2, (2, 3, 0, 1)).reshape(9, C, C)
    vm = pl.BlockSpec(memory_space=pltpu.VMEM)
    hbm = pl.BlockSpec(memory_space=pl.ANY)
    out = pl.pallas_call(
        _kernel,
        out_shape=jax.ShapeDtypeStruct((B, H, W, C), BF16),
        in_specs=[hbm] * 9,
        out_specs=hbm,
        scratch_shapes=[
            pltpu.VMEM((ZP * 8, 128), U32),
            pltpu.VMEM((4, NCH, H, WT, 128), U32),
            pltpu.VMEM((2, NCH, 9, C // 2, 128), U32),
            pltpu.VMEM((36, NCH, C // 2 + WPAD, 128), U32),
            pltpu.VMEM((36, NCH, C // 2 + WPAD, 128), U32),
            pltpu.VMEM((E, C), BF16),
            pltpu.VMEM((NS, 12 + PPAD, 8, 128), F32),
            pltpu.VMEM((36, NCH, M + UPAD, 128), BF16),
            pltpu.VMEM((36, NCH, M + UPAD, 128), BF16),
            pltpu.VMEM((5, NCH, NU, 3, 8, 128), F32),
            pltpu.VMEM((4, NCH, 8, 128), F32),
            pltpu.VMEM((4, NCH, 8, 128), F32),
            pltpu.VMEM((2, 2, 8, 128), F32),
            pltpu.VMEM((NCH, 2, 8, 128), F32),
            pltpu.VMEM((B, E), BF16),
            pltpu.VMEM((C,), BF16),
            pltpu.VMEM((C,), BF16),
            pltpu.VMEM((C,), BF16),
            pltpu.VMEM((C,), BF16),
            pltpu.SemaphoreType.DMA((NSEM + NCH * NP + 5,)),
        ],
        compiler_params=pltpu.CompilerParams(vmem_limit_bytes=110 * 1024 * 1024),
    )(xn, t_emb, g1, be1, w1n, w_emb, g2, be2, w2n)
    return jnp.transpose(out, (0, 3, 1, 2))
```
